```python
import jax
import jax.numpy as jnp

def _softmax(x, axis=-1):
    return jax.nn.softmax(x, axis=axis)

def _gelu(x):
    return jax.nn.gelu(x, approximate=True)

def _silu(x):
    return jax.nn.silu(x)

def _sigmoid(x):
    return jax.nn.sigmoid(x)

def _layernorm(x, axis=-1, eps=1e-05):
    m = jnp.mean(x, axis=axis, keepdims=True)
    v = jnp.var(x, axis=axis, keepdims=True)
    return (x - m) / jnp.sqrt(v + eps)

def _scatter_add(tgt, idx, src, axis=0):
    return tgt.at[idx].add(src)

def _segment_sum(src, seg, n):
    return jax.ops.segment_sum(src, seg, n)

class _Rng:

    def __init__(self, key):
        self._k = key

    def _next(self):
        self._k, sub = jax.random.split(self._k)
        return sub

    def normal(self, shape):
        return jax.random.normal(self._next(), shape, dtype=jnp.bfloat16)

    def randint(self, lo, hi, shape):
        return jax.random.randint(self._next(), shape, lo, hi, dtype=jnp.int32)

    def uniform(self, shape, lo=0.0, hi=1.0):
        return jax.random.uniform(self._next(), shape, jnp.bfloat16, lo, hi)

    def permutation(self, n):
        return jax.random.permutation(self._next(), n)
kernel_name = 'adaLN_cond__ssm_conv_h3__glu_gated_swiglu__prompt'

def setup_inputs():
    _rng = _Rng(jax.random.key(int.from_bytes(__import__("os").urandom(4), "little")))
    _w = lambda a: (lambda t: t.astype(jnp.bfloat16) if jnp.issubdtype(t.dtype, jnp.floating) else t)(jnp.asarray(a))

    def _A_setup():
        B, S, D = (1, 2048, 640)
        ks = 4
        return {'q': _w((lambda *s: _rng.normal(s) * 0.05)(B, S, D)), 'k': _w((lambda *s: _rng.normal(s) * 0.05)(B, S, D)), 'v': _w((lambda *s: _rng.normal(s) * 0.05)(B, S, D)), 'shift_k': _w((lambda *s: _rng.normal(s) * 0.05)(D, ks) * 0.5), 'ssm_k': _w((lambda *s: _rng.normal(s) * 0.05)(D, S) * (1.0 / S ** 0.5)), 'ssm_D': _w((lambda *s: _rng.normal(s) * 0.05)(D))}
    _A_in = _A_setup()

    def _B_setup():
        B, S, D, F = (1, 2048, 640, 1536)
        return {'x': _w((lambda *s: _rng.normal(s) * 0.05)(B, S, D)), 'w1': _w((lambda *s: _rng.normal(s) * 0.05)(D, F) * (2.0 / D) ** 0.5), 'w3': _w((lambda *s: _rng.normal(s) * 0.05)(D, F) * (2.0 / D) ** 0.5), 'w2': _w((lambda *s: _rng.normal(s) * 0.05)(F, D) * (2.0 / F) ** 0.5)}
    _B_in = _B_setup()
    return {'A_q': _A_in['q'], 'A_k': _A_in['k'], 'A_v': _A_in['v'], 'A_shift_k': _A_in['shift_k'], 'A_ssm_k': _A_in['ssm_k'], 'A_ssm_D': _A_in['ssm_D'], 'B_x': _B_in['x'], 'B_w1': _B_in['w1'], 'B_w3': _B_in['w3'], 'B_w2': _B_in['w2'], 'c': _w((lambda *s: _rng.normal(s) * 0.05)(1, 640)), 'w_mod': _w((lambda *s: _rng.normal(s) * 0.05)(640, 6 * 640) * 640 ** (-0.5))}

def reference(A_q, A_k, A_v, A_shift_k, A_ssm_k, A_ssm_D, B_x, B_w1, B_w3, B_w2, c, w_mod):

    def _A_ref(q, k, v, shift_k, ssm_k, ssm_D):
        B, S, D = q.shape
        ks = shift_k.shape[-1]
        k_pad = jnp.pad(k, ((0, 0), (ks - 1, 0), (0, 0)))
        k_shift = jnp.zeros_like(k)
        for t in range(ks):
            k_shift = k_shift + k_pad[:, t:t + S, :] * shift_k[:, ks - 1 - t][None, None, :]
        kv = k_shift * v
        L = 2 * S
        kv_pad = jnp.pad(kv, ((0, 0), (0, S), (0, 0)))
        kf_pad = jnp.pad(ssm_k, ((0, 0), (0, S)))
        kv_f = (lambda x, axes=(-2, -1): jnp.fft.rfft2(x.astype(jnp.float32), axes=axes))(kv_pad[:, None, :, :], axes=(1, 2))
        kf_f = (lambda x, axes=(-2, -1): jnp.fft.rfft2(x.astype(jnp.float32), axes=axes))(kf_pad[:, None, :], axes=(1, 2))
        kf_f = (lambda x, *d: x.transpose(*d))(kf_f, 1, 2, 0)
        y_f = kv_f * kf_f[None, :, :, :]
        y = (lambda x, s, axes=(-2, -1): jnp.fft.irfft2(x, s=s, axes=axes).astype(jnp.bfloat16))(y_f, (1, L), axes=(1, 2))[:, 0, :S, :]
        y = y + kv * ssm_D[None, None, :]
        return q * y

    def _B_ref(x, w1, w3, w2):
        gate = jnp.einsum('bsd,df->bsf', x, w1)
        up = jnp.einsum('bsd,df->bsf', x, w3)
        h = _silu(gate) * up
        out = jnp.einsum('bsf,fd->bsd', h, w2)
        return out
    x = A_q
    mod = (_silu(c) @ w_mod).reshape(c.shape[0], 6, 1, -1)
    sa, ca, ga, sb, cb, gb = (mod[:, 0].copy(), mod[:, 1].copy(), mod[:, 2].copy(), mod[:, 3].copy(), mod[:, 4].copy(), mod[:, 5].copy())
    h = _layernorm(x, axis=-1) * (1 + ca) + sa
    x = x + ga * _A_ref(h, A_k, A_v, A_shift_k, A_ssm_k, A_ssm_D)
    h = _layernorm(x, axis=-1) * (1 + cb) + sb
    x = x + gb * _B_ref(h, B_w1, B_w3, B_w2)
    return x
```

```python
import numpy as np

import jax
import jax.numpy as jnp
import jax.experimental.pallas as pl
import jax.experimental.pallas.tpu as pltpu

C = 256
H = C // 2
HALO = 16
FT = 256
EPS = 1e-5
F32 = jnp.float32
BF16 = jnp.bfloat16


def _dft_matrices():
    f = np.concatenate([np.arange(0, H, 2), np.arange(1, H, 2)]).astype(np.float64)
    theta = 2.0 * np.pi * (f + 0.5) / (2 * C)
    r = np.arange(H, dtype=np.float64)
    fwd, inv = [], []
    for phase in (0, 1):
        ang = theta[:, None] * (2.0 * r + phase)[None, :]
        m = np.concatenate([np.cos(ang), -np.sin(ang)], axis=0)
        fwd.append(m)
        inv.append(m.T / C)
    return np.stack(fwd).astype(BF16), np.stack(inv).astype(BF16)


def _words(x):
    return pltpu.bitcast(x, jnp.uint32)


def _even(w):
    return pltpu.bitcast(w << 16, F32)


def _odd(w):
    return pltpu.bitcast(w & jnp.uint32(0xFFFF0000), F32)


def _layernorm(x):
    m = jnp.mean(x, axis=-1, keepdims=True)
    d = x - m
    v = jnp.mean(d * d, axis=-1, keepdims=True)
    return d * jax.lax.rsqrt(v + EPS)


def _interleave(*gens):
    gens = list(gens)
    while gens:
        for g in list(gens):
            try:
                next(g)
            except StopIteration:
                gens.remove(g)


def _kernel(q_hbm, k_hbm, v_hbm, shk_hbm, ssmk_hbm, ssmd_hbm, w1_hbm, w3_hbm, w2_hbm, c_hbm,
            wmod_hbm, fwd_hbm, inv_hbm, out_hbm,
            q_v, k_v, v_v, ssmk_v, w1_v, w3_v, w2_v, wmod_v, out_v,
            shk_v, ssmd_v, c_v, fwd_v, inv_v, mod_v,
            kv_s, xu_s, xk_s, uf_s, kf_s, ab_s, prev_s, y_s, h2_s, x2n_s, x2_s, act_s,
            sem_in, sem_w, sem_small, sem_out):
    S, D = q_v.shape
    F = w1_v.shape[1]
    n_chunks = S // C

    def rows(i):
        return pl.ds(pl.multiple_of(i * C, C), C)

    def chunk_copies(i):
        return (
            pltpu.make_async_copy(k_hbm.at[rows(i)],
                                  k_v.at[pl.ds(pl.multiple_of(i * C + HALO, HALO), C)],
                                  sem_in.at[0, i]),
            pltpu.make_async_copy(v_hbm.at[rows(i)], v_v.at[rows(i)], sem_in.at[1, i]),
            pltpu.make_async_copy(ssmk_hbm.at[:, rows(i)], ssmk_v.at[i], sem_in.at[2, i]),
            pltpu.make_async_copy(q_hbm.at[rows(i)], q_v.at[rows(i)], sem_in.at[3, i]),
        )

    def out_copy(i):
        return pltpu.make_async_copy(out_v.at[rows(i)], out_hbm.at[rows(i)], sem_out.at[i])

    small = [pltpu.make_async_copy(s, d, sem_small.at[n]) for n, (s, d) in enumerate(
        ((shk_hbm, shk_v), (fwd_hbm, fwd_v), (inv_hbm, inv_v), (ssmd_hbm, ssmd_v), (c_hbm, c_v)))]
    wmod_copies = [pltpu.make_async_copy(wmod_hbm.at[:, pl.ds(n * D, D)], wmod_v.at[n], sem_w.at[n])
                   for n in range(6)]
    w1_copy = pltpu.make_async_copy(w1_hbm, w1_v, sem_w.at[6])
    w3_copy = pltpu.make_async_copy(w3_hbm, w3_v, sem_w.at[7])
    w2_copy = pltpu.make_async_copy(w2_hbm, w2_v, sem_w.at[8])

    def spectrum(x_ref, dst, slot):
        e = jnp.dot(fwd_v[0], x_ref[0], preferred_element_type=F32)
        t = jnp.dot(fwd_v[1], x_ref[1], preferred_element_type=F32)
        dst[slot, 0:C, :] = e + t
        dst[slot, C:2 * C, :] = e - t

    def conv_chunk(i, first):
        w = [shk_v[j:j + 1, :].astype(F32) for j in range(4)]
        g = 16
        for r in range(0, H, g):
            base = pl.multiple_of(i * C + 2 * r, 2 * g)
            kw = _words(k_v[pl.ds(base, 2 * g + HALO), :])
            k0, k1, k2 = kw[8:8 + g], kw[7:7 + g], kw[6:6 + g]
            vw = _words(v_v[pl.ds(base, 2 * g), :])
            ke, ko, ke1, ko1, ko2 = _even(k0), _odd(k0), _even(k1), _odd(k1), _odd(k2)
            kve = (w[0] * ke + w[1] * ko1 + w[2] * ke1 + w[3] * ko2) * _even(vw)
            kvo = (w[0] * ko + w[1] * ke + w[2] * ko1 + w[3] * ke1) * _odd(vw)
            kv_s[r:r + g, :] = kve
            kv_s[H + r:H + r + g, :] = kvo
            xu_s[0, r:r + g, :] = kve.astype(BF16)
            xu_s[1, r:r + g, :] = kvo.astype(BF16)
        yield
        spectrum(xu_s, uf_s, i)
        yield
        tw = _words(ssmk_v[i].T)
        xk_s[0] = _even(tw).astype(BF16)
        xk_s[1] = _odd(tw).astype(BF16)
        yield
        spectrum(xk_s, kf_s, i)
        yield
        if first:
            terms = [(0, 0)]
        else:
            terms = [(jnp.maximum(i - m, 0), jnp.where(m <= i, m, n_chunks))
                     for m in range(n_chunks)]
        g = 16
        for r in range(0, H, g):
            for l in range(0, D, 128):
                acc = []
                for half in (0, C):
                    re = im = None
                    for us, ks in terms:
                        ur = uf_s[us, half + r:half + r + g, l:l + 128]
                        ui = uf_s[us, half + H + r:half + H + r + g, l:l + 128]
                        kr = kf_s[ks, half + r:half + r + g, l:l + 128]
                        ki = kf_s[ks, half + H + r:half + H + r + g, l:l + 128]
                        pr, pi = ur * kr - ui * ki, ur * ki + ui * kr
                        re, im = (pr, pi) if re is None else (re + pr, im + pi)
                    acc.append((re, im))
                (pr, pi), (qr, qi) = acc
                for n, (re, im) in enumerate(((pr + qr, pi + qi), (pr - qr, pi - qi))):
                    if first:
                        ore, oim = re, im
                    else:
                        lre = prev_s[n, r:r + g, l:l + 128]
                        lim = prev_s[n, H + r:H + r + g, l:l + 128]
                        ore, oim = (re - lim, im + lre) if r < H // 2 else (re + lim, im - lre)
                    prev_s[n, r:r + g, l:l + 128] = re
                    prev_s[n, H + r:H + r + g, l:l + 128] = im
                    ab_s[n, r:r + g, l:l + 128] = ore.astype(BF16)
                    ab_s[n, H + r:H + r + g, l:l + 128] = oim.astype(BF16)
            yield
        for n in range(2):
            y_s[n * H:(n + 1) * H, :] = jnp.dot(inv_v[n], ab_s[n], preferred_element_type=F32)
        yield

    def mix_chunk(i):
        sa, ca, ga, sb, cb = (mod_v[n, 0:1, :] for n in range(5))
        ssm_d = ssmd_v[...].astype(F32)
        g = 16
        for r in range(0, H, g):
            qw = _words(q_v[pl.ds(pl.multiple_of(i * C + 2 * r, 2 * g), 2 * g), :])
            for off, x in ((r, _even(qw)), (H + r, _odd(qw))):
                y = y_s[off:off + g, :] + kv_s[off:off + g, :] * ssm_d
                x2 = x + ga * ((_layernorm(x) * (1.0 + ca) + sa) * y)
                x2n_s[off:off + g, :] = x2
                h2_s[off:off + g, :] = (_layernorm(x2) * (1.0 + cb) + sb).astype(BF16)
            yield

    def prepare(i):
        yield from conv_chunk(i, False)
        yield from mix_chunk(i)

    def ffn_chunk(i):
        x2_s[...] = x2n_s[...]
        h = h2_s[...]
        for j in range(0, F, FT):
            gate = jnp.dot(h, w1_v[:, j:j + FT], preferred_element_type=F32)
            yield
            up = jnp.dot(h, w3_v[:, j:j + FT], preferred_element_type=F32)
            act_s[:, j:j + FT] = (gate * jax.nn.sigmoid(gate) * up).astype(BF16)
            yield
        gb = mod_v[5, 0:1, :]
        for l in range(0, D, 128):
            o = jnp.dot(act_s[...], w2_v[:, l:l + 128], preferred_element_type=F32)
            o = x2_s[:, l:l + 128] + gb[:, l:l + 128] * o
            packed = pltpu.pack_elementwise([o[:H], o[H:]], packed_dtype=BF16)
            out_v[rows(i), l:l + 128] = pltpu.bitcast(packed, BF16)
            yield

    first = chunk_copies(0)
    for cp in (*small, *first[:3], *wmod_copies[:5], first[3], w1_copy, w3_copy, w2_copy,
               wmod_copies[5]):
        cp.start()
    for i in range(1, n_chunks):
        for cp in chunk_copies(i):
            cp.start()

    k_v[0:HALO, :] = jnp.zeros((HALO, D), BF16)
    kf_s[n_chunks] = jnp.zeros(kf_s.shape[1:], F32)
    for cp in (*small, *first[:3]):
        cp.wait()
    _interleave(conv_chunk(0, True))

    cf = c_v[...].astype(F32)
    sc = jnp.broadcast_to(cf * jax.nn.sigmoid(cf), (16, D)).astype(BF16)
    for n in range(5):
        wmod_copies[n].wait()
        mod_v[n] = jnp.dot(sc, wmod_v[n], preferred_element_type=F32)[0:8]
    first[3].wait()
    _interleave(mix_chunk(0))
    for cp in (w1_copy, w3_copy, w2_copy, wmod_copies[5]):
        cp.wait()
    mod_v[5] = jnp.dot(sc, wmod_v[5], preferred_element_type=F32)[0:8]

    def step(i, carry):
        for cp in chunk_copies(i + 1):
            cp.wait()
        _interleave(ffn_chunk(i), prepare(i + 1))
        out_copy(i).start()
        return carry

    jax.lax.fori_loop(0, n_chunks - 1, step, 0)
    _interleave(ffn_chunk(n_chunks - 1))
    out_copy(n_chunks - 1).start()
    for i in range(n_chunks):
        out_copy(i).wait()


@jax.jit
def pallas_adaLN_cond__ssm_conv_h3__glu_gated_swiglu__prompt_kernel(
    A_q: jax.Array,
    A_k: jax.Array,
    A_v: jax.Array,
    A_shift_k: jax.Array,
    A_ssm_k: jax.Array,
    A_ssm_D: jax.Array,
    B_x: jax.Array,
    B_w1: jax.Array,
    B_w3: jax.Array,
    B_w2: jax.Array,
    c: jax.Array,
    w_mod: jax.Array,
):
    del B_x
    B, S, D = A_q.shape
    F = B_w1.shape[1]
    ks = A_shift_k.shape[1]
    assert B == 1 and ks == 4 and S % C == 0 and D % 128 == 0 and F % FT == 0
    n_chunks = S // C
    fwd, inv = _dft_matrices()

    vmem = pltpu.VMEM
    scratch = [
        vmem((S, D), BF16),
        vmem((HALO + S, D), BF16),
        vmem((S, D), BF16),
        vmem((n_chunks, D, C), BF16),
        vmem((D, F), BF16), vmem((D, F), BF16), vmem((F, D), BF16),
        vmem((6, D, D), BF16),
        vmem((S, D), BF16),
        vmem((ks, D), BF16), vmem((1, D), BF16), vmem((1, D), BF16),
        vmem(fwd.shape, BF16), vmem(inv.shape, BF16),
        vmem((6, 8, D), F32),
        vmem((C, D), F32),
        vmem((2, H, D), BF16), vmem((2, H, D), BF16),
        vmem((n_chunks, 2 * C, D), F32),
        vmem((n_chunks + 1, 2 * C, D), F32),
        vmem((2, C, D), BF16),
        vmem((2, C, D), F32),
        vmem((C, D), F32),
        vmem((C, D), BF16),
        vmem((C, D), F32), vmem((C, D), F32),
        vmem((C, F), BF16),
        pltpu.SemaphoreType.DMA((4, n_chunks)),
        pltpu.SemaphoreType.DMA((9,)),
        pltpu.SemaphoreType.DMA((5,)),
        pltpu.SemaphoreType.DMA((n_chunks,)),
    ]
    out = pl.pallas_call(
        _kernel,
        out_shape=jax.ShapeDtypeStruct((S, D), A_q.dtype),
        in_specs=[pl.BlockSpec(memory_space=pl.ANY)] * 13,
        out_specs=pl.BlockSpec(memory_space=pl.ANY),
        scratch_shapes=scratch,
        compiler_params=pltpu.CompilerParams(vmem_limit_bytes=100 * 2**20),
    )(A_q.reshape(S, D), A_k.reshape(S, D), A_v.reshape(S, D), A_shift_k.T, A_ssm_k,
      A_ssm_D.reshape(1, D), B_w1, B_w3, B_w2, c, w_mod, fwd, inv)
    return out.reshape(B, S, D)
```

```python
import functools

import numpy as np

import jax
import jax.numpy as jnp
import jax.experimental.pallas as pl
import jax.experimental.pallas.tpu as pltpu

C = 256
H = C // 2
HALO = 16
FT = 256
EPS = 1e-5
MAC_G = 16
MAC_L = 128
MAC_SEQ = False
FLAGS = {}
POS = (2, 3, 14)
LOOPS = ((1, 7),)
F32 = jnp.float32
BF16 = jnp.bfloat16
U32 = jnp.uint32


def _dft_matrices():
    f = np.concatenate([np.arange(0, H, 2), np.arange(1, H, 2)]).astype(np.float64)
    theta = 2.0 * np.pi * (f + 0.5) / (2 * C)
    r = np.arange(H, dtype=np.float64)
    fwd, inv = [], []
    for phase in (0, 1):
        ang = theta[:, None] * (2.0 * r + phase)[None, :]
        m = np.concatenate([np.cos(ang), -np.sin(ang)], axis=0)
        fwd.append(m)
        inv.append(m.T / C)
    return np.stack(fwd).astype(BF16), np.stack(inv).astype(BF16)


def _words(x):
    return pltpu.bitcast(x, jnp.uint32)


def _halves(w):
    return pltpu.bitcast(w, BF16)


def _even(w):
    return pltpu.bitcast(w << 16, F32)


def _odd(w):
    return pltpu.bitcast(w & jnp.uint32(0xFFFF0000), F32)


def _layernorm(x):
    m = jnp.mean(x, axis=-1, keepdims=True)
    d = x - m
    v = jnp.mean(d * d, axis=-1, keepdims=True)
    return d * jax.lax.rsqrt(v + EPS)


def _silu(x):
    hx = 0.5 * x
    return hx * jnp.tanh(hx) + hx


def _order(a, b, c, n_mac):
    mac = ""
    for n in range(c - b):
        mac += "P" * ((n + 1) * n_mac // (c - b) - n * n_mac // (c - b)) + "F"
    return "PP" + "F" * a + "PP" + "F" * (b - a) + "P" + mac + "P" + "FPP" * 4


def _emit(gens, order=""):
    for key in order:
        next(gens[key], None)
    for g in gens.values():
        for _ in g:
            pass


def _kernel(q_hbm, k_hbm, v_hbm, shk_hbm, ssmk_hbm, ssmd_hbm, w1_hbm, w3_hbm, w2_hbm, c_hbm,
            wmod_hbm, fwd_hbm, inv_hbm, out_hbm,
            q_v, k_v, v_v, ssmk_v, w1_v, w3_v, w2_v, wmod_v, out_v, w1_s, w3_s, w2_s,
            shk_v, ssmd_v, c_v, fwd_v, inv_v, mod_v,
            kv_s, xu_s, xk_s, spec_s, ab_s, y_s, gate_s, h2_s, x2n_s, x2_s, act_s,
            sem_in, sem_mod, sem_w13, sem_w2, sem_small, sem_out):
    S, D = q_v.shape
    F = w1_v.shape[1]
    n_chunks = S // C
    K0, ZERO, PREV = n_chunks, 2 * n_chunks, 2 * n_chunks + 1

    def aligned(start, size, align):
        return pl.ds(start if isinstance(start, int) else pl.multiple_of(start, align), size)

    def rows(i):
        return aligned(i * C, C, C)

    def chunk_copies(i):
        return (
            pltpu.make_async_copy(k_hbm.at[rows(i)],
                                  k_v.at[aligned(i * C + HALO, C, HALO)],
                                  sem_in.at[0, i]),
            pltpu.make_async_copy(v_hbm.at[rows(i)], v_v.at[rows(i)], sem_in.at[1, i]),
            pltpu.make_async_copy(ssmk_hbm.at[:, rows(i)], ssmk_v.at[i], sem_in.at[2, i]),
            pltpu.make_async_copy(q_hbm.at[rows(i)], q_v.at[rows(i)], sem_in.at[3, i]),
        )

    def out_copy(i):
        return pltpu.make_async_copy(out_v.at[rows(i)], out_hbm.at[rows(i)], sem_out.at[i])

    small = [pltpu.make_async_copy(s, d, sem_small.at[n]) for n, (s, d) in enumerate(
        ((shk_hbm, shk_v), (fwd_hbm, fwd_v), (inv_hbm, inv_v), (ssmd_hbm, ssmd_v), (c_hbm, c_v)))]
    wmod_copies = [pltpu.make_async_copy(wmod_hbm.at[:, pl.ds(n * D, D)], wmod_v.at[n], sem_mod.at[n])
                   for n in range(6)]
    w1_copies = [pltpu.make_async_copy(w1_hbm.at[:, pl.ds(j, FT)], w1_v.at[:, pl.ds(j, FT)],
                                       sem_w13.at[0, j // FT]) for j in range(0, F, FT)]
    w3_copies = [pltpu.make_async_copy(w3_hbm.at[:, pl.ds(j, FT)], w3_v.at[:, pl.ds(j, FT)],
                                       sem_w13.at[1, j // FT]) for j in range(0, F, FT)]
    w2_copies = [pltpu.make_async_copy(w2_hbm.at[:, pl.ds(l, 128)], w2_v.at[:, pl.ds(l, 128)],
                                       sem_w2.at[l // 128]) for l in range(0, D, 128)]

    def spectrum(x_ref, slot):
        e = jnp.dot(fwd_v[0], _halves(x_ref[0]), preferred_element_type=F32)
        t = jnp.dot(fwd_v[1], _halves(x_ref[1]), preferred_element_type=F32)
        spec_s[slot, 0:C, :] = e + t
        spec_s[slot, C:2 * C, :] = e - t

    def conv_chunk(i, n_terms):
        w = [shk_v[j:j + 1, :].astype(F32) for j in range(4)]
        g = 32
        for r in range(0, H, g):
            base = i * C + 2 * r
            kw = _words(k_v[aligned(base, 2 * g + HALO, HALO), :])
            k0, k1, k2 = kw[8:], pltpu.roll(kw, 1, 0)[8:], pltpu.roll(kw, 2, 0)[8:]
            vw = _words(v_v[aligned(base, 2 * g, 2 * g), :])
            ke, ko, ke1, ko1, ko2 = _even(k0), _odd(k0), _even(k1), _odd(k1), _odd(k2)
            kve = (w[0] * ke + w[1] * ko1 + w[2] * ke1 + w[3] * ko2) * _even(vw)
            kvo = (w[0] * ko + w[1] * ke + w[2] * ko1 + w[3] * ke1) * _odd(vw)
            kv_s[r:r + g, :] = kve
            kv_s[H + r:H + r + g, :] = kvo
            xu_s[0, r // 2:(r + g) // 2, :] = _words(kve.astype(BF16))
            xu_s[1, r // 2:(r + g) // 2, :] = _words(kvo.astype(BF16))
        yield
        spectrum(xu_s, i)
        yield
        tw = _words(ssmk_v[i].T)
        xk_s[0] = _words(_even(tw).astype(BF16))
        xk_s[1] = _words(_odd(tw).astype(BF16))
        yield
        spectrum(xk_s, K0 + i)
        yield
        first = n_terms == 1
        if isinstance(i, int):
            terms = [(i - m, K0 + m) for m in range(n_terms)]
        else:
            terms = [(jnp.maximum(i - m, 0), jnp.where(m <= i, K0 + m, ZERO))
                     for m in range(n_terms)]
        def products(half, r, l, g):
            re = im = None
            for us, ks in terms:
                ur = spec_s[us, half + r:half + r + g, l:l + MAC_L]
                ui = spec_s[us, half + H + r:half + H + r + g, l:l + MAC_L]
                kr = spec_s[ks, half + r:half + r + g, l:l + MAC_L]
                ki = spec_s[ks, half + H + r:half + H + r + g, l:l + MAC_L]
                if re is None:
                    re, im = ur * kr - ui * ki, ur * ki + ui * kr
                elif MAC_SEQ:
                    re = re + ur * kr
                    im = im + ur * ki
                    re = re - ui * ki
                    im = im + ui * kr
                else:
                    re, im = re + (ur * kr - ui * ki), im + (ur * ki + ui * kr)
            return re, im

        g = MAC_G
        gg = max(16, g)
        for r16 in range(0, H, gg):
            for l in range(0, D, MAC_L):
                outs = []
                for r in range(r16, r16 + gg, g):
                    (pr, pi), (qr, qi) = products(0, r, l, g), products(C, r, l, g)
                    cur = []
                    for n, (re, im) in enumerate(((pr + qr, pi + qi), (pr - qr, pi - qi))):
                        if first:
                            ore, oim = re, im
                        else:
                            lre = spec_s[PREV, n * C + r:n * C + r + g, l:l + MAC_L]
                            lim = spec_s[PREV, n * C + H + r:n * C + H + r + g, l:l + MAC_L]
                            ore, oim = (re - lim, im + lre) if r < H // 2 else (re + lim, im - lre)
                        spec_s[PREV, n * C + r:n * C + r + g, l:l + MAC_L] = re
                        spec_s[PREV, n * C + H + r:n * C + H + r + g, l:l + MAC_L] = im
                        cur += [ore, oim]
                    outs.append(cur)
                for n in range(2):
                    for p in range(2):
                        val = jnp.concatenate([o[2 * n + p] for o in outs], axis=0)
                        row = (p * H + r16) // 2
                        ab_s[n, row:row + gg // 2, l:l + MAC_L] = _words(val.astype(BF16))
                yield
        for n in range(2):
            y_s[n * H:(n + 1) * H, :] = jnp.dot(inv_v[n], _halves(ab_s[n]),
                                                 preferred_element_type=F32)
        yield

    def q_rows(i, r, g):
        qw = _words(q_v[aligned(i * C + 2 * r, 2 * g, 2 * g), :])
        return (r, _even(qw)), (H + r, _odd(qw))

    def gate_chunk(i):
        sa, ca1, ga = (mod_v[n, 0:1, :] for n in range(3))
        g = 16
        for r in range(0, H, g):
            for off, x in q_rows(i, r, g):
                gate_s[off:off + g, :] = ga * (_layernorm(x) * ca1 + sa)
        yield

    def mix_chunk(i):
        sb, cb1 = mod_v[3, 0:1, :], mod_v[4, 0:1, :]
        ssm_d = mod_v[6, 0:1, :]
        g = 16
        for r in range(0, H, g):
            for off, x in q_rows(i, r, g):
                y = y_s[off:off + g, :] + kv_s[off:off + g, :] * ssm_d
                x2 = x + gate_s[off:off + g, :] * y
                x2n_s[off:off + g, :] = x2
                h2 = _layernorm(x2) * cb1 + sb
                h2_s[off // 2:(off + g) // 2, :] = _words(h2.astype(BF16))
            yield

    def prepare(i, n_terms):
        yield from gate_chunk(i)
        yield from conv_chunk(i, n_terms)
        yield from mix_chunk(i)

    def modulation(n):
        cf = c_v[...].astype(F32)
        sc = jnp.broadcast_to(_silu(cf), (16, D)).astype(BF16)
        m = jnp.dot(sc, wmod_v[n], preferred_element_type=F32)[0:8]
        mod_v[n] = 1.0 + m if n in (1, 4) else m

    def ffn_chunk(i, first=False):
        def weight(landed, packed, cols):
            if not first:
                return _halves(packed[:, cols])
            w = landed[:, cols]
            packed[:, cols] = _words(w)
            return w

        x2_s[...] = x2n_s[...]
        for j in range(0, F, FT):
            cols = slice(j, j + FT)
            w1 = weight(w1_v, w1_s, cols)
            gate = jnp.dot(_halves(h2_s[...]), w1, preferred_element_type=F32)
            yield
            w3 = weight(w3_v, w3_s, cols)
            up = jnp.dot(_halves(h2_s[...]), w3, preferred_element_type=F32)
            act_s[:, cols] = _words((_silu(gate) * up).astype(BF16))
            yield
        for l in range(0, D, 128):
            cols = slice(l, l + 128)
            w2 = weight(w2_v, w2_s, cols)
            o = jnp.dot(_halves(act_s[...]), w2, preferred_element_type=F32)
            o = x2_s[:, cols] + mod_v[5, 0:1, cols] * o
            packed = pltpu.pack_elementwise([o[:H], o[H:]], packed_dtype=BF16)
            out_v[rows(i), cols] = pltpu.bitcast(packed, BF16)
            yield

    in0, in1 = chunk_copies(0), chunk_copies(1)
    w13_copies = list(zip(w1_copies, w3_copies))
    queue = [*small, *in0[:3], *wmod_copies[:3], in0[3], *wmod_copies[3:5],
             *w13_copies[0], *w13_copies[1], *in1]
    for pair in w13_copies[2:]:
        queue += pair
    queue += [wmod_copies[5], *w2_copies]
    for cp in queue:
        cp.start()
        pl.delay(1)

    def start_chunk(i, carry):
        for cp in chunk_copies(i):
            cp.start()
        return carry

    jax.lax.fori_loop(2, n_chunks, start_chunk, 0)

    k_v[0:HALO, :] = jnp.zeros((HALO, D), BF16)
    spec_s[ZERO] = jnp.zeros(spec_s.shape[1:], F32)
    with jax.named_scope("wait0"):
        for cp in (*small, *in0[:3]):
            cp.wait()
    with jax.named_scope("conv0"):
        for n in range(D // 128):
            mod_v[6, :, n * 128:(n + 1) * 128] = jnp.broadcast_to(
                ssmd_v[n:n + 1, :].astype(F32), (8, 128))
        _emit({"P": conv_chunk(0, 1)})
    with jax.named_scope("mod"):
        for n in range(3):
            wmod_copies[n].wait()
            modulation(n)
        in0[3].wait()
        _emit({"P": gate_chunk(0)})
        for n in range(3, 5):
            wmod_copies[n].wait()
            modulation(n)
    with jax.named_scope("mix0"):
        _emit({"P": mix_chunk(0)})

    n_mac = (H // max(16, MAC_G)) * (D // MAC_L)

    def arrivals():
        groups = (w13_copies[0], w13_copies[1], in1, w13_copies[2] + w13_copies[3],
                  w13_copies[4] + w13_copies[5], [wmod_copies[5]] + w2_copies[:3], w2_copies[3:])
        for n, group in enumerate(groups):
            for cp in group:
                cp.wait()
            if n == 5:
                modulation(5)
            yield

    with jax.named_scope("step0"):
        _emit({"W": arrivals(), "F": ffn_chunk(0, True), "P": prepare(1, 2)},
              "WFF" "WFF" "WPPPPP" "WFF" + "P" * n_mac + "FF" "WFFPFF" "WFFF" + "P" * 8 + "WFF")
    out_copy(0).start()

    def step(n_terms, i, carry):
        with jax.named_scope("waitc"):
            for cp in chunk_copies(i + 1):
                cp.wait()
        with jax.named_scope("body"):
            _emit({"F": ffn_chunk(i), "P": prepare(i + 1, n_terms)}, _order(*POS, n_mac))
        out_copy(i).start()
        return carry

    for lo, hi in LOOPS:
        if hi - lo == 1:
            step(hi + 1, lo, 0)
        else:
            jax.lax.fori_loop(lo, hi, functools.partial(step, hi + 1), 0)
    with jax.named_scope("last"):
        _emit({"F": ffn_chunk(n_chunks - 1)})
    out_copy(n_chunks - 1).start()
    with jax.named_scope("outwait"):
        for i in range(n_chunks):
            out_copy(i).wait()


@jax.jit
def pallas_adaLN_cond__ssm_conv_h3__glu_gated_swiglu__prompt_kernel(
    A_q: jax.Array,
    A_k: jax.Array,
    A_v: jax.Array,
    A_shift_k: jax.Array,
    A_ssm_k: jax.Array,
    A_ssm_D: jax.Array,
    B_x: jax.Array,
    B_w1: jax.Array,
    B_w3: jax.Array,
    B_w2: jax.Array,
    c: jax.Array,
    w_mod: jax.Array,
):
    del B_x
    B, S, D = A_q.shape
    F = B_w1.shape[1]
    ks = A_shift_k.shape[1]
    assert B == 1 and ks == 4 and S % C == 0 and D % 128 == 0 and F % FT == 0
    n_chunks = S // C
    fwd, inv = _dft_matrices()

    vmem = pltpu.VMEM
    scratch = [
        vmem((S, D), BF16),
        vmem((HALO + S, D), BF16),
        vmem((S, D), BF16),
        vmem((n_chunks, D, C), BF16),
        vmem((D, F), BF16), vmem((D, F), BF16), vmem((F, D), BF16),
        vmem((6, D, D), BF16),
        vmem((S, D), BF16),
        vmem((D // 2, F), U32), vmem((D // 2, F), U32), vmem((F // 2, D), U32),
        vmem((ks, D), BF16), vmem((D // 128, 128), BF16), vmem((1, D), BF16),
        vmem(fwd.shape, BF16), vmem(inv.shape, BF16),
        vmem((7, 8, D), F32),
        vmem((C, D), F32),
        vmem((2, H // 2, D), U32), vmem((2, H // 2, D), U32),
        vmem((2 * n_chunks + 2, 2 * C, D), F32),
        vmem((2, C // 2, D), U32),
        vmem((C, D), F32),
        vmem((C, D), F32),
        vmem((C // 2, D), U32),
        vmem((C, D), F32), vmem((C, D), F32),
        vmem((C // 2, F), U32),
        pltpu.SemaphoreType.DMA((4, n_chunks)),
        pltpu.SemaphoreType.DMA((6,)),
        pltpu.SemaphoreType.DMA((2, F // FT)),
        pltpu.SemaphoreType.DMA((D // 128,)),
        pltpu.SemaphoreType.DMA((5,)),
        pltpu.SemaphoreType.DMA((n_chunks,)),
    ]
    out = pl.pallas_call(
        _kernel,
        out_shape=jax.ShapeDtypeStruct((S, D), A_q.dtype),
        in_specs=[pl.BlockSpec(memory_space=pl.ANY)] * 13,
        out_specs=pl.BlockSpec(memory_space=pl.ANY),
        scratch_shapes=scratch,
        compiler_params=pltpu.CompilerParams(vmem_limit_bytes=100 * 2**20, flags=FLAGS or None),
    )(A_q.reshape(S, D), A_k.reshape(S, D), A_v.reshape(S, D), A_shift_k.T, A_ssm_k,
      A_ssm_D.reshape(D // 128, 128), B_w1, B_w3, B_w2, c, w_mod, fwd, inv)
    return out.reshape(B, S, D)
```

```python
import functools

import numpy as np

import jax
import jax.numpy as jnp
import jax.experimental.pallas as pl
import jax.experimental.pallas.tpu as pltpu

C = 256
H = C // 2
HALO = 16
FT = 256
EPS = 1e-5
PADQ = 16
PADS = 64
KOFF = 32
PREP_G = 32
GATE_G = 16
MIX_G = 16
MAC_G = 16
MAC_L = 128
MAC_SEQ = False
FLAGS = {}
POS = (3, 4, 13)
LOOPS = ((2, 7),)
F32 = jnp.float32
BF16 = jnp.bfloat16
U32 = jnp.uint32


def _dft_matrices():
    f = np.concatenate([np.arange(0, H, 2), np.arange(1, H, 2)]).astype(np.float64)
    theta = 2.0 * np.pi * (f + 0.5) / (2 * C)
    r = np.arange(H, dtype=np.float64)
    fwd, inv = [], []
    for phase in (0, 1):
        ang = theta[:, None] * (2.0 * r + phase)[None, :]
        m = np.concatenate([np.cos(ang), -np.sin(ang)], axis=0)
        fwd.append(m.reshape(C, H // 16, 2, 8).transpose(0, 1, 3, 2).reshape(C, H))
        inv.append(m.reshape(2, H, H).transpose(2, 1, 0).reshape(H, C) / C)
    return np.stack(fwd).astype(BF16), np.stack(inv).astype(BF16)


def _words(x):
    return pltpu.bitcast(x, jnp.uint32)


def _halves(w):
    return pltpu.bitcast(w, BF16)


def _pack(lo, hi):
    return pltpu.bitcast(pltpu.pack_elementwise([lo, hi], packed_dtype=BF16), U32)


def _even(w):
    return pltpu.bitcast(w << 16, F32)


def _odd(w):
    return pltpu.bitcast(w & jnp.uint32(0xFFFF0000), F32)


def _layernorm(x):
    m = jnp.mean(x, axis=-1, keepdims=True)
    d = x - m
    v = jnp.mean(d * d, axis=-1, keepdims=True)
    return d * jax.lax.rsqrt(v + EPS)


def _silu(x):
    hx = 0.5 * x
    return hx * jnp.tanh(hx) + hx


def _order(a, b, c, n_mac):
    mac = ""
    for n in range(c - b):
        mac += "P" * ((n + 1) * n_mac // (c - b) - n * n_mac // (c - b)) + "F"
    return "PP" + "F" * a + "PP" + "F" * (b - a) + "P" + mac + "P" + "FPP" * 4


def _emit(gens, order=""):
    for key in order:
        next(gens[key], None)
    for g in gens.values():
        for _ in g:
            pass


def _kernel(q_hbm, k_hbm, v_hbm, shk_hbm, ssmk_hbm, ssmd_hbm, w1_hbm, w3_hbm, w2_hbm, c_hbm,
            wmod_hbm, fwd_hbm, inv_hbm, out_hbm,
            q_v, k_v, v_v, ssmk_v, w1_v, w3_v, w2_v, wmod_v, out_v, w1_s, w3_s, w2_s,
            shk_v, ssmd_v, c_v, fwd_v, inv_v, mod_v,
            xu_s, xk_s, spec_s, ab_s, y_s, gate_s, h2_s, x2n_s, x2_s, act_s,
            sem_in, sem_mod, sem_w13, sem_w2, sem_small, sem_out):
    S, D = q_v.shape
    F = w1_v.shape[1]
    n_chunks = S // C
    HP = H + PADQ
    K0, ZERO, PREV = n_chunks, 2 * n_chunks, 2 * n_chunks + 1

    def aligned(start, size, align):
        return pl.ds(start if isinstance(start, int) else pl.multiple_of(start, align), size)

    def rows(i):
        return aligned(i * C, C, C)

    def chunk_copies(i):
        return (
            pltpu.make_async_copy(k_hbm.at[rows(i)],
                                  k_v.at[aligned(i * C + HALO, C, HALO)],
                                  sem_in.at[0, i]),
            pltpu.make_async_copy(v_hbm.at[rows(i)], v_v.at[rows(i)], sem_in.at[1, i]),
            pltpu.make_async_copy(ssmk_hbm.at[:, rows(i)], ssmk_v.at[i], sem_in.at[2, i]),
            pltpu.make_async_copy(q_hbm.at[rows(i)], q_v.at[rows(i)], sem_in.at[3, i]),
        )

    def out_copy(i):
        return pltpu.make_async_copy(out_v.at[rows(i)], out_hbm.at[rows(i)], sem_out.at[i])

    small = [pltpu.make_async_copy(s, d, sem_small.at[n]) for n, (s, d) in enumerate(
        ((shk_hbm, shk_v), (fwd_hbm, fwd_v), (inv_hbm, inv_v), (ssmd_hbm, ssmd_v), (c_hbm, c_v)))]
    wmod_copies = [pltpu.make_async_copy(wmod_hbm.at[:, pl.ds(n * D, D)], wmod_v.at[n], sem_mod.at[n])
                   for n in range(6)]
    w1_copies = [pltpu.make_async_copy(w1_hbm.at[:, pl.ds(j, FT)], w1_v.at[:, pl.ds(j, FT)],
                                       sem_w13.at[0, j // FT]) for j in range(0, F, FT)]
    w3_copies = [pltpu.make_async_copy(w3_hbm.at[:, pl.ds(j, FT)], w3_v.at[:, pl.ds(j, FT)],
                                       sem_w13.at[1, j // FT]) for j in range(0, F, FT)]
    w2_copies = [pltpu.make_async_copy(w2_hbm.at[:, pl.ds(l, 128)], w2_v.at[:, pl.ds(l, 128)],
                                       sem_w2.at[l // 128]) for l in range(0, D, 128)]

    def spectrum(x_ref, slot, off, tap0=None):
        e = jnp.dot(fwd_v[0], _halves(x_ref[0]), preferred_element_type=F32)
        t = jnp.dot(fwd_v[1], _halves(x_ref[1]), preferred_element_type=F32)
        if tap0 is not None:
            e = jnp.concatenate([e[:H] + tap0, e[H:]], axis=0)
        for n, x in enumerate((e + t, e - t)):
            spec_s[slot, off + 2 * n * HP:off + 2 * n * HP + H, :] = x[:H]
            spec_s[slot, off + (2 * n + 1) * HP:off + (2 * n + 1) * HP + H, :] = x[H:]

    def ssm_d():
        return jnp.concatenate([ssmd_v[n:n + 1, :] for n in range(D // 128)], axis=1).astype(F32)

    def forward_chunk(i, first=False):
        w = [shk_v[j:j + 1, :].astype(F32) for j in range(4)]
        g = PREP_G
        for r in range(0, H, g):
            base = i * C + 2 * r
            kw = _words(k_v[aligned(base, 2 * g + HALO, HALO), :])
            k0, k1, k2 = kw[8:], pltpu.roll(kw, 1, 0)[8:], pltpu.roll(kw, 2, 0)[8:]
            vw = _words(v_v[aligned(base, 2 * g, 2 * g), :])
            ke, ko, ke1, ko1, ko2 = _even(k0), _odd(k0), _even(k1), _odd(k1), _odd(k2)
            kve = (w[0] * ke + w[1] * ko1 + w[2] * ke1 + w[3] * ko2) * _even(vw)
            kvo = (w[0] * ko + w[1] * ke + w[2] * ko1 + w[3] * ke1) * _odd(vw)
            for n, x in enumerate((kve, kvo)):
                for t in range(0, g, 16):
                    xu_s[n, (r + t) // 2:(r + t) // 2 + 8, :] = _pack(x[t:t + 8], x[t + 8:t + 16])
        yield
        spectrum(xu_s, i, 0)
        yield
        tw = _words(ssmk_v[i].T)
        for t in range(0, H, 16):
            lo, hi = tw[t:t + 8], tw[t + 8:t + 16]
            xk_s[0, t // 2:t // 2 + 8, :] = (lo & U32(0xFFFF)) | (hi << 16)
            xk_s[1, t // 2:t // 2 + 8, :] = (lo >> 16) | (hi & U32(0xFFFF0000))
        yield
        spectrum(xk_s, K0 + i, KOFF, ssm_d() if first else None)
        yield

    def conv_chunk(i, n_terms, dst=0):
        first = n_terms == 1
        if isinstance(i, int):
            terms = [(i - m, K0 + m) for m in range(n_terms)]
        else:
            terms = [(jnp.maximum(i - m, 0), jnp.where(m <= i, K0 + m, ZERO))
                     for m in range(n_terms)]
        def products(half, r, l, g):
            re = im = None
            for us, ks in terms:
                ur = spec_s[us, half + r:half + r + g, l:l + MAC_L]
                ui = spec_s[us, half + HP + r:half + HP + r + g, l:l + MAC_L]
                kr = spec_s[ks, KOFF + half + r:KOFF + half + r + g, l:l + MAC_L]
                ki = spec_s[ks, KOFF + half + HP + r:KOFF + half + HP + r + g, l:l + MAC_L]
                if re is None:
                    re, im = ur * kr - ui * ki, ur * ki + ui * kr
                elif MAC_SEQ:
                    re = re + ur * kr
                    im = im + ur * ki
                    re = re - ui * ki
                    im = im + ui * kr
                else:
                    re, im = re + (ur * kr - ui * ki), im + (ur * ki + ui * kr)
            return re, im

        g = MAC_G
        gg = max(16, g)
        for r16 in range(0, H, gg):
            for l in range(0, D, MAC_L):
                for r in range(r16, r16 + gg, g):
                    (pr, pi), (qr, qi) = products(0, r, l, g), products(2 * HP, r, l, g)
                    for n, (re, im) in enumerate(((pr + qr, pi + qi), (pr - qr, pi - qi))):
                        if first:
                            ore, oim = re, im
                        else:
                            lre = spec_s[PREV, 2 * n * HP + r:2 * n * HP + r + g, l:l + MAC_L]
                            lim = spec_s[PREV, (2 * n + 1) * HP + r:(2 * n + 1) * HP + r + g, l:l + MAC_L]
                            ore, oim = (re - lim, im + lre) if r < H // 2 else (re + lim, im - lre)
                        spec_s[PREV, 2 * n * HP + r:2 * n * HP + r + g, l:l + MAC_L] = re
                        spec_s[PREV, (2 * n + 1) * HP + r:(2 * n + 1) * HP + r + g, l:l + MAC_L] = im
                        ab_s[n, r:r + g, l:l + MAC_L] = _pack(ore, oim)
                yield
        for n in range(2):
            y_s[dst + n * H:dst + (n + 1) * H, :] = jnp.dot(inv_v[n], _halves(ab_s[n]),
                                                 preferred_element_type=F32)
        yield

    def q_rows(i, r, g):
        qw = _words(q_v[aligned(i * C + 2 * r, 2 * g, 2 * g), :])
        return (r, _even(qw)), (H + r, _odd(qw))

    def gate_chunk(i, dst=0):
        sa, ca1, ga = (mod_v[n, 0:1, :] for n in range(3))
        scale, shift = ga * ca1, ga * sa
        g = GATE_G
        for r in range(0, H, g):
            for off, x in q_rows(i, r, g):
                val = _layernorm(x) * scale + shift
                gate_s[dst + off:dst + off + g, :] = val
        yield

    def mix_chunk(i, dst=0):
        sb, cb1 = mod_v[3, 0:1, :], mod_v[4, 0:1, :]
        g = MIX_G
        for r in range(0, H, g):
            for off, x in q_rows(i, r, g):
                x2 = x + gate_s[dst + off:dst + off + g, :] * y_s[dst + off:dst + off + g, :]
                x2n_s[dst + off:dst + off + g, :] = x2
                h2 = _layernorm(x2) * cb1 + sb
                h2_s[(dst + off) // 2:(dst + off + g) // 2, :] = _words(h2.astype(BF16))
            yield

    def prepare(i, n_terms):
        yield from gate_chunk(i)
        yield from forward_chunk(i)
        yield from conv_chunk(i, n_terms)
        yield from mix_chunk(i)

    def modulation(n):
        cf = c_v[...].astype(F32)
        sc = jnp.broadcast_to(_silu(cf), (16, D)).astype(BF16)
        m = jnp.dot(sc, wmod_v[n], preferred_element_type=F32)[0:8]
        mod_v[n] = 1.0 + m if n in (1, 4) else m

    def ffn_chunk(i, n=1, first=False):
        def weight(landed, packed, cols):
            if not first:
                return _halves(packed[:, cols])
            w = landed[:, cols]
            packed[:, cols] = _words(w)
            return w

        x2_s[0:n * C, :] = x2n_s[0:n * C, :]
        for j in range(0, F, FT):
            cols = slice(j, j + FT)
            gate = jnp.dot(_halves(h2_s[0:n * H, :]), weight(w1_v, w1_s, cols),
                           preferred_element_type=F32)
            yield
            up = jnp.dot(_halves(h2_s[0:n * H, :]), weight(w3_v, w3_s, cols),
                         preferred_element_type=F32)
            act_s[0:n * H, cols] = _words((_silu(gate) * up).astype(BF16))
            yield
        for l in range(0, D, 128):
            cols = slice(l, l + 128)
            o = jnp.dot(_halves(act_s[0:n * H, :]), weight(w2_v, w2_s, cols),
                        preferred_element_type=F32)
            o = x2_s[0:n * C, cols] + mod_v[5, 0:1, cols] * o
            for t in range(n):
                out_v[rows(i + t), cols] = _halves(_pack(o[t * C:t * C + H], o[t * C + H:(t + 1) * C]))
            yield

    in0, in1, in2 = chunk_copies(0), chunk_copies(1), chunk_copies(2)
    w13_copies = list(zip(w1_copies, w3_copies))
    queue = [*small, *in0[:3], *in1[:3], *wmod_copies[:3], in0[3], in1[3], *wmod_copies[3:5],
             *w13_copies[0], *w13_copies[1], *in2]
    for pair in w13_copies[2:]:
        queue += pair
    queue += [wmod_copies[5], *w2_copies]
    for cp in queue:
        cp.start()
        pl.delay(1)

    def start_chunk(i, carry):
        for cp in chunk_copies(i):
            cp.start()
        return carry

    jax.lax.fori_loop(3, n_chunks, start_chunk, 0)

    k_v[0:HALO, :] = jnp.zeros((HALO, D), BF16)
    spec_s[ZERO] = jnp.zeros(spec_s.shape[1:], F32)
    with jax.named_scope("conv0"):
        for cp in (*small, *in0[:3]):
            cp.wait()
        _emit({"A": forward_chunk(0, True), "P": conv_chunk(0, 1)})
    with jax.named_scope("conv1"):
        for cp in in1[:3]:
            cp.wait()
        _emit({"A": forward_chunk(1), "P": conv_chunk(1, 2, C)})
    with jax.named_scope("mod"):
        for n in range(3):
            wmod_copies[n].wait()
            modulation(n)
        in0[3].wait()
        in1[3].wait()
        _emit({"P": gate_chunk(0), "Q": gate_chunk(1, C)})
        for n in range(3, 5):
            wmod_copies[n].wait()
            modulation(n)
    with jax.named_scope("mix0"):
        _emit({"P": mix_chunk(0), "Q": mix_chunk(1, C)})

    n_mac = (H // max(16, MAC_G)) * (D // MAC_L)

    def arrivals():
        groups = (w13_copies[0], w13_copies[1] + in2, w13_copies[2] + w13_copies[3],
                  w13_copies[4] + w13_copies[5] + (wmod_copies[5], *w2_copies))
        for n, group in enumerate(groups):
            for cp in group:
                cp.wait()
            if n == 3:
                modulation(5)
            yield

    with jax.named_scope("step0"):
        _emit({"W": arrivals(), "F": ffn_chunk(0, 2, True), "P": prepare(2, 3)},
              "WFF" "WPPFPPFP" "WFF" + "P" * n_mac + "FF" "WFPFFF" + "FPP" * 4)
    out_copy(0).start()
    out_copy(1).start()

    def step(n_terms, i, carry):
        with jax.named_scope("waitc"):
            for cp in chunk_copies(i + 1):
                cp.wait()
        with jax.named_scope("body"):
            _emit({"F": ffn_chunk(i), "P": prepare(i + 1, n_terms)}, _order(*POS, n_mac))
        out_copy(i).start()
        return carry

    for lo, hi in LOOPS:
        if hi - lo == 1:
            step(hi + 1, lo, 0)
        else:
            jax.lax.fori_loop(lo, hi, functools.partial(step, hi + 1), 0)
    with jax.named_scope("last"):
        _emit({"F": ffn_chunk(n_chunks - 1)})
    out_copy(n_chunks - 1).start()
    with jax.named_scope("outwait"):
        for i in range(n_chunks):
            out_copy(i).wait()


@jax.jit
def pallas_adaLN_cond__ssm_conv_h3__glu_gated_swiglu__prompt_kernel(
    A_q: jax.Array,
    A_k: jax.Array,
    A_v: jax.Array,
    A_shift_k: jax.Array,
    A_ssm_k: jax.Array,
    A_ssm_D: jax.Array,
    B_x: jax.Array,
    B_w1: jax.Array,
    B_w3: jax.Array,
    B_w2: jax.Array,
    c: jax.Array,
    w_mod: jax.Array,
):
    del B_x
    B, S, D = A_q.shape
    F = B_w1.shape[1]
    ks = A_shift_k.shape[1]
    assert B == 1 and ks == 4 and S % C == 0 and D % 128 == 0 and F % FT == 0
    n_chunks = S // C
    fwd, inv = _dft_matrices()

    vmem = pltpu.VMEM
    scratch = [
        vmem((S, D), BF16),
        vmem((HALO + S, D), BF16),
        vmem((S, D), BF16),
        vmem((n_chunks, D, C), BF16),
        vmem((D, F), BF16), vmem((D, F), BF16), vmem((F, D), BF16),
        vmem((6, D, D), BF16),
        vmem((S, D), BF16),
        vmem((D // 2, F), U32), vmem((D // 2, F), U32), vmem((F // 2, D), U32),
        vmem((ks, D), BF16), vmem((D // 128, 128), BF16), vmem((1, D), BF16),
        vmem(fwd.shape, BF16), vmem(inv.shape, BF16),
        vmem((6, 8, D), F32),
        vmem((2, H // 2, D), U32), vmem((2, H // 2, D), U32),
        vmem((2 * n_chunks + 2, 4 * (H + PADQ) + PADS, D), F32),
        vmem((2, C // 2, D), U32),
        vmem((2 * C, D), F32),
        vmem((2 * C, D), F32),
        vmem((C, D), U32),
        vmem((2 * C, D), F32), vmem((2 * C, D), F32),
        vmem((C, F), U32),
        pltpu.SemaphoreType.DMA((4, n_chunks)),
        pltpu.SemaphoreType.DMA((6,)),
        pltpu.SemaphoreType.DMA((2, F // FT)),
        pltpu.SemaphoreType.DMA((D // 128,)),
        pltpu.SemaphoreType.DMA((5,)),
        pltpu.SemaphoreType.DMA((n_chunks,)),
    ]
    out = pl.pallas_call(
        _kernel,
        out_shape=jax.ShapeDtypeStruct((S, D), A_q.dtype),
        in_specs=[pl.BlockSpec(memory_space=pl.ANY)] * 13,
        out_specs=pl.BlockSpec(memory_space=pl.ANY),
        scratch_shapes=scratch,
        compiler_params=pltpu.CompilerParams(vmem_limit_bytes=100 * 2**20, flags=FLAGS or None),
    )(A_q.reshape(S, D), A_k.reshape(S, D), A_v.reshape(S, D), A_shift_k.T, A_ssm_k,
      A_ssm_D.reshape(D // 128, 128), B_w1, B_w3, B_w2, c, w_mod, fwd, inv)
    return out.reshape(B, S, D)
```

```python
import functools

import numpy as np

import jax
import jax.numpy as jnp
import jax.experimental.pallas as pl
import jax.experimental.pallas.tpu as pltpu

C = 256
H = C // 2
HALO = 16
FT = 256
EPS = 1e-5
PADQ = 16
PADS = 64
KOFF = 32
PREP_G = 32
GATE_G = 16
MIX_G = 16
MAC_G = 16
MAC_L = 128
MAC_SEQ = False
FLAGS = {}
POS = (3, 4, 13)
LOOPS = ((2, 7),)
F32 = jnp.float32
BF16 = jnp.bfloat16
U32 = jnp.uint32


def _dft_matrices():
    f = np.concatenate([np.arange(0, H, 2), np.arange(1, H, 2)]).astype(np.float64)
    theta = 2.0 * np.pi * (f + 0.5) / (2 * C)
    r = np.arange(H, dtype=np.float64)
    fwd, inv = [], []
    for phase in (0, 1):
        ang = theta[:, None] * (2.0 * r + phase)[None, :]
        m = np.concatenate([np.cos(ang), -np.sin(ang)], axis=0)
        fwd.append(m.reshape(C, H // 16, 2, 8).transpose(0, 1, 3, 2).reshape(C, H))
        inv.append(m.reshape(2, H, H).transpose(2, 1, 0).reshape(H, C) / C)
    return np.stack(fwd).astype(BF16), np.stack(inv).astype(BF16)


def _words(x):
    return pltpu.bitcast(x, jnp.uint32)


def _halves(w):
    return pltpu.bitcast(w, BF16)


def _pack(lo, hi):
    return pltpu.bitcast(pltpu.pack_elementwise([lo, hi], packed_dtype=BF16), U32)


def _even(w):
    return pltpu.bitcast(w << 16, F32)


def _odd(w):
    return pltpu.bitcast(w & jnp.uint32(0xFFFF0000), F32)


def _layernorm(x):
    m = jnp.mean(x, axis=-1, keepdims=True)
    d = x - m
    v = jnp.mean(d * d, axis=-1, keepdims=True)
    return d * jax.lax.rsqrt(v + EPS)


def _silu(x):
    hx = 0.5 * x
    return hx * jnp.tanh(hx) + hx


def _order(a, b, c, n_mac):
    mac = ""
    for n in range(c - b):
        mac += "P" * ((n + 1) * n_mac // (c - b) - n * n_mac // (c - b)) + "F"
    return "PP" + "F" * a + "PP" + "F" * (b - a) + "P" + mac + "P" + "FPP" * 4


def _emit(gens, order=""):
    for key in order:
        next(gens[key], None)
    for g in gens.values():
        for _ in g:
            pass


def _kernel(q_hbm, k_hbm, v_hbm, shk_hbm, ssmk_hbm, ssmd_hbm, w1_hbm, w3_hbm, w2_hbm, c_hbm,
            wmod_hbm, fwd_hbm, inv_hbm, out_hbm,
            q_v, k_v, v_v, ssmk_v, w1_v, w3_v, w2_v, wmod_v, out_v, w1_s, w3_s, w2_s,
            shk_v, ssmd_v, c_v, fwd_v, inv_v, mod_v,
            xu_s, xk_s, spec_s, ab_s, y_s, gate_s, h2_s, x2n_s, x2_s, act_s,
            sem_in, sem_mod, sem_w13, sem_w2, sem_small, sem_out):
    S, D = q_v.shape
    F = w1_v.shape[1]
    n_chunks = S // C
    HP = H + PADQ
    K0, ZERO, PREV = n_chunks, 2 * n_chunks, 2 * n_chunks + 1

    def aligned(start, size, align):
        return pl.ds(start if isinstance(start, int) else pl.multiple_of(start, align), size)

    def rows(i):
        return aligned(i * C, C, C)

    def chunk_copies(i):
        return (
            pltpu.make_async_copy(k_hbm.at[rows(i)],
                                  k_v.at[aligned(i * C + HALO, C, HALO)],
                                  sem_in.at[0, i]),
            pltpu.make_async_copy(v_hbm.at[rows(i)], v_v.at[rows(i)], sem_in.at[1, i]),
            pltpu.make_async_copy(ssmk_hbm.at[:, rows(i)], ssmk_v.at[i], sem_in.at[2, i]),
            pltpu.make_async_copy(q_hbm.at[rows(i)], q_v.at[rows(i)], sem_in.at[3, i]),
        )

    def out_copy(i):
        return pltpu.make_async_copy(out_v.at[rows(i)], out_hbm.at[rows(i)], sem_out.at[i])

    small = [pltpu.make_async_copy(s, d, sem_small.at[n]) for n, (s, d) in enumerate(
        ((shk_hbm, shk_v), (fwd_hbm, fwd_v), (inv_hbm, inv_v), (ssmd_hbm, ssmd_v), (c_hbm, c_v)))]
    wmod_copies = [pltpu.make_async_copy(wmod_hbm.at[:, pl.ds(n * D, D)], wmod_v.at[n], sem_mod.at[n])
                   for n in range(6)]
    w1_copies = [pltpu.make_async_copy(w1_hbm.at[:, pl.ds(j, FT)], w1_v.at[:, pl.ds(j, FT)],
                                       sem_w13.at[0, j // FT]) for j in range(0, F, FT)]
    w3_copies = [pltpu.make_async_copy(w3_hbm.at[:, pl.ds(j, FT)], w3_v.at[:, pl.ds(j, FT)],
                                       sem_w13.at[1, j // FT]) for j in range(0, F, FT)]
    w2_copies = [pltpu.make_async_copy(w2_hbm.at[:, pl.ds(l, 128)], w2_v.at[:, pl.ds(l, 128)],
                                       sem_w2.at[l // 128]) for l in range(0, D, 128)]

    def spectrum(x_ref, slot, off, tap0=None):
        e = jnp.dot(fwd_v[0], _halves(x_ref[0]), preferred_element_type=F32)
        t = jnp.dot(fwd_v[1], _halves(x_ref[1]), preferred_element_type=F32)
        if tap0 is not None:
            e = jnp.concatenate([e[:H] + tap0, e[H:]], axis=0)
        for n, x in enumerate((e + t, e - t)):
            spec_s[slot, off + 2 * n * HP:off + 2 * n * HP + H, :] = x[:H]
            spec_s[slot, off + (2 * n + 1) * HP:off + (2 * n + 1) * HP + H, :] = x[H:]

    def ssm_d():
        return jnp.concatenate([ssmd_v[n:n + 1, :] for n in range(D // 128)], axis=1).astype(F32)

    def forward_chunk(i, first=False):
        w = [shk_v[j:j + 1, :].astype(F32) for j in range(4)]
        g = PREP_G
        for r in range(0, H, g):
            base = i * C + 2 * r
            kw = _words(k_v[aligned(base, 2 * g + HALO, HALO), :])
            k0, k1, k2 = kw[8:], pltpu.roll(kw, 1, 0)[8:], pltpu.roll(kw, 2, 0)[8:]
            vw = _words(v_v[aligned(base, 2 * g, 2 * g), :])
            ke, ko, ke1, ko1, ko2 = _even(k0), _odd(k0), _even(k1), _odd(k1), _odd(k2)
            kve = (w[0] * ke + w[1] * ko1 + w[2] * ke1 + w[3] * ko2) * _even(vw)
            kvo = (w[0] * ko + w[1] * ke + w[2] * ko1 + w[3] * ke1) * _odd(vw)
            for n, x in enumerate((kve, kvo)):
                for t in range(0, g, 16):
                    xu_s[n, (r + t) // 2:(r + t) // 2 + 8, :] = _pack(x[t:t + 8], x[t + 8:t + 16])
        yield
        spectrum(xu_s, i, 0)
        yield
        tw = _words(ssmk_v[i].T)
        for t in range(0, H, 16):
            lo, hi = tw[t:t + 8], tw[t + 8:t + 16]
            xk_s[0, t // 2:t // 2 + 8, :] = (lo & U32(0xFFFF)) | (hi << 16)
            xk_s[1, t // 2:t // 2 + 8, :] = (lo >> 16) | (hi & U32(0xFFFF0000))
        yield
        spectrum(xk_s, K0 + i, KOFF, ssm_d() if first else None)
        yield

    def conv_chunk(i, n_terms, dst=0):
        first = n_terms == 1
        if isinstance(i, int):
            terms = [(i - m, K0 + m) for m in range(n_terms)]
        else:
            terms = [(jnp.maximum(i - m, 0), jnp.where(m <= i, K0 + m, ZERO))
                     for m in range(n_terms)]
        def products(half, r, l, g):
            re = im = None
            for us, ks in terms:
                ur = spec_s[us, half + r:half + r + g, l:l + MAC_L]
                ui = spec_s[us, half + HP + r:half + HP + r + g, l:l + MAC_L]
                kr = spec_s[ks, KOFF + half + r:KOFF + half + r + g, l:l + MAC_L]
                ki = spec_s[ks, KOFF + half + HP + r:KOFF + half + HP + r + g, l:l + MAC_L]
                if re is None:
                    re, im = ur * kr - ui * ki, ur * ki + ui * kr
                elif MAC_SEQ:
                    re = re + ur * kr
                    im = im + ur * ki
                    re = re - ui * ki
                    im = im + ui * kr
                else:
                    re, im = re + (ur * kr - ui * ki), im + (ur * ki + ui * kr)
            return re, im

        g = MAC_G
        gg = max(16, g)
        for r16 in range(0, H, gg):
            for l in range(0, D, MAC_L):
                for r in range(r16, r16 + gg, g):
                    (pr, pi), (qr, qi) = products(0, r, l, g), products(2 * HP, r, l, g)
                    for n, (re, im) in enumerate(((pr + qr, pi + qi), (pr - qr, pi - qi))):
                        if first:
                            ore, oim = re, im
                        else:
                            lre = spec_s[PREV, 2 * n * HP + r:2 * n * HP + r + g, l:l + MAC_L]
                            lim = spec_s[PREV, (2 * n + 1) * HP + r:(2 * n + 1) * HP + r + g, l:l + MAC_L]
                            ore, oim = (re - lim, im + lre) if r < H // 2 else (re + lim, im - lre)
                        spec_s[PREV, 2 * n * HP + r:2 * n * HP + r + g, l:l + MAC_L] = re
                        spec_s[PREV, (2 * n + 1) * HP + r:(2 * n + 1) * HP + r + g, l:l + MAC_L] = im
                        ab_s[n, r:r + g, l:l + MAC_L] = _pack(ore, oim)
                yield
        for n in range(2):
            y_s[dst + n * H:dst + (n + 1) * H, :] = jnp.dot(inv_v[n], _halves(ab_s[n]),
                                                 preferred_element_type=F32)
        yield

    def q_rows(i, r, g):
        qw = _words(q_v[aligned(i * C + 2 * r, 2 * g, 2 * g), :])
        return (r, _even(qw)), (H + r, _odd(qw))

    def gate_chunk(i, dst=0):
        sa, ca1, ga = (mod_v[n, 0:1, :] for n in range(3))
        scale, shift = ga * ca1, ga * sa
        g = GATE_G
        for r in range(0, H, g):
            for off, x in q_rows(i, r, g):
                val = _layernorm(x) * scale + shift
                gate_s[dst + off:dst + off + g, :] = val
        yield

    def mix_chunk(i, dst=0):
        sb, cb1 = mod_v[3, 0:1, :], mod_v[4, 0:1, :]
        g = MIX_G
        for r in range(0, H, g):
            for off, x in q_rows(i, r, g):
                x2 = x + gate_s[dst + off:dst + off + g, :] * y_s[dst + off:dst + off + g, :]
                x2n_s[dst + off:dst + off + g, :] = x2
                h2 = _layernorm(x2) * cb1 + sb
                h2_s[(dst + off) // 2:(dst + off + g) // 2, :] = _words(h2.astype(BF16))
            yield

    def prepare(i, n_terms):
        yield from gate_chunk(i)
        yield from forward_chunk(i)
        yield from conv_chunk(i, n_terms)
        yield from mix_chunk(i)

    def modulation(n):
        cf = c_v[...].astype(F32)
        sc = jnp.broadcast_to(_silu(cf), (16, D)).astype(BF16)
        m = jnp.dot(sc, wmod_v[n], preferred_element_type=F32)[0:8]
        mod_v[n] = 1.0 + m if n in (1, 4) else m

    def ffn_chunk(i, n=1, first=False):
        def weight(landed, packed, cols):
            if not first:
                return _halves(packed[:, cols])
            w = landed[:, cols]
            packed[:, cols] = _words(w)
            return w

        x2_s[0:n * C, :] = x2n_s[0:n * C, :]
        for j in range(0, F, FT):
            cols = slice(j, j + FT)
            gate = jnp.dot(_halves(h2_s[0:n * H, :]), weight(w1_v, w1_s, cols),
                           preferred_element_type=F32)
            yield
            up = jnp.dot(_halves(h2_s[0:n * H, :]), weight(w3_v, w3_s, cols),
                         preferred_element_type=F32)
            act_s[0:n * H, cols] = _words((_silu(gate) * up).astype(BF16))
            yield
        for l in range(0, D, 128):
            cols = slice(l, l + 128)
            o = jnp.dot(_halves(act_s[0:n * H, :]), weight(w2_v, w2_s, cols),
                        preferred_element_type=F32)
            o = x2_s[0:n * C, cols] + mod_v[5, 0:1, cols] * o
            for t in range(n):
                out_v[rows(i + t), cols] = _halves(_pack(o[t * C:t * C + H], o[t * C + H:(t + 1) * C]))
            yield

    in0, in1, in2 = chunk_copies(0), chunk_copies(1), chunk_copies(2)
    w13_copies = list(zip(w1_copies, w3_copies))
    queue = [*small, *in0[:3], *in1[:3], *wmod_copies[:3], in0[3], in1[3], *wmod_copies[3:5],
             *w13_copies[0], *w13_copies[1], *w13_copies[2], *in2]
    for pair in w13_copies[3:]:
        queue += pair
    queue += [wmod_copies[5], *w2_copies]
    for cp in queue:
        cp.start()
        pl.delay(1)

    def start_chunk(i, carry):
        for cp in chunk_copies(i):
            cp.start()
        return carry

    jax.lax.fori_loop(3, n_chunks, start_chunk, 0)

    k_v[0:HALO, :] = jnp.zeros((HALO, D), BF16)
    spec_s[ZERO] = jnp.zeros(spec_s.shape[1:], F32)
    with jax.named_scope("conv0"):
        for cp in (*small, *in0[:3]):
            cp.wait()
        _emit({"A": forward_chunk(0, True), "P": conv_chunk(0, 1)})
    with jax.named_scope("conv1"):
        for cp in in1[:3]:
            cp.wait()
        _emit({"A": forward_chunk(1), "P": conv_chunk(1, 2, C)})
    with jax.named_scope("mod"):
        for n in range(3):
            wmod_copies[n].wait()
            modulation(n)
        in0[3].wait()
        in1[3].wait()
        _emit({"P": gate_chunk(0), "Q": gate_chunk(1, C)})
        for n in range(3, 5):
            wmod_copies[n].wait()
            modulation(n)
    with jax.named_scope("mix0"):
        _emit({"P": mix_chunk(0), "Q": mix_chunk(1, C)})

    n_mac = (H // max(16, MAC_G)) * (D // MAC_L)

    def arrivals():
        groups = (w13_copies[0], w13_copies[1] + w13_copies[2],
                  in2 + w13_copies[3] + w13_copies[4],
                  w13_copies[5] + (wmod_copies[5], *w2_copies))
        for n, group in enumerate(groups):
            for cp in group:
                cp.wait()
            if n == 3:
                modulation(5)
            yield

    with jax.named_scope("step0"):
        _emit({"W": arrivals(), "F": ffn_chunk(0, 2, True), "P": prepare(2, 3)},
              "WFF" "WFFFF" "WPPFFPPFPF" "W" + "P" * n_mac + "FFP" + "FPP" * 4)
    out_copy(0).start()
    out_copy(1).start()

    def step(n_terms, i, carry):
        with jax.named_scope("waitc"):
            for cp in chunk_copies(i + 1):
                cp.wait()
        with jax.named_scope("body"):
            _emit({"F": ffn_chunk(i), "P": prepare(i + 1, n_terms)}, _order(*POS, n_mac))
        out_copy(i).start()
        return carry

    for lo, hi in LOOPS:
        if hi - lo == 1:
            step(hi + 1, lo, 0)
        else:
            jax.lax.fori_loop(lo, hi, functools.partial(step, hi + 1), 0)
    with jax.named_scope("last"):
        _emit({"F": ffn_chunk(n_chunks - 1)})
    out_copy(n_chunks - 1).start()
    with jax.named_scope("outwait"):
        for i in range(n_chunks):
            out_copy(i).wait()


@jax.jit
def pallas_adaLN_cond__ssm_conv_h3__glu_gated_swiglu__prompt_kernel(
    A_q: jax.Array,
    A_k: jax.Array,
    A_v: jax.Array,
    A_shift_k: jax.Array,
    A_ssm_k: jax.Array,
    A_ssm_D: jax.Array,
    B_x: jax.Array,
    B_w1: jax.Array,
    B_w3: jax.Array,
    B_w2: jax.Array,
    c: jax.Array,
    w_mod: jax.Array,
):
    del B_x
    B, S, D = A_q.shape
    F = B_w1.shape[1]
    ks = A_shift_k.shape[1]
    assert B == 1 and ks == 4 and S % C == 0 and D % 128 == 0 and F % FT == 0
    n_chunks = S // C
    fwd, inv = _dft_matrices()

    vmem = pltpu.VMEM
    scratch = [
        vmem((S, D), BF16),
        vmem((HALO + S, D), BF16),
        vmem((S, D), BF16),
        vmem((n_chunks, D, C), BF16),
        vmem((D, F), BF16), vmem((D, F), BF16), vmem((F, D), BF16),
        vmem((6, D, D), BF16),
        vmem((S, D), BF16),
        vmem((D // 2, F), U32), vmem((D // 2, F), U32), vmem((F // 2, D), U32),
        vmem((ks, D), BF16), vmem((D // 128, 128), BF16), vmem((1, D), BF16),
        vmem(fwd.shape, BF16), vmem(inv.shape, BF16),
        vmem((6, 8, D), F32),
        vmem((2, H // 2, D), U32), vmem((2, H // 2, D), U32),
        vmem((2 * n_chunks + 2, 4 * (H + PADQ) + PADS, D), F32),
        vmem((2, C // 2, D), U32),
        vmem((2 * C, D), F32),
        vmem((2 * C, D), F32),
        vmem((C, D), U32),
        vmem((2 * C, D), F32), vmem((2 * C, D), F32),
        vmem((C, F), U32),
        pltpu.SemaphoreType.DMA((4, n_chunks)),
        pltpu.SemaphoreType.DMA((6,)),
        pltpu.SemaphoreType.DMA((2, F // FT)),
        pltpu.SemaphoreType.DMA((D // 128,)),
        pltpu.SemaphoreType.DMA((5,)),
        pltpu.SemaphoreType.DMA((n_chunks,)),
    ]
    out = pl.pallas_call(
        _kernel,
        out_shape=jax.ShapeDtypeStruct((S, D), A_q.dtype),
        in_specs=[pl.BlockSpec(memory_space=pl.ANY)] * 13,
        out_specs=pl.BlockSpec(memory_space=pl.ANY),
        scratch_shapes=scratch,
        compiler_params=pltpu.CompilerParams(vmem_limit_bytes=100 * 2**20, flags=FLAGS or None),
    )(A_q.reshape(S, D), A_k.reshape(S, D), A_v.reshape(S, D), A_shift_k.T, A_ssm_k,
      A_ssm_D.reshape(D // 128, 128), B_w1, B_w3, B_w2, c, w_mod, fwd, inv)
    return out.reshape(B, S, D)
```

```python
import functools

import numpy as np

import jax
import jax.numpy as jnp
import jax.experimental.pallas as pl
import jax.experimental.pallas.tpu as pltpu

C = 256
H = C // 2
HALO = 16
FT = 256
EPS = 1e-5
LAST_AT = (0, 1, 2, 3, 4)
STATIC_K = True
PADQ = 16
PADS = 64
KOFF = 32
PREP_G = 32
GATE_G = 16
MIX_G = 16
MAC_G = 16
MAC_L = 128
MAC_SEQ = False
FLAGS = {}
POS = (2, 4, 14)
LOOPS = ((2, 7),)
F32 = jnp.float32
BF16 = jnp.bfloat16
U32 = jnp.uint32


def _dft_matrices():
    f = np.concatenate([np.arange(0, H, 2), np.arange(1, H, 2)]).astype(np.float64)
    theta = 2.0 * np.pi * (f + 0.5) / (2 * C)
    r = np.arange(H, dtype=np.float64)
    fwd, inv = [], []
    for phase in (0, 1):
        ang = theta[:, None] * (2.0 * r + phase)[None, :]
        m = np.concatenate([np.cos(ang), -np.sin(ang)], axis=0)
        fwd.append(m.reshape(C, H // 16, 2, 8).transpose(0, 1, 3, 2).reshape(C, H))
        inv.append(m.reshape(2, H, H).transpose(2, 1, 0).reshape(H, C) / C)
    return np.stack(fwd).astype(BF16), np.stack(inv).astype(BF16)


def _words(x):
    return pltpu.bitcast(x, jnp.uint32)


def _halves(w):
    return pltpu.bitcast(w, BF16)


def _pack(lo, hi):
    return pltpu.bitcast(pltpu.pack_elementwise([lo, hi], packed_dtype=BF16), U32)


def _even(w):
    return pltpu.bitcast(w << 16, F32)


def _odd(w):
    return pltpu.bitcast(w & jnp.uint32(0xFFFF0000), F32)


def _layernorm(x):
    m = jnp.mean(x, axis=-1, keepdims=True)
    d = x - m
    v = jnp.mean(d * d, axis=-1, keepdims=True)
    return d * jax.lax.rsqrt(v + EPS)


def _silu(x):
    hx = 0.5 * x
    return hx * jnp.tanh(hx) + hx


def _order(a, b, c, n_mac):
    mac = ""
    for n in range(c - b):
        mac += "P" * ((n + 1) * n_mac // (c - b) - n * n_mac // (c - b)) + "F"
    return "PP" + "F" * a + "PP" + "F" * (b - a) + "P" + mac + "P" + "FPP" * 4


def _emit(gens, order=""):
    for key in order:
        next(gens[key], None)
    for g in gens.values():
        for _ in g:
            pass


def _kernel(q_hbm, k_hbm, v_hbm, shk_hbm, ssmk_hbm, ssmd_hbm, w1_hbm, w3_hbm, w2_hbm, c_hbm,
            wmod_hbm, fwd_hbm, inv_hbm, out_hbm,
            q_v, k_v, v_v, ssmk_v, w1_v, w3_v, w2_v, wmod_v, out_v, w1_s, w3_s, w2_s,
            shk_v, ssmd_v, c_v, fwd_v, inv_v, mod_v,
            xu_s, xk_s, spec_s, ab_s, y_s, gate_s, h2_s, x2n_s, x2_s, act_s,
            sem_in, sem_start, sem_out):
    S, D = q_v.shape
    F = w1_v.shape[1]
    n_chunks = S // C
    HP = H + PADQ
    K0, PREV = n_chunks, 2 * n_chunks

    def aligned(start, size, align):
        return pl.ds(start if isinstance(start, int) else pl.multiple_of(start, align), size)

    def rows(i):
        return aligned(i * C, C, C)

    def chunk_refs(i):
        return [(k_hbm.at[rows(i)], k_v.at[aligned(i * C + HALO, C, HALO)]),
                (v_hbm.at[rows(i)], v_v.at[rows(i)]),
                (ssmk_hbm.at[:, rows(i)], ssmk_v.at[i]),
                (q_hbm.at[rows(i)], q_v.at[rows(i)])]

    def chunk_copies(i):
        return [pltpu.make_async_copy(s, d, sem_in.at[i - 3]) for s, d in chunk_refs(i)]

    def out_copy(i, cols=slice(None)):
        return pltpu.make_async_copy(out_v.at[rows(i), cols], out_hbm.at[rows(i), cols], sem_out)

    last_copies = [out_copy(n_chunks - 1, pl.ds(l, 128)) for l in range(0, D, 128)]

    wmod_refs = [(wmod_hbm.at[:, pl.ds(n * D, D)], wmod_v.at[n]) for n in range(6)]
    w13_refs = [[(w1_hbm.at[:, pl.ds(j, FT)], w1_v.at[:, pl.ds(j, FT)]),
                 (w3_hbm.at[:, pl.ds(j, FT)], w3_v.at[:, pl.ds(j, FT)])] for j in range(0, F, FT)]
    start_groups = [
        [(shk_hbm, shk_v), (fwd_hbm, fwd_v), (inv_hbm, inv_v), (ssmd_hbm, ssmd_v), (c_hbm, c_v)]
        + chunk_refs(0)[:3],
        chunk_refs(1)[:3],
        wmod_refs[:3] + [chunk_refs(0)[3], chunk_refs(1)[3]],
        wmod_refs[3:4],
        wmod_refs[4:5],
        w13_refs[0],
        w13_refs[1] + w13_refs[2],
        chunk_refs(2) + w13_refs[3] + w13_refs[4],
        w13_refs[5] + [wmod_refs[5], (w2_hbm, w2_v)],
    ]
    start_groups = [[pltpu.make_async_copy(s, d, sem_start.at[n]) for s, d in group]
                    for n, group in enumerate(start_groups)]

    def wait_group(n):
        for cp in start_groups[n]:
            cp.wait()

    def spectrum(x_ref, slot, off, tap0=None):
        e = jnp.dot(fwd_v[0], _halves(x_ref[0]), preferred_element_type=F32)
        t = jnp.dot(fwd_v[1], _halves(x_ref[1]), preferred_element_type=F32)
        if tap0 is not None:
            e = jnp.concatenate([e[:H] + tap0, e[H:]], axis=0)
        for n, x in enumerate((e + t, e - t)):
            spec_s[slot, off + 2 * n * HP:off + 2 * n * HP + H, :] = x[:H]
            spec_s[slot, off + (2 * n + 1) * HP:off + (2 * n + 1) * HP + H, :] = x[H:]

    def ssm_d():
        return jnp.concatenate([ssmd_v[n:n + 1, :] for n in range(D // 128)], axis=1).astype(F32)

    def forward_chunk(i, first=False):
        w = [shk_v[j:j + 1, :].astype(F32) for j in range(4)]
        g = PREP_G
        for r in range(0, H, g):
            base = i * C + 2 * r
            kw = _words(k_v[aligned(base, 2 * g + HALO, HALO), :])
            k0, k1, k2 = kw[8:], pltpu.roll(kw, 1, 0)[8:], pltpu.roll(kw, 2, 0)[8:]
            vw = _words(v_v[aligned(base, 2 * g, 2 * g), :])
            ke, ko, ke1, ko1, ko2 = _even(k0), _odd(k0), _even(k1), _odd(k1), _odd(k2)
            kve = (w[0] * ke + w[1] * ko1 + w[2] * ke1 + w[3] * ko2) * _even(vw)
            kvo = (w[0] * ko + w[1] * ke + w[2] * ko1 + w[3] * ke1) * _odd(vw)
            for n, x in enumerate((kve, kvo)):
                for t in range(0, g, 16):
                    xu_s[n, (r + t) // 2:(r + t) // 2 + 8, :] = _pack(x[t:t + 8], x[t + 8:t + 16])
        yield
        spectrum(xu_s, i, 0)
        yield
        tw = _words(ssmk_v[i].T)
        for t in range(0, H, 16):
            lo, hi = tw[t:t + 8], tw[t + 8:t + 16]
            xk_s[0, t // 2:t // 2 + 8, :] = (lo & U32(0xFFFF)) | (hi << 16)
            xk_s[1, t // 2:t // 2 + 8, :] = (lo >> 16) | (hi & U32(0xFFFF0000))
        yield
        spectrum(xk_s, K0 + i, KOFF, ssm_d() if first else None)
        yield

    def conv_chunk(i, n_terms, dst=0):
        first = n_terms == 1
        if isinstance(i, int):
            terms = [(i - m, K0 + m) for m in range(n_terms)]
        else:
            if STATIC_K:
                terms = [(jnp.maximum(i - m, 0), K0 + m) for m in range(n_terms)]
            else:
                terms = [(m, K0 + jnp.maximum(i - m, 0)) for m in range(n_terms)]
        def products(half, r, l, g):
            re = im = None
            for us, ks in terms:
                ur = spec_s[us, half + r:half + r + g, l:l + MAC_L]
                ui = spec_s[us, half + HP + r:half + HP + r + g, l:l + MAC_L]
                kr = spec_s[ks, KOFF + half + r:KOFF + half + r + g, l:l + MAC_L]
                ki = spec_s[ks, KOFF + half + HP + r:KOFF + half + HP + r + g, l:l + MAC_L]
                if re is None:
                    re, im = ur * kr - ui * ki, ur * ki + ui * kr
                elif MAC_SEQ:
                    re = re + ur * kr
                    im = im + ur * ki
                    re = re - ui * ki
                    im = im + ui * kr
                else:
                    re, im = re + (ur * kr - ui * ki), im + (ur * ki + ui * kr)
            return re, im

        g = MAC_G
        gg = max(16, g)
        for r16 in range(0, H, gg):
            for l in range(0, D, MAC_L):
                for r in range(r16, r16 + gg, g):
                    (pr, pi), (qr, qi) = products(0, r, l, g), products(2 * HP, r, l, g)
                    for n, (re, im) in enumerate(((pr + qr, pi + qi), (pr - qr, pi - qi))):
                        if first:
                            ore, oim = re, im
                        else:
                            lre = spec_s[PREV, 2 * n * HP + r:2 * n * HP + r + g, l:l + MAC_L]
                            lim = spec_s[PREV, (2 * n + 1) * HP + r:(2 * n + 1) * HP + r + g, l:l + MAC_L]
                            ore, oim = (re - lim, im + lre) if r < H // 2 else (re + lim, im - lre)
                        spec_s[PREV, 2 * n * HP + r:2 * n * HP + r + g, l:l + MAC_L] = re
                        spec_s[PREV, (2 * n + 1) * HP + r:(2 * n + 1) * HP + r + g, l:l + MAC_L] = im
                        ab_s[n, r:r + g, l:l + MAC_L] = _pack(ore, oim)
                yield
        for n in range(2):
            y_s[dst + n * H:dst + (n + 1) * H, :] = jnp.dot(inv_v[n], _halves(ab_s[n]),
                                                 preferred_element_type=F32)
        yield

    def q_rows(i, r, g):
        qw = _words(q_v[aligned(i * C + 2 * r, 2 * g, 2 * g), :])
        return (r, _even(qw)), (H + r, _odd(qw))

    def gate_chunk(i, dst=0):
        sa, ca1, ga = (mod_v[n, 0:1, :] for n in range(3))
        scale, shift = ga * ca1, ga * sa
        g = GATE_G
        for r in range(0, H, g):
            for off, x in q_rows(i, r, g):
                val = _layernorm(x) * scale + shift
                gate_s[dst + off:dst + off + g, :] = val
        yield

    def mix_chunk(i, dst=0):
        sb, cb1 = mod_v[3, 0:1, :], mod_v[4, 0:1, :]
        g = MIX_G
        for r in range(0, H, g):
            for off, x in q_rows(i, r, g):
                x2 = x + gate_s[dst + off:dst + off + g, :] * y_s[dst + off:dst + off + g, :]
                x2n_s[dst + off:dst + off + g, :] = x2
                h2 = _layernorm(x2) * cb1 + sb
                h2_s[(dst + off) // 2:(dst + off + g) // 2, :] = _words(h2.astype(BF16))
            yield

    def prepare(i, n_terms):
        yield from gate_chunk(i)
        yield from forward_chunk(i)
        yield from conv_chunk(i, n_terms)
        yield from mix_chunk(i)

    def modulation(n):
        cf = c_v[...].astype(F32)
        sc = jnp.broadcast_to(_silu(cf), (16, D)).astype(BF16)
        m = jnp.dot(sc, wmod_v[n], preferred_element_type=F32)[0:8]
        m = 1.0 + m if n in (1, 4) else m
        mod_v[n] = m * {3: 0.5, 4: 0.5, 5: 2.0}.get(n, 1.0)

    def ffn_chunk(i, n=1, first=False, last=False):
        def weight(landed, packed, cols):
            if not first:
                return _halves(packed[:, cols])
            w = landed[:, cols]
            packed[:, cols] = _words(w)
            return w

        x2_s[0:n * C, :] = x2n_s[0:n * C, :]
        for j in range(0, F, FT):
            cols = slice(j, j + FT)
            gate = jnp.dot(_halves(h2_s[0:n * H, :]), weight(w1_v, w1_s, cols),
                           preferred_element_type=F32)
            yield
            up = jnp.dot(_halves(h2_s[0:n * H, :]), weight(w3_v, w3_s, cols),
                         preferred_element_type=F32)
            act_s[0:n * H, cols] = _words(((gate * jnp.tanh(gate) + gate) * up).astype(BF16))
            yield
        for l in range(0, D, 128):
            cols = slice(l, l + 128)
            o = jnp.dot(_halves(act_s[0:n * H, :]), weight(w2_v, w2_s, cols),
                        preferred_element_type=F32)
            o = x2_s[0:n * C, cols] + mod_v[5, 0:1, cols] * o
            for t in range(n):
                out_v[rows(i + t), cols] = _halves(_pack(o[t * C:t * C + H], o[t * C + H:(t + 1) * C]))
            if last and l // 128 in LAST_AT:
                for cp in last_copies[max([-1] + [x for x in LAST_AT if x < l // 128]) + 1:l // 128 + 1]:
                    cp.start()
            yield

    for group in start_groups:
        for cp in group:
            cp.start()
        pl.delay(1)

    def start_chunk(i, carry):
        for cp in chunk_copies(i):
            cp.start()
        return carry

    jax.lax.fori_loop(3, n_chunks, start_chunk, 0)

    k_v[0:HALO, :] = jnp.zeros((HALO, D), BF16)
    for m in range(3, n_chunks):
        for n in range(4):
            if STATIC_K:
                spec_s[K0 + m, KOFF + n * HP:KOFF + n * HP + H, :] = jnp.zeros((H, D), F32)
            else:
                spec_s[m, n * HP:n * HP + H, :] = jnp.zeros((H, D), F32)
    with jax.named_scope("conv0"):
        wait_group(0)
        _emit({"A": forward_chunk(0, True), "P": conv_chunk(0, 1)})
    with jax.named_scope("conv1"):
        wait_group(1)
        _emit({"A": forward_chunk(1), "P": conv_chunk(1, 2, C)})
    with jax.named_scope("mod"):
        wait_group(2)
        for n in range(3):
            modulation(n)
        _emit({"P": gate_chunk(0), "Q": gate_chunk(1, C)})
        for n in range(3, 5):
            wait_group(n)
            modulation(n)
    with jax.named_scope("mix0"):
        _emit({"P": mix_chunk(0), "Q": mix_chunk(1, C)})

    n_mac = (H // max(16, MAC_G)) * (D // MAC_L)

    def arrivals():
        for n in range(5, 9):
            wait_group(n)
            if n == 8:
                modulation(5)
            yield

    with jax.named_scope("step0"):
        _emit({"W": arrivals(), "F": ffn_chunk(0, 2, True), "P": prepare(2, 3)},
              "WFF" "WFFFF" "WPPFFPPFPF" "W" + "P" * n_mac + "FFP" + "FPP" * 4)
    out_copy(0).start()
    out_copy(1).start()

    def step(n_terms, i, carry):
        with jax.named_scope("waitc"):
            for cp in chunk_copies(i + 1):
                cp.wait()
        with jax.named_scope("body"):
            _emit({"F": ffn_chunk(i), "P": prepare(i + 1, n_terms)}, _order(*POS, n_mac))
        out_copy(i).start()
        return carry

    for lo, hi in LOOPS:
        if hi - lo == 1:
            step(hi + 1, lo, 0)
        else:
            jax.lax.fori_loop(lo, hi, functools.partial(step, hi + 1), 0)
    with jax.named_scope("last"):
        _emit({"F": ffn_chunk(n_chunks - 1, last=True)})
    with jax.named_scope("outwait"):
        for i in range(n_chunks - 1):
            out_copy(i).wait()
        for cp in last_copies:
            cp.wait()


@jax.jit
def pallas_adaLN_cond__ssm_conv_h3__glu_gated_swiglu__prompt_kernel(
    A_q: jax.Array,
    A_k: jax.Array,
    A_v: jax.Array,
    A_shift_k: jax.Array,
    A_ssm_k: jax.Array,
    A_ssm_D: jax.Array,
    B_x: jax.Array,
    B_w1: jax.Array,
    B_w3: jax.Array,
    B_w2: jax.Array,
    c: jax.Array,
    w_mod: jax.Array,
):
    del B_x
    B, S, D = A_q.shape
    F = B_w1.shape[1]
    ks = A_shift_k.shape[1]
    assert B == 1 and ks == 4 and S % C == 0 and D % 128 == 0 and F % FT == 0
    n_chunks = S // C
    fwd, inv = _dft_matrices()

    vmem = pltpu.VMEM
    scratch = [
        vmem((S, D), BF16),
        vmem((HALO + S, D), BF16),
        vmem((S, D), BF16),
        vmem((n_chunks, D, C), BF16),
        vmem((D, F), BF16), vmem((D, F), BF16), vmem((F, D), BF16),
        vmem((6, D, D), BF16),
        vmem((S, D), BF16),
        vmem((D // 2, F), U32), vmem((D // 2, F), U32), vmem((F // 2, D), U32),
        vmem((ks, D), BF16), vmem((D // 128, 128), BF16), vmem((1, D), BF16),
        vmem(fwd.shape, BF16), vmem(inv.shape, BF16),
        vmem((6, 8, D), F32),
        vmem((2, H // 2, D), U32), vmem((2, H // 2, D), U32),
        vmem((2 * n_chunks + 1, 4 * (H + PADQ) + PADS, D), F32),
        vmem((2, C // 2, D), U32),
        vmem((2 * C, D), F32),
        vmem((2 * C, D), F32),
        vmem((C, D), U32),
        vmem((2 * C, D), F32), vmem((2 * C, D), F32),
        vmem((C, F), U32),
        pltpu.SemaphoreType.DMA((n_chunks - 3,)),
        pltpu.SemaphoreType.DMA((9,)),
        pltpu.SemaphoreType.DMA(()),
    ]
    out = pl.pallas_call(
        _kernel,
        out_shape=jax.ShapeDtypeStruct((S, D), A_q.dtype),
        in_specs=[pl.BlockSpec(memory_space=pl.ANY)] * 13,
        out_specs=pl.BlockSpec(memory_space=pl.ANY),
        scratch_shapes=scratch,
        compiler_params=pltpu.CompilerParams(vmem_limit_bytes=100 * 2**20, **FLAGS),
    )(A_q.reshape(S, D), A_k.reshape(S, D), A_v.reshape(S, D), A_shift_k.T, A_ssm_k,
      A_ssm_D.reshape(D // 128, 128), B_w1, B_w3, B_w2, c, w_mod, fwd, inv)
    return out.reshape(B, S, D)
```

```python
import functools

import numpy as np

import jax
import jax.numpy as jnp
import jax.experimental.pallas as pl
import jax.experimental.pallas.tpu as pltpu

C = 256
H = C // 2
HALO = 16
FT = 256
EPS = 1e-5
OPAQUE = True
ORDER0 = "WFF" "WFFFF" "WFFFF" "WPFF" + "FPP" * 4
ORDER1 = "A" + "P" * 40 + "AAAP"
LAST_AT = (0, 1, 2, 3, 4)
STATIC_K = True
PADQ = 24
PADS = 96
KOFF = 48
PREP_G = 32
GATE_G = 16
MIX_G = 16
MAC_G = 16
MAC_L = 128
MAC_SEQ = False
FLAGS = {}
POS = (2, 4, 14)
LOOPS = ((2, 7),)
F32 = jnp.float32
BF16 = jnp.bfloat16
U32 = jnp.uint32


def _dft_matrices():
    f = np.concatenate([np.arange(0, H, 2), np.arange(1, H, 2)]).astype(np.float64)
    theta = 2.0 * np.pi * (f + 0.5) / (2 * C)
    r = np.arange(H, dtype=np.float64)
    fwd, inv = [], []
    for phase in (0, 1):
        ang = theta[:, None] * (2.0 * r + phase)[None, :]
        m = np.concatenate([np.cos(ang), -np.sin(ang)], axis=0)
        fwd.append(m.reshape(C, H // 16, 2, 8).transpose(0, 1, 3, 2).reshape(C, H))
        inv.append(m.reshape(2, H, H).transpose(2, 1, 0).reshape(H, C) / C)
    return np.stack(fwd).astype(BF16), np.stack(inv).astype(BF16)


def _words(x):
    return pltpu.bitcast(x, jnp.uint32)


def _halves(w):
    return pltpu.bitcast(w, BF16)


def _pack(lo, hi):
    return pltpu.bitcast(pltpu.pack_elementwise([lo, hi], packed_dtype=BF16), U32)


def _even(w):
    return pltpu.bitcast(w << 16, F32)


def _odd(w):
    return pltpu.bitcast(w & jnp.uint32(0xFFFF0000), F32)


def _layernorm(x):
    m = jnp.mean(x, axis=-1, keepdims=True)
    d = x - m
    v = jnp.mean(d * d, axis=-1, keepdims=True)
    return d * jax.lax.rsqrt(v + EPS)


def _silu(x):
    hx = 0.5 * x
    return hx * jnp.tanh(hx) + hx


def _order(a, b, c, n_mac):
    mac = ""
    for n in range(c - b):
        mac += "P" * ((n + 1) * n_mac // (c - b) - n * n_mac // (c - b)) + "F"
    return "PP" + "F" * a + "PP" + "F" * (b - a) + "P" + mac + "P" + "FPP" * 4


def _emit(gens, order=""):
    for key in order:
        next(gens[key], None)
    for g in gens.values():
        for _ in g:
            pass


def _kernel(q_hbm, k_hbm, v_hbm, shk_hbm, ssmk_hbm, ssmd_hbm, w1_hbm, w3_hbm, w2_hbm, c_hbm,
            wmod_hbm, fwd_hbm, inv_hbm, out_hbm,
            q_v, k_v, v_v, ssmk_v, w1_v, w3_v, w2_v, wmod_v, out_v, w1_s, w3_s, w2_s,
            shk_v, ssmd_v, c_v, fwd_v, inv_v, mod_v,
            xu_s, xk_s, spec_s, ab_s, y_s, gate_s, h2_s, x2n_s, x2_s, act_s,
            sem_in, sem_start, sem_out):
    S, D = q_v.shape
    F = w1_v.shape[1]
    n_chunks = S // C
    HP = H + PADQ
    K0, PREV = n_chunks, 2 * n_chunks

    def aligned(start, size, align):
        return pl.ds(start if isinstance(start, int) else pl.multiple_of(start, align), size)

    def rows(i):
        return aligned(i * C, C, C)

    def chunk_refs(i):
        return [(k_hbm.at[rows(i)], k_v.at[aligned(i * C + HALO, C, HALO)]),
                (v_hbm.at[rows(i)], v_v.at[rows(i)]),
                (ssmk_hbm.at[:, rows(i)], ssmk_v.at[i]),
                (q_hbm.at[rows(i)], q_v.at[rows(i)])]

    def chunk_copies(i):
        return [pltpu.make_async_copy(s, d, sem_in.at[i - 3]) for s, d in chunk_refs(i)]

    def out_copy(i, cols=slice(None)):
        return pltpu.make_async_copy(out_v.at[rows(i), cols], out_hbm.at[rows(i), cols], sem_out)

    last_copies = [out_copy(n_chunks - 1, pl.ds(l, 128)) for l in range(0, D, 128)]

    wmod_refs = [(wmod_hbm.at[:, pl.ds(n * D, D)], wmod_v.at[n]) for n in range(6)]
    w13_refs = [[(w1_hbm.at[:, pl.ds(j, FT)], w1_v.at[:, pl.ds(j, FT)]),
                 (w3_hbm.at[:, pl.ds(j, FT)], w3_v.at[:, pl.ds(j, FT)])] for j in range(0, F, FT)]
    start_groups = [
        [(shk_hbm, shk_v), (fwd_hbm, fwd_v), (inv_hbm, inv_v), (ssmd_hbm, ssmd_v), (c_hbm, c_v)]
        + chunk_refs(0)[:3],
        chunk_refs(1)[:3],
        chunk_refs(2)[:3],
        wmod_refs[:3] + [chunk_refs(0)[3], chunk_refs(1)[3]],
        wmod_refs[3:4],
        wmod_refs[4:5],
        w13_refs[0],
        w13_refs[1] + w13_refs[2],
        w13_refs[3] + w13_refs[4],
        w13_refs[5] + [chunk_refs(2)[3], wmod_refs[5], (w2_hbm, w2_v)],
    ]
    start_groups = [[pltpu.make_async_copy(s, d, sem_start.at[n]) for s, d in group]
                    for n, group in enumerate(start_groups)]

    def wait_group(n):
        for cp in start_groups[n]:
            cp.wait()

    def spectrum(x_ref, slot, off, tap0=None):
        e = jnp.dot(fwd_v[0], _halves(x_ref[0]), preferred_element_type=F32)
        t = jnp.dot(fwd_v[1], _halves(x_ref[1]), preferred_element_type=F32)
        if tap0 is not None:
            e = jnp.concatenate([e[:H] + tap0, e[H:]], axis=0)
        for n, x in enumerate((e + t, e - t)):
            spec_s[slot, off + 2 * n * HP:off + 2 * n * HP + H, :] = x[:H]
            spec_s[slot, off + (2 * n + 1) * HP:off + (2 * n + 1) * HP + H, :] = x[H:]

    def ssm_d():
        return jnp.concatenate([ssmd_v[n:n + 1, :] for n in range(D // 128)], axis=1).astype(F32)

    def forward_chunk(i, first=False):
        w = [shk_v[j:j + 1, :].astype(F32) for j in range(4)]
        g = PREP_G
        for r in range(0, H, g):
            base = i * C + 2 * r
            kw = _words(k_v[aligned(base, 2 * g + HALO, HALO), :])
            k0, k1, k2 = kw[8:], pltpu.roll(kw, 1, 0)[8:], pltpu.roll(kw, 2, 0)[8:]
            vw = _words(v_v[aligned(base, 2 * g, 2 * g), :])
            ke, ko, ke1, ko1, ko2 = _even(k0), _odd(k0), _even(k1), _odd(k1), _odd(k2)
            kve = (w[0] * ke + w[1] * ko1 + w[2] * ke1 + w[3] * ko2) * _even(vw)
            kvo = (w[0] * ko + w[1] * ke + w[2] * ko1 + w[3] * ke1) * _odd(vw)
            for n, x in enumerate((kve, kvo)):
                for t in range(0, g, 16):
                    xu_s[n, (r + t) // 2:(r + t) // 2 + 8, :] = _pack(x[t:t + 8], x[t + 8:t + 16])
        yield
        spectrum(xu_s, i, 0)
        yield
        tw = _words(ssmk_v[i].T)
        for t in range(0, H, 16):
            lo, hi = tw[t:t + 8], tw[t + 8:t + 16]
            xk_s[0, t // 2:t // 2 + 8, :] = (lo & U32(0xFFFF)) | (hi << 16)
            xk_s[1, t // 2:t // 2 + 8, :] = (lo >> 16) | (hi & U32(0xFFFF0000))
        yield
        spectrum(xk_s, K0 + i, KOFF, ssm_d() if first else None)
        yield

    def conv_chunk(i, n_terms, dst=0):
        first = n_terms == 1
        if isinstance(i, int):
            terms = [(i - m, K0 + m) for m in range(n_terms)]
        else:
            if STATIC_K:
                terms = [(jnp.maximum(i - m, 0), K0 + m) for m in range(n_terms)]
            else:
                terms = [(m, K0 + jnp.maximum(i - m, 0)) for m in range(n_terms)]
        def products(half, r, l, g):
            re = im = None
            for us, ks in terms:
                ur = spec_s[us, half + r:half + r + g, l:l + MAC_L]
                ui = spec_s[us, half + HP + r:half + HP + r + g, l:l + MAC_L]
                kr = spec_s[ks, KOFF + half + r:KOFF + half + r + g, l:l + MAC_L]
                ki = spec_s[ks, KOFF + half + HP + r:KOFF + half + HP + r + g, l:l + MAC_L]
                if re is None:
                    re, im = ur * kr - ui * ki, ur * ki + ui * kr
                elif MAC_SEQ:
                    re = re + ur * kr
                    im = im + ur * ki
                    re = re - ui * ki
                    im = im + ui * kr
                else:
                    re, im = re + (ur * kr - ui * ki), im + (ur * ki + ui * kr)
            return re, im

        g = MAC_G
        gg = max(16, g)
        for r16 in range(0, H, gg):
            for l in range(0, D, MAC_L):
                for r in range(r16, r16 + gg, g):
                    (pr, pi), (qr, qi) = products(0, r, l, g), products(2 * HP, r, l, g)
                    for n, (re, im) in enumerate(((pr + qr, pi + qi), (pr - qr, pi - qi))):
                        if first:
                            ore, oim = re, im
                        else:
                            lre = spec_s[PREV, 2 * n * HP + r:2 * n * HP + r + g, l:l + MAC_L]
                            lim = spec_s[PREV, (2 * n + 1) * HP + r:(2 * n + 1) * HP + r + g, l:l + MAC_L]
                            ore, oim = (re - lim, im + lre) if r < H // 2 else (re + lim, im - lre)
                        spec_s[PREV, 2 * n * HP + r:2 * n * HP + r + g, l:l + MAC_L] = re
                        spec_s[PREV, (2 * n + 1) * HP + r:(2 * n + 1) * HP + r + g, l:l + MAC_L] = im
                        ab_s[n, r:r + g, l:l + MAC_L] = _pack(ore, oim)
                yield
        for n in range(2):
            y_s[dst + n * H:dst + (n + 1) * H, :] = jnp.dot(inv_v[n], _halves(ab_s[n]),
                                                 preferred_element_type=F32)
        yield

    def q_rows(i, r, g):
        qw = _words(q_v[aligned(i * C + 2 * r, 2 * g, 2 * g), :])
        return (r, _even(qw)), (H + r, _odd(qw))

    def gate_chunk(i, dst=0):
        sa, ca1, ga = (mod_v[n, 0:1, :] for n in range(3))
        scale, shift = ga * ca1, ga * sa
        g = GATE_G
        for r in range(0, H, g):
            for off, x in q_rows(i, r, g):
                val = _layernorm(x) * scale + shift
                gate_s[dst + off:dst + off + g, :] = val
        yield

    def mix_chunk(i, src=0, dst=0):
        sb, cb1 = mod_v[3, 0:1, :], mod_v[4, 0:1, :]
        g = MIX_G
        for r in range(0, H, g):
            for off, x in q_rows(i, r, g):
                x2 = x + gate_s[src + off:src + off + g, :] * y_s[src + off:src + off + g, :]
                x2n_s[dst + off:dst + off + g, :] = x2
                h2 = _layernorm(x2) * cb1 + sb
                h2_s[(dst + off) // 2:(dst + off + g) // 2, :] = _words(h2.astype(BF16))
            yield

    def prepare(i, n_terms):
        yield from gate_chunk(i)
        yield from forward_chunk(i)
        yield from conv_chunk(i, n_terms)
        yield from mix_chunk(i)

    def modulation(n):
        cf = c_v[...].astype(F32)
        sc = jnp.broadcast_to(_silu(cf), (16, D)).astype(BF16)
        m = jnp.dot(sc, wmod_v[n], preferred_element_type=F32)[0:8]
        m = 1.0 + m if n in (1, 4) else m
        mod_v[n] = m * {3: 0.5, 4: 0.5, 5: 2.0}.get(n, 1.0)

    def ffn_chunk(i, n=1, first=False, last=False):
        def weight(landed, packed, cols):
            if not first:
                return _halves(packed[:, cols])
            w = landed[:, cols]
            packed[:, cols] = _words(w)
            return w

        x2_s[0:n * C, :] = x2n_s[0:n * C, :]
        for j in range(0, F, FT):
            cols = slice(j, j + FT)
            gate = jnp.dot(_halves(h2_s[0:n * H, :]), weight(w1_v, w1_s, cols),
                           preferred_element_type=F32)
            yield
            up = jnp.dot(_halves(h2_s[0:n * H, :]), weight(w3_v, w3_s, cols),
                         preferred_element_type=F32)
            act_s[0:n * H, cols] = _words(((gate * jnp.tanh(gate) + gate) * up).astype(BF16))
            yield
        for l in range(0, D, 128):
            cols = slice(l, l + 128)
            o = jnp.dot(_halves(act_s[0:n * H, :]), weight(w2_v, w2_s, cols),
                        preferred_element_type=F32)
            o = x2_s[0:n * C, cols] + mod_v[5, 0:1, cols] * o
            for t in range(n):
                out_v[rows(i + t), cols] = _halves(_pack(o[t * C:t * C + H], o[t * C + H:(t + 1) * C]))
            if last and l // 128 in LAST_AT:
                for cp in last_copies[max([-1] + [x for x in LAST_AT if x < l // 128]) + 1:l // 128 + 1]:
                    cp.start()
            yield

    for group in start_groups:
        for cp in group:
            cp.start()
        pl.delay(1)

    def start_chunk(i, carry):
        for cp in chunk_copies(i):
            cp.start()
        return i

    zero = jax.lax.fori_loop(3, n_chunks, start_chunk, 0) - (n_chunks - 1)
    zero = zero if OPAQUE else 0

    k_v[0:HALO, :] = jnp.zeros((HALO, D), BF16)
    for m in range(3, n_chunks):
        for n in range(4):
            if STATIC_K:
                spec_s[K0 + m, KOFF + n * HP:KOFF + n * HP + H, :] = jnp.zeros((H, D), F32)
            else:
                spec_s[m, n * HP:n * HP + H, :] = jnp.zeros((H, D), F32)
    with jax.named_scope("conv0"):
        conv = [conv_chunk(zero + i, i + 1, i * C) for i in range(3)]
        wait_group(0)
        _emit({"A": forward_chunk(0, True)})
        wait_group(1)
        _emit({"A": forward_chunk(1), "P": conv[0]}, ORDER1)
        wait_group(2)
        _emit({"A": forward_chunk(2), "P": conv[1]}, ORDER1)
        _emit({"P": conv[2]})
    with jax.named_scope("mod"):
        wait_group(3)
        for n in range(3):
            modulation(n)
        _emit({"P": gate_chunk(0), "Q": gate_chunk(1, C)})
        for n in range(3, 5):
            wait_group(n + 1)
            modulation(n)
    with jax.named_scope("mix0"):
        _emit({"P": mix_chunk(0), "Q": mix_chunk(1, C, C)})

    n_mac = (H // max(16, MAC_G)) * (D // MAC_L)

    def arrivals():
        for n in range(6, 10):
            wait_group(n)
            if n == 9:
                modulation(5)
            yield

    def third_chunk():
        yield from gate_chunk(2, 2 * C)
        yield from mix_chunk(2, 2 * C)

    with jax.named_scope("step0"):
        _emit({"W": arrivals(), "F": ffn_chunk(0, 2, True), "P": third_chunk()}, ORDER0)
    out_copy(0).start()
    out_copy(1).start()

    def step(n_terms, i, carry):
        with jax.named_scope("waitc"):
            for cp in chunk_copies(i + 1):
                cp.wait()
        with jax.named_scope("body"):
            _emit({"F": ffn_chunk(i), "P": prepare(i + 1, n_terms)}, _order(*POS, n_mac))
        out_copy(i).start()
        return carry

    for lo, hi in LOOPS:
        if hi - lo == 1:
            step(hi + 1, lo, 0)
        else:
            jax.lax.fori_loop(lo, hi, functools.partial(step, hi + 1), 0)
    with jax.named_scope("last"):
        _emit({"F": ffn_chunk(n_chunks - 1, last=True)})
    with jax.named_scope("outwait"):
        for i in range(n_chunks - 1):
            out_copy(i).wait()
        for cp in last_copies:
            cp.wait()


@jax.jit
def pallas_adaLN_cond__ssm_conv_h3__glu_gated_swiglu__prompt_kernel(
    A_q: jax.Array,
    A_k: jax.Array,
    A_v: jax.Array,
    A_shift_k: jax.Array,
    A_ssm_k: jax.Array,
    A_ssm_D: jax.Array,
    B_x: jax.Array,
    B_w1: jax.Array,
    B_w3: jax.Array,
    B_w2: jax.Array,
    c: jax.Array,
    w_mod: jax.Array,
):
    del B_x
    B, S, D = A_q.shape
    F = B_w1.shape[1]
    ks = A_shift_k.shape[1]
    assert B == 1 and ks == 4 and S % C == 0 and D % 128 == 0 and F % FT == 0
    n_chunks = S // C
    fwd, inv = _dft_matrices()

    vmem = pltpu.VMEM
    scratch = [
        vmem((S, D), BF16),
        vmem((HALO + S, D), BF16),
        vmem((S, D), BF16),
        vmem((n_chunks, D, C), BF16),
        vmem((D, F), BF16), vmem((D, F), BF16), vmem((F, D), BF16),
        vmem((6, D, D), BF16),
        vmem((S, D), BF16),
        vmem((D // 2, F), U32), vmem((D // 2, F), U32), vmem((F // 2, D), U32),
        vmem((ks, D), BF16), vmem((D // 128, 128), BF16), vmem((1, D), BF16),
        vmem(fwd.shape, BF16), vmem(inv.shape, BF16),
        vmem((6, 8, D), F32),
        vmem((2, H // 2, D), U32), vmem((2, H // 2, D), U32),
        vmem((2 * n_chunks + 1, 4 * (H + PADQ) + PADS, D), F32),
        vmem((2, C // 2, D), U32),
        vmem((3 * C, D), F32),
        vmem((3 * C, D), F32),
        vmem((C, D), U32),
        vmem((2 * C, D), F32), vmem((2 * C, D), F32),
        vmem((C, F), U32),
        pltpu.SemaphoreType.DMA((n_chunks - 3,)),
        pltpu.SemaphoreType.DMA((9,)),
        pltpu.SemaphoreType.DMA(()),
    ]
    out = pl.pallas_call(
        _kernel,
        out_shape=jax.ShapeDtypeStruct((S, D), A_q.dtype),
        in_specs=[pl.BlockSpec(memory_space=pl.ANY)] * 13,
        out_specs=pl.BlockSpec(memory_space=pl.ANY),
        scratch_shapes=scratch,
        compiler_params=pltpu.CompilerParams(vmem_limit_bytes=100 * 2**20, **FLAGS),
    )(A_q.reshape(S, D), A_k.reshape(S, D), A_v.reshape(S, D), A_shift_k.T, A_ssm_k,
      A_ssm_D.reshape(D // 128, 128), B_w1, B_w3, B_w2, c, w_mod, fwd, inv)
    return out.reshape(B, S, D)
```

```python
import functools

import numpy as np

import jax
import jax.numpy as jnp
import jax.experimental.pallas as pl
import jax.experimental.pallas.tpu as pltpu

C = 256
H = C // 2
HALO = 16
FT = 256
EPS = 1e-5
MAC_G = 8
FTB = 256
DOWN = [(l, l + 128) for l in range(0, 640, 128)]
OPAQUE = True
ORDER0 = "WFF" "WFFFF" "WFFFF" "WPFF" + "FPP" * 4
ORDER1 = "A" + "P" * (640 // MAC_G) + "AAAP"
LAST_AT = (0, 1, 2, 3, 4)
PREP_G = 32
GATE_G = 16
MIX_G = 16
FLAGS = {}
POS = (1, 3, 15)
LOOPS = ((2, 7),)
F32 = jnp.float32
BF16 = jnp.bfloat16
U32 = jnp.uint32


def _dft_matrices():
    f = np.concatenate([np.arange(0, H, 2), np.arange(1, H, 2)]).astype(np.float64)
    theta = 2.0 * np.pi * (f + 0.5) / (2 * C)
    r = np.arange(H, dtype=np.float64)
    fwd, inv = [], []
    for phase in (0, 1):
        ang = theta[:, None] * (2.0 * r + phase)[None, :]
        m = np.concatenate([np.cos(ang), -np.sin(ang)], axis=0)
        fwd.append(m.reshape(C, H // 16, 2, 8).transpose(0, 1, 3, 2).reshape(C, H))
        inv.append(m.reshape(2, H, H).transpose(2, 1, 0).reshape(H, C) / C)
    return np.stack(fwd).astype(BF16), np.stack(inv).astype(BF16)


def lanes(n):
    return slice(n * 128, (n + 1) * 128)


def _words(x):
    return pltpu.bitcast(x, jnp.uint32)


def _halves(w):
    return pltpu.bitcast(w, BF16)


def _pack(lo, hi):
    return pltpu.bitcast(pltpu.pack_elementwise([lo, hi], packed_dtype=BF16), U32)


def _even(w):
    return pltpu.bitcast(w << 16, F32)


def _odd(w):
    return pltpu.bitcast(w & jnp.uint32(0xFFFF0000), F32)


def _layernorm(x):
    m = jnp.mean(x, axis=-1, keepdims=True)
    d = x - m
    v = jnp.mean(d * d, axis=-1, keepdims=True)
    return d * jax.lax.rsqrt(v + EPS)


def _silu(x):
    hx = 0.5 * x
    return hx * jnp.tanh(hx) + hx


def _order(a, b, c, n_mac):
    mac = ""
    for n in range(c - b):
        mac += "P" * ((n + 1) * n_mac // (c - b) - n * n_mac // (c - b)) + "F"
    return "PP" + "F" * a + "PP" + "F" * (b - a) + "P" + mac + "P" + "FPP" * 4


def _emit(gens, order=""):
    for key in order:
        next(gens[key], None)
    for g in gens.values():
        for _ in g:
            pass


def _kernel(q_hbm, k_hbm, v_hbm, shk_hbm, ssmk_hbm, ssmd_hbm, w1_hbm, w3_hbm, w2_hbm, c_hbm,
            wmod_hbm, fwd_hbm, inv_hbm, out_hbm,
            q_v, k_v, v_v, ssmk_v, w1_v, w3_v, w2_v, wmod_v, out_v, w1_s, w3_s, w2_s,
            shk_v, ssmd_v, c_v, fwd_v, inv_v, mod_v,
            xu_s, xk_s, spec_s, ab_s, y_s, gate_s, h2_s, x2n_s, x2_s, act_s,
            sem_in, sem_start, sem_out):
    S, D = q_v.shape
    F = w1_v.shape[1]
    n_chunks = S // C
    PREV = n_chunks

    def aligned(start, size, align):
        return pl.ds(start if isinstance(start, int) else pl.multiple_of(start, align), size)

    def rows(i):
        return aligned(i * C, C, C)

    def chunk_refs(i):
        return [(k_hbm.at[rows(i)], k_v.at[aligned(i * C + HALO, C, HALO)]),
                (v_hbm.at[rows(i)], v_v.at[rows(i)]),
                (ssmk_hbm.at[:, rows(i)], ssmk_v.at[i]),
                (q_hbm.at[rows(i)], q_v.at[rows(i)])]

    def chunk_copies(i):
        return [pltpu.make_async_copy(s, d, sem_in.at[i - 3]) for s, d in chunk_refs(i)]

    def out_copy(i, cols=slice(None)):
        return pltpu.make_async_copy(out_v.at[rows(i), cols], out_hbm.at[rows(i), cols], sem_out)

    last_copies = [out_copy(n_chunks - 1, pl.ds(l, 128)) for l in range(0, D, 128)]

    wmod_refs = [(wmod_hbm.at[:, pl.ds(n * D, D)], wmod_v.at[n]) for n in range(6)]
    w13_refs = [[(w1_hbm.at[:, pl.ds(j, FT)], w1_v.at[:, pl.ds(j, FT)]),
                 (w3_hbm.at[:, pl.ds(j, FT)], w3_v.at[:, pl.ds(j, FT)])] for j in range(0, F, FT)]
    start_groups = [
        [(shk_hbm, shk_v), (fwd_hbm, fwd_v), (inv_hbm, inv_v), (ssmd_hbm, ssmd_v), (c_hbm, c_v)]
        + chunk_refs(0)[:3],
        chunk_refs(1)[:3],
        chunk_refs(2)[:3],
        wmod_refs[:3] + [chunk_refs(0)[3], chunk_refs(1)[3]],
        wmod_refs[3:4],
        wmod_refs[4:5],
        w13_refs[0],
        w13_refs[1] + w13_refs[2],
        w13_refs[3] + w13_refs[4],
        w13_refs[5] + [chunk_refs(2)[3], wmod_refs[5], (w2_hbm, w2_v)],
    ]
    start_groups = [[pltpu.make_async_copy(s, d, sem_start.at[n]) for s, d in group]
                    for n, group in enumerate(start_groups)]

    def wait_group(n):
        for cp in start_groups[n]:
            cp.wait()

    def spectrum(x_ref, slot, off, tap0=None):
        e = jnp.dot(fwd_v[0], _halves(x_ref[0]), preferred_element_type=F32)
        t = jnp.dot(fwd_v[1], _halves(x_ref[1]), preferred_element_type=F32)
        if tap0 is not None:
            e = jnp.concatenate([e[:H] + tap0, e[H:]], axis=0)
        for n, x in enumerate((e + t, e - t)):
            for l in range(D // 128):
                for part in range(2):
                    spec_s[slot, (2 * l + n) * H:(2 * l + n + 1) * H, lanes(off + part)] = (
                        x[part * H:(part + 1) * H, lanes(l)])

    def ssm_d():
        return jnp.concatenate([ssmd_v[n:n + 1, :] for n in range(D // 128)], axis=1).astype(F32)

    def forward_chunk(i, first=False):
        w = [shk_v[j:j + 1, :].astype(F32) for j in range(4)]
        g = PREP_G
        for r in range(0, H, g):
            base = i * C + 2 * r
            kw = _words(k_v[aligned(base, 2 * g + HALO, HALO), :])
            k0, k1, k2 = kw[8:], pltpu.roll(kw, 1, 0)[8:], pltpu.roll(kw, 2, 0)[8:]
            vw = _words(v_v[aligned(base, 2 * g, 2 * g), :])
            ke, ko, ke1, ko1, ko2 = _even(k0), _odd(k0), _even(k1), _odd(k1), _odd(k2)
            kve = (w[0] * ke + w[1] * ko1 + w[2] * ke1 + w[3] * ko2) * _even(vw)
            kvo = (w[0] * ko + w[1] * ke + w[2] * ko1 + w[3] * ke1) * _odd(vw)
            for n, x in enumerate((kve, kvo)):
                for t in range(0, g, 16):
                    xu_s[n, (r + t) // 2:(r + t) // 2 + 8, :] = _pack(x[t:t + 8], x[t + 8:t + 16])
        yield
        spectrum(xu_s, i, 0)
        yield
        tw = _words(ssmk_v[i].T)
        for t in range(0, H, 16):
            lo, hi = tw[t:t + 8], tw[t + 8:t + 16]
            xk_s[0, t // 2:t // 2 + 8, :] = (lo & U32(0xFFFF)) | (hi << 16)
            xk_s[1, t // 2:t // 2 + 8, :] = (lo >> 16) | (hi & U32(0xFFFF0000))
        yield
        spectrum(xk_s, i, 2, ssm_d() if first else None)
        yield

    def conv_chunk(i, n_terms, dst=0):
        first = n_terms == 1
        if isinstance(i, int):
            terms = [(i - m, m) for m in range(n_terms)]
        else:
            terms = [(jnp.maximum(i - m, 0), m) for m in range(n_terms)]
        def products(row, g):
            re = im = None
            for us, ks in terms:
                ur, ui = spec_s[us, row:row + g, lanes(0)], spec_s[us, row:row + g, lanes(1)]
                kr, ki = spec_s[ks, row:row + g, lanes(2)], spec_s[ks, row:row + g, lanes(3)]
                pr, pi = ur * kr - ui * ki, ur * ki + ui * kr
                re, im = (pr, pi) if re is None else (re + pr, im + pi)
            return re, im

        g = MAC_G
        for l in range(D // 128):
            for r in range(0, H, g):
                pr, pi = products(2 * l * H + r, g)
                qr, qi = products((2 * l + 1) * H + r, g)
                for n, (re, im) in enumerate(((pr + qr, pi + qi), (pr - qr, pi - qi))):
                    last_re = spec_s.at[PREV, l * H + r:l * H + r + g, lanes(2 * n)]
                    last_im = spec_s.at[PREV, l * H + r:l * H + r + g, lanes(2 * n + 1)]
                    if first:
                        ore, oim = re, im
                    else:
                        lre, lim = last_re[...], last_im[...]
                        ore, oim = (re - lim, im + lre) if r < H // 2 else (re + lim, im - lre)
                    last_re[...] = re
                    last_im[...] = im
                    ab_s[n, r:r + g, lanes(l)] = _pack(ore, oim)
                yield
        for n in range(2):
            y_s[dst, n * H:(n + 1) * H, :] = jnp.dot(inv_v[n], _halves(ab_s[n]),
                                                 preferred_element_type=F32)
        yield

    def q_rows(i, r, g):
        qw = _words(q_v[aligned(i * C + 2 * r, 2 * g, 2 * g), :])
        return (r, _even(qw)), (H + r, _odd(qw))

    def gate_chunk(i, dst=0):
        sa, ca1, ga = (mod_v[n, 0:1, :] for n in range(3))
        scale, shift = ga * ca1, ga * sa
        g = GATE_G
        for r in range(0, H, g):
            for off, x in q_rows(i, r, g):
                val = _layernorm(x) * scale + shift
                gate_s[dst, off:off + g, :] = val
        yield

    def mix_chunk(i, src=0, dst=0):
        sb, cb1 = mod_v[3, 0:1, :], mod_v[4, 0:1, :]
        g = MIX_G
        for r in range(0, H, g):
            for off, x in q_rows(i, r, g):
                x2 = x + gate_s[src, off:off + g, :] * y_s[src, off:off + g, :]
                x2n_s[dst + off:dst + off + g, :] = x2
                h2 = _layernorm(x2) * cb1 + sb
                h2_s[(dst + off) // 2:(dst + off + g) // 2, :] = _words(h2.astype(BF16))
            yield

    def prepare(i, n_terms):
        yield from gate_chunk(i)
        yield from forward_chunk(i)
        yield from conv_chunk(i, n_terms)
        yield from mix_chunk(i)

    def modulation(n):
        cf = c_v[...].astype(F32)
        sc = jnp.broadcast_to(_silu(cf), (16, D)).astype(BF16)
        m = jnp.dot(sc, wmod_v[n], preferred_element_type=F32)[0:8]
        m = 1.0 + m if n in (1, 4) else m
        mod_v[n] = m * {3: 0.5, 4: 0.5, 5: 2.0}.get(n, 1.0)

    def ffn_chunk(i, n=1, first=False, last=False):
        def weight(landed, packed, cols):
            if not first:
                return _halves(packed[:, cols])
            w = landed[:, cols]
            packed[:, cols] = _words(w)
            return w

        x2_s[0:n * C, :] = x2n_s[0:n * C, :]
        ft = FT if first else FTB
        for j in range(0, F, ft):
            cols = slice(j, j + ft)
            gate = jnp.dot(_halves(h2_s[0:n * H, :]), weight(w1_v, w1_s, cols),
                           preferred_element_type=F32)
            yield
            up = jnp.dot(_halves(h2_s[0:n * H, :]), weight(w3_v, w3_s, cols),
                         preferred_element_type=F32)
            act_s[0:n * H, cols] = _words(((gate * jnp.tanh(gate) + gate) * up).astype(BF16))
            yield
        tiles = [(l, l + 128) for l in range(0, D, 128)] if first or last else DOWN
        for l, l1 in tiles:
            cols = slice(l, l1)
            o = jnp.dot(_halves(act_s[0:n * H, :]), weight(w2_v, w2_s, cols),
                        preferred_element_type=F32)
            o = x2_s[0:n * C, cols] + mod_v[5, 0:1, cols] * o
            for t in range(n):
                out_v[rows(i + t), cols] = _halves(_pack(o[t * C:t * C + H], o[t * C + H:(t + 1) * C]))
            if last and l // 128 in LAST_AT:
                for cp in last_copies[max([-1] + [x for x in LAST_AT if x < l // 128]) + 1:l // 128 + 1]:
                    cp.start()
            yield

    for group in start_groups:
        for cp in group:
            cp.start()
        pl.delay(1)

    def start_chunk(i, carry):
        for cp in chunk_copies(i):
            cp.start()
        return i

    zero = jax.lax.fori_loop(3, n_chunks, start_chunk, 0) - (n_chunks - 1)
    zero = zero if OPAQUE else 0

    k_v[0:HALO, :] = jnp.zeros((HALO, D), BF16)
    for m in range(3, n_chunks):
        spec_s[m, :, 256:512] = jnp.zeros((spec_s.shape[1], 256), F32)
    with jax.named_scope("conv0"):
        conv = [conv_chunk(zero + i, i + 1, i) for i in range(3)]
        wait_group(0)
        _emit({"A": forward_chunk(0, True)})
        wait_group(1)
        _emit({"A": forward_chunk(1), "P": conv[0]}, ORDER1)
        wait_group(2)
        _emit({"A": forward_chunk(2), "P": conv[1]}, ORDER1)
        _emit({"P": conv[2]})
    with jax.named_scope("mod"):
        wait_group(3)
        for n in range(3):
            modulation(n)
        _emit({"P": gate_chunk(0), "Q": gate_chunk(1, 1)})
        for n in range(3, 5):
            wait_group(n + 1)
            modulation(n)
    with jax.named_scope("mix0"):
        _emit({"P": mix_chunk(0), "Q": mix_chunk(1, 1, C)})

    n_mac = H // MAC_G * (D // 128)

    def arrivals():
        for n in range(6, 10):
            wait_group(n)
            if n == 9:
                modulation(5)
            yield

    def third_chunk():
        yield from gate_chunk(2, 2)
        yield from mix_chunk(2, 2)

    with jax.named_scope("step0"):
        _emit({"W": arrivals(), "F": ffn_chunk(0, 2, True), "P": third_chunk()}, ORDER0)
    out_copy(0).start()
    out_copy(1).start()

    def step(n_terms, i, carry):
        with jax.named_scope("waitc"):
            for cp in chunk_copies(i + 1):
                cp.wait()
        with jax.named_scope("body"):
            _emit({"F": ffn_chunk(i), "P": prepare(i + 1, n_terms)}, _order(*POS, n_mac))
        out_copy(i).start()
        return carry

    for lo, hi in LOOPS:
        if hi - lo == 1:
            step(hi + 1, lo, 0)
        else:
            jax.lax.fori_loop(lo, hi, functools.partial(step, hi + 1), 0)
    with jax.named_scope("last"):
        _emit({"F": ffn_chunk(n_chunks - 1, last=True)})
    with jax.named_scope("outwait"):
        for i in range(n_chunks - 1):
            out_copy(i).wait()
        for cp in last_copies:
            cp.wait()


@jax.jit
def pallas_adaLN_cond__ssm_conv_h3__glu_gated_swiglu__prompt_kernel(
    A_q: jax.Array,
    A_k: jax.Array,
    A_v: jax.Array,
    A_shift_k: jax.Array,
    A_ssm_k: jax.Array,
    A_ssm_D: jax.Array,
    B_x: jax.Array,
    B_w1: jax.Array,
    B_w3: jax.Array,
    B_w2: jax.Array,
    c: jax.Array,
    w_mod: jax.Array,
):
    del B_x
    B, S, D = A_q.shape
    F = B_w1.shape[1]
    ks = A_shift_k.shape[1]
    assert B == 1 and ks == 4 and S % C == 0 and D % 128 == 0 and F % FT == 0
    n_chunks = S // C
    fwd, inv = _dft_matrices()

    vmem = pltpu.VMEM
    scratch = [
        vmem((S, D), BF16),
        vmem((HALO + S, D), BF16),
        vmem((S, D), BF16),
        vmem((n_chunks, D, C), BF16),
        vmem((D, F), BF16), vmem((D, F), BF16), vmem((F, D), BF16),
        vmem((6, D, D), BF16),
        vmem((S, D), BF16),
        vmem((D // 2, F), U32), vmem((D // 2, F), U32), vmem((F // 2, D), U32),
        vmem((ks, D), BF16), vmem((D // 128, 128), BF16), vmem((1, D), BF16),
        vmem(fwd.shape, BF16), vmem(inv.shape, BF16),
        vmem((6, 8, D), F32),
        vmem((2, H // 2, D), U32), vmem((2, H // 2, D), U32),
        vmem((n_chunks + 1, D // 128 * C, 4 * 128), F32),
        vmem((2, C // 2, D), U32),
        vmem((3, C, D), F32),
        vmem((3, C, D), F32),
        vmem((C, D), U32),
        vmem((2 * C, D), F32), vmem((2 * C, D), F32),
        vmem((C, F), U32),
        pltpu.SemaphoreType.DMA((n_chunks - 3,)),
        pltpu.SemaphoreType.DMA((9,)),
        pltpu.SemaphoreType.DMA(()),
    ]
    out = pl.pallas_call(
        _kernel,
        out_shape=jax.ShapeDtypeStruct((S, D), A_q.dtype),
        in_specs=[pl.BlockSpec(memory_space=pl.ANY)] * 13,
        out_specs=pl.BlockSpec(memory_space=pl.ANY),
        scratch_shapes=scratch,
        compiler_params=pltpu.CompilerParams(vmem_limit_bytes=100 * 2**20, **FLAGS),
    )(A_q.reshape(S, D), A_k.reshape(S, D), A_v.reshape(S, D), A_shift_k.T, A_ssm_k,
      A_ssm_D.reshape(D // 128, 128), B_w1, B_w3, B_w2, c, w_mod, fwd, inv)
    return out.reshape(B, S, D)
```

```python
import functools

import numpy as np

import jax
import jax.numpy as jnp
import jax.experimental.pallas as pl
import jax.experimental.pallas.tpu as pltpu

C = 256
H = C // 2
HALO = 16
FT = 256
KS = 512
EPS = 1e-5
MAC_G = 8
OPAQUE = True
ORDER0 = "WFF" "WFFFF" "WFFFFFF" "WP" + "FP" * 8
ORDER1 = "A" + "P" * (640 // MAC_G) + "AAAP"
PREP_G = 32
GATE_G = 16
MIX_G = 16
FLAGS = {}
POS = (0, 2, 11)
F32 = jnp.float32
BF16 = jnp.bfloat16
U32 = jnp.uint32


def _dft_matrices():
    f = np.concatenate([np.arange(0, H, 2), np.arange(1, H, 2)]).astype(np.float64)
    theta = 2.0 * np.pi * (f + 0.5) / (2 * C)
    r = np.arange(H, dtype=np.float64)
    fwd, inv = [], []
    for phase in (0, 1):
        ang = theta[:, None] * (2.0 * r + phase)[None, :]
        m = np.concatenate([np.cos(ang), -np.sin(ang)], axis=0)
        fwd.append(m.reshape(C, H // 16, 2, 8).transpose(0, 1, 3, 2).reshape(C, H))
        inv.append(m.reshape(2, H, H).transpose(2, 1, 0).reshape(H, C) / C)
    return np.stack(fwd).astype(BF16), np.stack(inv).astype(BF16)


def lanes(n):
    return slice(n * 128, (n + 1) * 128)


def _words(x):
    return pltpu.bitcast(x, jnp.uint32)


def _halves(w):
    return pltpu.bitcast(w, BF16)


def _pack(lo, hi):
    return pltpu.bitcast(pltpu.pack_elementwise([lo, hi], packed_dtype=BF16), U32)


def _even(w):
    return pltpu.bitcast(w << 16, F32)


def _odd(w):
    return pltpu.bitcast(w & jnp.uint32(0xFFFF0000), F32)


def _left_operands(a11, a12, a21, a22):
    return [a11 + a22, a21 + a22, a11, a22, a11 + a12, a21 - a11, a12 - a22]


def _right_operands(b11, b12, b21, b22):
    return [b11 + b22, b11, b12 - b22, b21 - b11, b22, b11 + b12, b21 + b22]


def _product_blocks(m):
    return m[0] + m[3] - m[4] + m[6], m[2] + m[4], m[1] + m[3], m[0] - m[1] + m[2] + m[5]


def _dot(a, b):
    return jnp.dot(_halves(a), _halves(b), preferred_element_type=F32)


def _layernorm(x):
    m = jnp.mean(x, axis=-1, keepdims=True)
    d = x - m
    v = jnp.mean(d * d, axis=-1, keepdims=True)
    return d * jax.lax.rsqrt(v + EPS)


def _silu(x):
    hx = 0.5 * x
    return hx * jnp.tanh(hx) + hx


def _order(a, b, c, n_mac):
    mac = ""
    for n in range(c - b):
        mac += "P" * ((n + 1) * n_mac // (c - b) - n * n_mac // (c - b)) + "F"
    return "PP" + "F" * a + "PP" + "F" * (b - a) + "P" + mac + "P" + "FPP" * 4


def _emit(gens, order=""):
    for key in order:
        next(gens[key], None)
    for g in gens.values():
        for _ in g:
            pass


def _kernel(q_hbm, k_hbm, v_hbm, shk_hbm, ssmk_hbm, ssmd_hbm, w1_hbm, w3_hbm, w2_hbm, c_hbm,
            wmod_hbm, fwd_hbm, inv_hbm, out_hbm,
            q_v, k_v, v_v, ssmk_v, w1_v, w3_v, w2_v, wmod_v, out_v, b13_s, r13_s, b2_s, r2_s,
            shk_v, ssmd_v, c_v, fwd_v, inv_v, mod_v,
            xu_s, xk_s, spec_s, ab_s, y_s, gate_s, x2n_s, x2_s, a13_s, hr_s, a2_s,
            sem_in, sem_start, sem_out):
    S, D = q_v.shape
    F = w1_v.shape[1]
    n_chunks = S // C
    PREV = n_chunks

    def aligned(start, size, align):
        return pl.ds(start if isinstance(start, int) else pl.multiple_of(start, align), size)

    def rows(i):
        return aligned(i * C, C, C)

    def chunk_refs(i):
        return [(k_hbm.at[rows(i)], k_v.at[aligned(i * C + HALO, C, HALO)]),
                (v_hbm.at[rows(i)], v_v.at[rows(i)]),
                (ssmk_hbm.at[:, rows(i)], ssmk_v.at[i]),
                (q_hbm.at[rows(i)], q_v.at[rows(i)])]

    def chunk_copies(i):
        return [pltpu.make_async_copy(s, d, sem_in.at[i - 3]) for s, d in chunk_refs(i)]

    def out_copy(i, cols=slice(None)):
        return pltpu.make_async_copy(out_v.at[rows(i), cols], out_hbm.at[rows(i), cols], sem_out)

    last_copies = [out_copy(n_chunks - 1, pl.ds(l, n))
                   for l, n in ((0, KS // 2), (KS // 2, KS // 2), (KS, D - KS))]

    wmod_refs = [(wmod_hbm.at[:, pl.ds(n * D, D)], wmod_v.at[n]) for n in range(6)]
    w13_refs = [[(w_hbm.at[:, pl.ds(c0 + j, 128)], w_v.at[:, pl.ds(c0 + j, 128)])
                 for w_hbm, w_v in ((w1_hbm, w1_v), (w3_hbm, w3_v)) for c0 in (0, F // 2)]
                for j in range(0, F // 2, 128)]
    start_groups = [
        [(shk_hbm, shk_v), (fwd_hbm, fwd_v), (inv_hbm, inv_v), (ssmd_hbm, ssmd_v), (c_hbm, c_v)]
        + chunk_refs(0)[:3],
        chunk_refs(1)[:3],
        chunk_refs(2)[:3],
        wmod_refs[:3] + [chunk_refs(0)[3], chunk_refs(1)[3]],
        wmod_refs[3:4],
        wmod_refs[4:5],
        w13_refs[0],
        w13_refs[1] + w13_refs[2],
        w13_refs[3] + w13_refs[4] + w13_refs[5],
        [chunk_refs(2)[3], wmod_refs[5], (w2_hbm, w2_v)],
    ]
    start_groups = [[pltpu.make_async_copy(s, d, sem_start.at[n]) for s, d in group]
                    for n, group in enumerate(start_groups)]

    def wait_group(n):
        for cp in start_groups[n]:
            cp.wait()

    def spectrum(x_ref, slot, off, tap0=None):
        e = jnp.dot(fwd_v[0], _halves(x_ref[0]), preferred_element_type=F32)
        t = jnp.dot(fwd_v[1], _halves(x_ref[1]), preferred_element_type=F32)
        if tap0 is not None:
            e = jnp.concatenate([e[:H] + tap0, e[H:]], axis=0)
        for n, x in enumerate((e + t, e - t)):
            for l in range(D // 128):
                for part in range(2):
                    spec_s[slot, (2 * l + n) * H:(2 * l + n + 1) * H, lanes(off + part)] = (
                        x[part * H:(part + 1) * H, lanes(l)])

    def ssm_d():
        return jnp.concatenate([ssmd_v[n:n + 1, :] for n in range(D // 128)], axis=1).astype(F32)

    def forward_chunk(i, first=False):
        w = [shk_v[j:j + 1, :].astype(F32) for j in range(4)]
        g = PREP_G
        for r in range(0, H, g):
            base = i * C + 2 * r
            kw = _words(k_v[aligned(base, 2 * g + HALO, HALO), :])
            k0, k1, k2 = kw[8:], pltpu.roll(kw, 1, 0)[8:], pltpu.roll(kw, 2, 0)[8:]
            vw = _words(v_v[aligned(base, 2 * g, 2 * g), :])
            ke, ko, ke1, ko1, ko2 = _even(k0), _odd(k0), _even(k1), _odd(k1), _odd(k2)
            kve = (w[0] * ke + w[1] * ko1 + w[2] * ke1 + w[3] * ko2) * _even(vw)
            kvo = (w[0] * ko + w[1] * ke + w[2] * ko1 + w[3] * ke1) * _odd(vw)
            for n, x in enumerate((kve, kvo)):
                for t in range(0, g, 16):
                    xu_s[n, (r + t) // 2:(r + t) // 2 + 8, :] = _pack(x[t:t + 8], x[t + 8:t + 16])
        yield
        spectrum(xu_s, i, 0)
        yield
        tw = _words(ssmk_v[i].T)
        for t in range(0, H, 16):
            lo, hi = tw[t:t + 8], tw[t + 8:t + 16]
            xk_s[0, t // 2:t // 2 + 8, :] = (lo & U32(0xFFFF)) | (hi << 16)
            xk_s[1, t // 2:t // 2 + 8, :] = (lo >> 16) | (hi & U32(0xFFFF0000))
        yield
        spectrum(xk_s, i, 2, ssm_d() if first else None)
        yield

    def conv_chunk(i, n_terms, dst=0):
        first = n_terms == 1
        if isinstance(i, int):
            terms = [(i - m, m) for m in range(n_terms)]
        else:
            terms = [(jnp.maximum(i - m, 0), m) for m in range(n_terms)]
        def products(row, g):
            re = im = None
            for us, ks in terms:
                ur, ui = spec_s[us, row:row + g, lanes(0)], spec_s[us, row:row + g, lanes(1)]
                kr, ki = spec_s[ks, row:row + g, lanes(2)], spec_s[ks, row:row + g, lanes(3)]
                pr, pi = ur * kr - ui * ki, ur * ki + ui * kr
                re, im = (pr, pi) if re is None else (re + pr, im + pi)
            return re, im

        g = MAC_G
        for l in range(D // 128):
            for r in range(0, H, g):
                pr, pi = products(2 * l * H + r, g)
                qr, qi = products((2 * l + 1) * H + r, g)
                for n, (re, im) in enumerate(((pr + qr, pi + qi), (pr - qr, pi - qi))):
                    last_re = spec_s.at[PREV, l * H + r:l * H + r + g, lanes(2 * n)]
                    last_im = spec_s.at[PREV, l * H + r:l * H + r + g, lanes(2 * n + 1)]
                    if first:
                        ore, oim = re, im
                    else:
                        lre, lim = last_re[...], last_im[...]
                        ore, oim = (re - lim, im + lre) if r < H // 2 else (re + lim, im - lre)
                    last_re[...] = re
                    last_im[...] = im
                    ab_s[n, r:r + g, lanes(l)] = _pack(ore, oim)
                yield
        for n in range(2):
            y_s[dst, n * H:(n + 1) * H, :] = jnp.dot(inv_v[n], _halves(ab_s[n]),
                                                 preferred_element_type=F32)
        yield

    def q_rows(i, r, g):
        qw = _words(q_v[aligned(i * C + 2 * r, 2 * g, 2 * g), :])
        return (r, _even(qw)), (H + r, _odd(qw))

    def gate_chunk(i, dst=0):
        sa, ca1, ga = (mod_v[n, 0:1, :] for n in range(3))
        scale, shift = ga * ca1, ga * sa
        g = GATE_G
        for r in range(0, H, g):
            for off, x in q_rows(i, r, g):
                val = _layernorm(x) * scale + shift
                gate_s[dst, off:off + g, :] = val
        yield

    def mix_chunk(i, src=0, dst=0, x2_ref=x2n_s):
        sb, cb1 = mod_v[3, 0:1, :], mod_v[4, 0:1, :]
        g = MIX_G
        for r in range(0, H, g):
            h2 = []
            for off, x in q_rows(i, r, g):
                x2 = x + gate_s[src, off:off + g, :] * y_s[src, off:off + g, :]
                x2_ref[dst * C + off:dst * C + off + g, :] = x2
                h2.append(_layernorm(x2) * cb1 + sb)
            words = slice((dst * H + r) // 2, (dst * H + r + g) // 2)
            blocks = [x[:, l:l + KS // 2] for x in h2 for l in (0, KS // 2)]
            for n, x in enumerate(_left_operands(*blocks)):
                a13_s[n, words, :] = _words(x.astype(BF16))
            for n, x in enumerate(h2):
                hr_s[n, words, :] = _words(x[:, KS:].astype(BF16))
            yield

    def prepare(i, n_terms):
        yield from gate_chunk(i)
        yield from forward_chunk(i)
        yield from conv_chunk(i, n_terms)
        yield from mix_chunk(i)

    def modulation(n):
        cf = c_v[...].astype(F32)
        sc = jnp.broadcast_to(_silu(cf), (16, D)).astype(BF16)
        m = jnp.dot(sc, wmod_v[n], preferred_element_type=F32)[0:8]
        m = 1.0 + m if n in (1, 4) else m
        mod_v[n] = m * {3: 0.5, 4: 0.5, 5: 2.0}.get(n, 1.0)

    def swiglu(gate, up):
        return (gate * jnp.tanh(gate) + gate) * up

    def store_out(i, cols, src, even, odd):
        gb = mod_v[5, 0:1, cols]
        even = x2_s[src:src + H, cols] + gb * even
        odd = x2_s[src + H:src + C, cols] + gb * odd
        out_v[rows(i), cols] = _halves(_pack(even, odd))

    def right_factors(dst, src, row, col, cols):
        for r in range(0, row, 16):
            w = [_words(src[r0 + r:r0 + r + 16, c0 + cols.start:c0 + cols.stop])
                 for r0 in (0, row) for c0 in (0, col)]
            even = _right_operands(*map(_even, w))
            odd = _right_operands(*map(_odd, w))
            for n in range(7):
                dst[n, r // 2:r // 2 + 8, cols] = (
                    w[0] if n == 1 else w[3] if n == 4 else _pack(even[n], odd[n]))

    def ffn_chunk(i, n=1, first=False, last=False):
        m_rows, words = n * H, slice(0, n * H // 2)
        if not first:
            x2_s[0:C, :] = x2n_s[...]
        rest = jnp.concatenate([hr_s[0, words, :], hr_s[1, words, :]], axis=0)
        ft = 128 if first else FT
        for j in range(0, F // 2, ft):
            cols, cols2 = slice(j, j + ft), slice(F // 2 + j, F // 2 + j + ft)
            pre = []
            for t, w_v in enumerate((w1_v, w3_v)):
                if first:
                    right_factors(b13_s.at[t], w_v, KS // 2, F // 2, cols)
                    r13_s[t, :, cols] = _words(w_v[KS:, cols])
                    r13_s[t, :, cols2] = _words(w_v[KS:, cols2])
                c11, c12, c21, c22 = _product_blocks(
                    [_dot(a13_s[m, words, :], b13_s[t, m, :, cols]) for m in range(7)])
                r1, r2 = _dot(rest, r13_s[t, :, cols]), _dot(rest, r13_s[t, :, cols2])
                pre.append((c11 + r1[:m_rows], c12 + r2[:m_rows],
                            c21 + r1[m_rows:], c22 + r2[m_rows:]))
                yield
            act = [swiglu(gate, up) for gate, up in zip(*pre)]
            for m, x in enumerate(_left_operands(*act) + act[1:3]):
                a2_s[m, words, cols] = _words(x.astype(BF16))

        def store(cols, even, odd):
            for t in range(n):
                store_out(i + t, cols, t * C, even[t * H:(t + 1) * H], odd[t * H:(t + 1) * H])

        if first:
            r2_s[...] = _words(w2_v[:, KS:])
        act = jnp.concatenate(
            [jnp.concatenate([a2_s[m, words, :] for m in pair], axis=1) for pair in ((2, 7), (8, 3))],
            axis=0)
        o = _dot(act, r2_s[...])
        store(slice(KS, D), o[:m_rows], o[m_rows:])
        if last:
            last_copies[2].start()
        yield
        if first:
            right_factors(b2_s, w2_v, F // 2, KS // 2, slice(0, KS // 2))
        products = []
        for m in range(7):
            products.append(_dot(a2_s[m, words, :], b2_s[m]))
            yield
        c11, c12, c21, c22 = _product_blocks(products)
        store(slice(0, KS // 2), c11, c21)
        store(slice(KS // 2, KS), c12, c22)
        if last:
            last_copies[0].start()
            last_copies[1].start()

    for group in start_groups:
        for cp in group:
            cp.start()
        pl.delay(1)

    def start_chunk(i, carry):
        for cp in chunk_copies(i):
            cp.start()
        return i

    zero = jax.lax.fori_loop(3, n_chunks, start_chunk, 0) - (n_chunks - 1)
    zero = zero if OPAQUE else 0

    k_v[0:HALO, :] = jnp.zeros((HALO, D), BF16)
    for m in range(3, n_chunks):
        spec_s[m, :, 256:512] = jnp.zeros((spec_s.shape[1], 256), F32)
    with jax.named_scope("conv0"):
        conv = [conv_chunk(zero + i, i + 1, i) for i in range(3)]
        wait_group(0)
        _emit({"A": forward_chunk(0, True)})
        wait_group(1)
        _emit({"A": forward_chunk(1), "P": conv[0]}, ORDER1)
        wait_group(2)
        _emit({"A": forward_chunk(2), "P": conv[1]}, ORDER1)
        _emit({"P": conv[2]})
    with jax.named_scope("mod"):
        wait_group(3)
        for n in range(3):
            modulation(n)
        _emit({"P": gate_chunk(0), "Q": gate_chunk(1, 1)})
        for n in range(3, 5):
            wait_group(n + 1)
            modulation(n)
    with jax.named_scope("mix0"):
        _emit({"P": mix_chunk(0, 0, 0, x2_s), "Q": mix_chunk(1, 1, 1, x2_s)})

    n_mac = H // MAC_G * (D // 128)

    def arrivals():
        for n in range(6, 10):
            wait_group(n)
            if n == 9:
                modulation(5)
            yield

    def third_chunk():
        yield from gate_chunk(2, 2)
        yield from mix_chunk(2, 2)

    with jax.named_scope("step0"):
        _emit({"W": arrivals(), "F": ffn_chunk(0, 2, first=True), "P": third_chunk()}, ORDER0)
    out_copy(0).start()
    out_copy(1).start()

    def step(n_terms, i, carry):
        with jax.named_scope("waitc"):
            for cp in chunk_copies(i + 1):
                cp.wait()
        with jax.named_scope("body"):
            _emit({"F": ffn_chunk(i), "P": prepare(i + 1, n_terms)}, _order(*POS, n_mac))
        out_copy(i).start()
        return carry

    jax.lax.fori_loop(2, n_chunks - 1, functools.partial(step, n_chunks), 0)
    with jax.named_scope("last"):
        _emit({"F": ffn_chunk(n_chunks - 1, last=True)})
    with jax.named_scope("outwait"):
        for i in range(n_chunks - 1):
            out_copy(i).wait()
        for cp in last_copies:
            cp.wait()


@jax.jit
def pallas_adaLN_cond__ssm_conv_h3__glu_gated_swiglu__prompt_kernel(
    A_q: jax.Array,
    A_k: jax.Array,
    A_v: jax.Array,
    A_shift_k: jax.Array,
    A_ssm_k: jax.Array,
    A_ssm_D: jax.Array,
    B_x: jax.Array,
    B_w1: jax.Array,
    B_w3: jax.Array,
    B_w2: jax.Array,
    c: jax.Array,
    w_mod: jax.Array,
):
    del B_x
    B, S, D = A_q.shape
    F = B_w1.shape[1]
    ks = A_shift_k.shape[1]
    assert B == 1 and ks == 4 and S % C == 0 and D % 128 == 0 and F % FT == 0
    n_chunks = S // C
    fwd, inv = _dft_matrices()

    vmem = pltpu.VMEM
    scratch = [
        vmem((S, D), BF16),
        vmem((HALO + S, D), BF16),
        vmem((S, D), BF16),
        vmem((n_chunks, D, C), BF16),
        vmem((D, F), BF16), vmem((D, F), BF16), vmem((F, D), BF16),
        vmem((6, D, D), BF16),
        vmem((S, D), BF16),
        vmem((2, 7, KS // 4, F // 2), U32),
        vmem((2, (D - KS) // 2, F), U32),
        vmem((7, F // 4, KS // 2), U32),
        vmem((F // 2, D - KS), U32),
        vmem((ks, D), BF16), vmem((D // 128, 128), BF16), vmem((1, D), BF16),
        vmem(fwd.shape, BF16), vmem(inv.shape, BF16),
        vmem((6, 8, D), F32),
        vmem((2, H // 2, D), U32), vmem((2, H // 2, D), U32),
        vmem((n_chunks + 1, D // 128 * C, 4 * 128), F32),
        vmem((2, C // 2, D), U32),
        vmem((3, C, D), F32),
        vmem((3, C, D), F32),
        vmem((C, D), F32), vmem((2 * C, D), F32),
        vmem((7, H, KS // 2), U32),
        vmem((2, H, D - KS), U32),
        vmem((9, H, F // 2), U32),
        pltpu.SemaphoreType.DMA((n_chunks - 3,)),
        pltpu.SemaphoreType.DMA((9,)),
        pltpu.SemaphoreType.DMA(()),
    ]
    out = pl.pallas_call(
        _kernel,
        out_shape=jax.ShapeDtypeStruct((S, D), A_q.dtype),
        in_specs=[pl.BlockSpec(memory_space=pl.ANY)] * 13,
        out_specs=pl.BlockSpec(memory_space=pl.ANY),
        scratch_shapes=scratch,
        compiler_params=pltpu.CompilerParams(vmem_limit_bytes=100 * 2**20, **FLAGS),
    )(A_q.reshape(S, D), A_k.reshape(S, D), A_v.reshape(S, D), A_shift_k.T, A_ssm_k,
      A_ssm_D.reshape(D // 128, 128), B_w1, B_w3, B_w2, c, w_mod, fwd, inv)
    return out.reshape(B, S, D)
```

```python
import functools

import numpy as np

import jax
import jax.numpy as jnp
import jax.experimental.pallas as pl
import jax.experimental.pallas.tpu as pltpu

C = 256
H = C // 2
HALO = 16
FT = 256
KS = 512
EPS = 1e-5
MAC_G = 8
OPAQUE = True
CUTS = (3, 7, 11)
ORDER1 = "A" + "P" * (640 // MAC_G) + "AAAP"
PREP_G = 32
GATE_G = 16
MIX_G = 16
FLAGS = {}
POS = (0, 2, 11)
F32 = jnp.float32
BF16 = jnp.bfloat16
U32 = jnp.uint32


def _dft_matrices():
    f = np.concatenate([np.arange(0, H, 2), np.arange(1, H, 2)]).astype(np.float64)
    theta = 2.0 * np.pi * (f + 0.5) / (2 * C)
    r = np.arange(H, dtype=np.float64)
    fwd, inv = [], []
    for phase in (0, 1):
        ang = theta[:, None] * (2.0 * r + phase)[None, :]
        m = np.concatenate([np.cos(ang), -np.sin(ang)], axis=0)
        fwd.append(m.reshape(C, H // 16, 2, 8).transpose(0, 1, 3, 2).reshape(C, H))
        inv.append(m.reshape(2, H, H).transpose(2, 1, 0).reshape(H, C) / C)
    return np.stack(fwd).astype(BF16), np.stack(inv).astype(BF16)


def lanes(n):
    return slice(n * 128, (n + 1) * 128)


def _words(x):
    return pltpu.bitcast(x, jnp.uint32)


def _halves(w):
    return pltpu.bitcast(w, BF16)


def _pack(lo, hi):
    return pltpu.bitcast(pltpu.pack_elementwise([lo, hi], packed_dtype=BF16), U32)


def _even(w):
    return pltpu.bitcast(w << 16, F32)


def _odd(w):
    return pltpu.bitcast(w & jnp.uint32(0xFFFF0000), F32)


def _left_operands(a11, a12, a21, a22):
    return [a11 + a22, a21 + a22, a11, a22, a11 + a12, a21 - a11, a12 - a22]


def _right_operands(b11, b12, b21, b22):
    return [b11 + b22, b11, b12 - b22, b21 - b11, b22, b11 + b12, b21 + b22]


def _product_blocks(m):
    return m[0] + m[3] - m[4] + m[6], m[2] + m[4], m[1] + m[3], m[0] - m[1] + m[2] + m[5]


def _dot(a, b):
    return jnp.dot(_halves(a), _halves(b), preferred_element_type=F32)


def _layernorm(x):
    m = jnp.mean(x, axis=-1, keepdims=True)
    d = x - m
    v = jnp.mean(d * d, axis=-1, keepdims=True)
    return d * jax.lax.rsqrt(v + EPS)


def _silu(x):
    hx = 0.5 * x
    return hx * jnp.tanh(hx) + hx


def _order(a, b, c, n_mac):
    mac = ""
    for n in range(c - b):
        mac += "P" * ((n + 1) * n_mac // (c - b) - n * n_mac // (c - b)) + "F"
    return "PP" + "F" * a + "PP" + "F" * (b - a) + "P" + mac + "P" + "FPP" * 4


def _emit(gens, order=""):
    for key in order:
        next(gens[key], None)
    for g in gens.values():
        for _ in g:
            pass


def _kernel(q_hbm, k_hbm, v_hbm, shk_hbm, ssmk_hbm, ssmd_hbm, w1_hbm, w3_hbm, w2_hbm, c_hbm,
            wmod_hbm, fwd_hbm, inv_hbm, out_hbm,
            q_v, k_v, v_v, ssmk_v, w1_v, w3_v, w2_v, wmod_v, out_v, b13_s, r13_s, b2_s, r2_s,
            shk_v, ssmd_v, c_v, fwd_v, inv_v, mod_v,
            xu_s, xk_s, spec_s, ab_s, y_s, gate_s, x2n_s, x2_s, a13_s, hr_s, a2_s,
            sem_in, sem_start, sem_out):
    S, D = q_v.shape
    F = w1_v.shape[1]
    n_chunks = S // C
    PREV = n_chunks

    def aligned(start, size, align):
        return pl.ds(start if isinstance(start, int) else pl.multiple_of(start, align), size)

    def rows(i):
        return aligned(i * C, C, C)

    def chunk_refs(i):
        return [(k_hbm.at[rows(i)], k_v.at[aligned(i * C + HALO, C, HALO)]),
                (v_hbm.at[rows(i)], v_v.at[rows(i)]),
                (ssmk_hbm.at[:, rows(i)], ssmk_v.at[i]),
                (q_hbm.at[rows(i)], q_v.at[rows(i)])]

    def chunk_copies(i):
        return [pltpu.make_async_copy(s, d, sem_in.at[i - 3]) for s, d in chunk_refs(i)]

    def out_copy(i, cols=slice(None)):
        return pltpu.make_async_copy(out_v.at[rows(i), cols], out_hbm.at[rows(i), cols], sem_out)

    last_copies = [out_copy(n_chunks - 1, pl.ds(l, n))
                   for l, n in ((0, KS // 2), (KS // 2, KS // 2), (KS, D - KS))]

    wmod_refs = [(wmod_hbm.at[:, pl.ds(n * D, D)], wmod_v.at[n]) for n in range(6)]
    w13_refs = [(w_hbm.at[:, pl.ds(c0 + j, 128)], w_v.at[:, pl.ds(c0 + j, 128)])
                for j in range(0, F // 2, 128)
                for w_hbm, w_v in ((w1_hbm, w1_v), (w3_hbm, w3_v)) for c0 in (0, F // 2)]
    start_groups = [
        [(shk_hbm, shk_v), (fwd_hbm, fwd_v), (inv_hbm, inv_v), (ssmd_hbm, ssmd_v), (c_hbm, c_v)]
        + chunk_refs(0)[:3],
        chunk_refs(1)[:3],
        chunk_refs(2)[:3],
        wmod_refs[:3] + [chunk_refs(0)[3], chunk_refs(1)[3]],
        wmod_refs[3:4],
        wmod_refs[4:5],
        w13_refs[:2 * CUTS[0]],
        w13_refs[2 * CUTS[0]:2 * CUTS[1]],
        w13_refs[2 * CUTS[1]:2 * CUTS[2]],
        w13_refs[2 * CUTS[2]:] + [chunk_refs(2)[3], wmod_refs[5], (w2_hbm, w2_v)],
    ]
    start_groups = [[pltpu.make_async_copy(s, d, sem_start.at[n]) for s, d in group]
                    for n, group in enumerate(start_groups)]

    def wait_group(n):
        for cp in start_groups[n]:
            cp.wait()

    def spectrum(x_ref, slot, off, tap0=None):
        e = jnp.dot(fwd_v[0], _halves(x_ref[0]), preferred_element_type=F32)
        t = jnp.dot(fwd_v[1], _halves(x_ref[1]), preferred_element_type=F32)
        if tap0 is not None:
            e = jnp.concatenate([e[:H] + tap0, e[H:]], axis=0)
        for n, x in enumerate((e + t, e - t)):
            for l in range(D // 128):
                for part in range(2):
                    spec_s[slot, (2 * l + n) * H:(2 * l + n + 1) * H, lanes(off + part)] = (
                        x[part * H:(part + 1) * H, lanes(l)])

    def ssm_d():
        return jnp.concatenate([ssmd_v[n:n + 1, :] for n in range(D // 128)], axis=1).astype(F32)

    def forward_chunk(i, first=False):
        w = [shk_v[j:j + 1, :].astype(F32) for j in range(4)]
        g = PREP_G
        for r in range(0, H, g):
            base = i * C + 2 * r
            kw = _words(k_v[aligned(base, 2 * g + HALO, HALO), :])
            k0, k1, k2 = kw[8:], pltpu.roll(kw, 1, 0)[8:], pltpu.roll(kw, 2, 0)[8:]
            vw = _words(v_v[aligned(base, 2 * g, 2 * g), :])
            ke, ko, ke1, ko1, ko2 = _even(k0), _odd(k0), _even(k1), _odd(k1), _odd(k2)
            kve = (w[0] * ke + w[1] * ko1 + w[2] * ke1 + w[3] * ko2) * _even(vw)
            kvo = (w[0] * ko + w[1] * ke + w[2] * ko1 + w[3] * ke1) * _odd(vw)
            for n, x in enumerate((kve, kvo)):
                for t in range(0, g, 16):
                    xu_s[n, (r + t) // 2:(r + t) // 2 + 8, :] = _pack(x[t:t + 8], x[t + 8:t + 16])
        yield
        spectrum(xu_s, i, 0)
        yield
        tw = _words(ssmk_v[i].T)
        for t in range(0, H, 16):
            lo, hi = tw[t:t + 8], tw[t + 8:t + 16]
            xk_s[0, t // 2:t // 2 + 8, :] = (lo & U32(0xFFFF)) | (hi << 16)
            xk_s[1, t // 2:t // 2 + 8, :] = (lo >> 16) | (hi & U32(0xFFFF0000))
        yield
        spectrum(xk_s, i, 2, ssm_d() if first else None)
        yield

    def conv_chunk(i, n_terms, dst=0):
        first = n_terms == 1
        if isinstance(i, int):
            terms = [(i - m, m) for m in range(n_terms)]
        else:
            terms = [(jnp.maximum(i - m, 0), m) for m in range(n_terms)]
        def products(row, g):
            re = im = None
            for us, ks in terms:
                ur, ui = spec_s[us, row:row + g, lanes(0)], spec_s[us, row:row + g, lanes(1)]
                kr, ki = spec_s[ks, row:row + g, lanes(2)], spec_s[ks, row:row + g, lanes(3)]
                pr, pi = ur * kr - ui * ki, ur * ki + ui * kr
                re, im = (pr, pi) if re is None else (re + pr, im + pi)
            return re, im

        g = MAC_G
        for l in range(D // 128):
            for r in range(0, H, g):
                pr, pi = products(2 * l * H + r, g)
                qr, qi = products((2 * l + 1) * H + r, g)
                for n, (re, im) in enumerate(((pr + qr, pi + qi), (pr - qr, pi - qi))):
                    last_re = spec_s.at[PREV, l * H + r:l * H + r + g, lanes(2 * n)]
                    last_im = spec_s.at[PREV, l * H + r:l * H + r + g, lanes(2 * n + 1)]
                    if first:
                        ore, oim = re, im
                    else:
                        lre, lim = last_re[...], last_im[...]
                        ore, oim = (re - lim, im + lre) if r < H // 2 else (re + lim, im - lre)
                    last_re[...] = re
                    last_im[...] = im
                    ab_s[n, r:r + g, lanes(l)] = _pack(ore, oim)
                yield
        for n in range(2):
            y_s[dst, n * H:(n + 1) * H, :] = jnp.dot(inv_v[n], _halves(ab_s[n]),
                                                 preferred_element_type=F32)
        yield

    def q_rows(i, r, g):
        qw = _words(q_v[aligned(i * C + 2 * r, 2 * g, 2 * g), :])
        return (r, _even(qw)), (H + r, _odd(qw))

    def gate_chunk(i, dst=0):
        sa, ca1, ga = (mod_v[n, 0:1, :] for n in range(3))
        scale, shift = ga * ca1, ga * sa
        g = GATE_G
        for r in range(0, H, g):
            for off, x in q_rows(i, r, g):
                val = _layernorm(x) * scale + shift
                gate_s[dst, off:off + g, :] = val
        yield

    def mix_chunk(i, src=0, dst=0, x2_ref=x2n_s):
        sb, cb1 = mod_v[3, 0:1, :], mod_v[4, 0:1, :]
        g = MIX_G
        for r in range(0, H, g):
            h2 = []
            for off, x in q_rows(i, r, g):
                x2 = x + gate_s[src, off:off + g, :] * y_s[src, off:off + g, :]
                x2_ref[dst * C + off:dst * C + off + g, :] = x2
                h2.append(_layernorm(x2) * cb1 + sb)
            w0 = (dst * H + r) // 2
            blocks = [x[:, l:l + KS // 2] for x in h2 for l in (0, KS // 2)]
            for n, x in enumerate(_left_operands(*blocks)):
                a13_s[n * H + w0:n * H + w0 + g // 2, :] = _words(x.astype(BF16))
            for n, x in enumerate(h2):
                hr_s[n * H + w0:n * H + w0 + g // 2, :] = _words(x[:, KS:].astype(BF16))
            yield

    def prepare(i, n_terms):
        yield from gate_chunk(i)
        yield from forward_chunk(i)
        yield from conv_chunk(i, n_terms)
        yield from mix_chunk(i)

    def modulation(n):
        cf = c_v[...].astype(F32)
        sc = jnp.broadcast_to(_silu(cf), (16, D)).astype(BF16)
        m = jnp.dot(sc, wmod_v[n], preferred_element_type=F32)[0:8]
        m = 1.0 + m if n in (1, 4) else m
        mod_v[n] = m * {3: 0.5, 4: 0.5, 5: 2.0}.get(n, 1.0)

    def swiglu(gate, up):
        return (gate * jnp.tanh(gate) + gate) * up

    def store_out(i, cols, src, even, odd):
        gb = mod_v[5, 0:1, cols]
        even = x2_s[src:src + H, cols] + gb * even
        odd = x2_s[src + H:src + C, cols] + gb * odd
        out_v[rows(i), cols] = _halves(_pack(even, odd))

    def right_factors(dst, src, row, col, cols):
        for r in range(0, row, 16):
            w = [_words(src[r0 + r:r0 + r + 16, c0 + cols.start:c0 + cols.stop])
                 for r0 in (0, row) for c0 in (0, col)]
            even = _right_operands(*map(_even, w))
            odd = _right_operands(*map(_odd, w))
            for n in range(7):
                dst[n, r // 2:r // 2 + 8, cols] = (
                    w[0] if n == 1 else w[3] if n == 4 else _pack(even[n], odd[n]))

    def ffn_chunk(i, n=1, first=False, last=False):
        m_rows = n * H

        def words(m):
            return slice(m * H, m * H + m_rows // 2)

        if not first:
            x2_s[0:C, :] = x2n_s[...]
        rest = jnp.concatenate([hr_s[words(0), :], hr_s[words(1), :]], axis=0)
        ft = 128 if first else FT
        for j in range(0, F // 2, ft):
            cols, cols2 = slice(j, j + ft), slice(F // 2 + j, F // 2 + j + ft)
            pre = []
            for t, w_v in enumerate((w1_v, w3_v)):
                if first:
                    right_factors(b13_s.at[t], w_v, KS // 2, F // 2, cols)
                    r13_s[t, :, cols] = _words(w_v[KS:, cols])
                    r13_s[t, :, cols2] = _words(w_v[KS:, cols2])
                c11, c12, c21, c22 = _product_blocks(
                    [_dot(a13_s[words(m), :], b13_s[t, m, :, cols]) for m in range(7)])
                r1, r2 = _dot(rest, r13_s[t, :, cols]), _dot(rest, r13_s[t, :, cols2])
                pre.append((c11 + r1[:m_rows], c12 + r2[:m_rows],
                            c21 + r1[m_rows:], c22 + r2[m_rows:]))
                yield
            act = [swiglu(gate, up) for gate, up in zip(*pre)]
            for m, x in enumerate(_left_operands(*act) + act[1:3]):
                a2_s[words(m), cols] = _words(x.astype(BF16))

        def store(cols, even, odd):
            for t in range(n):
                store_out(i + t, cols, t * C, even[t * H:(t + 1) * H], odd[t * H:(t + 1) * H])

        if first:
            r2_s[...] = _words(w2_v[:, KS:])
        act = jnp.concatenate(
            [jnp.concatenate([a2_s[words(m), :] for m in pair], axis=1) for pair in ((2, 7), (8, 3))],
            axis=0)
        o = _dot(act, r2_s[...])
        store(slice(KS, D), o[:m_rows], o[m_rows:])
        if last:
            last_copies[2].start()
        yield
        if first:
            right_factors(b2_s, w2_v, F // 2, KS // 2, slice(0, KS // 2))
        products = []
        for m in range(7):
            products.append(_dot(a2_s[words(m), :], b2_s[m]))
            yield
        c11, c12, c21, c22 = _product_blocks(products)
        store(slice(0, KS // 2), c11, c21)
        store(slice(KS // 2, KS), c12, c22)
        if last:
            last_copies[0].start()
            last_copies[1].start()

    for group in start_groups:
        for cp in group:
            cp.start()
        pl.delay(1)

    def start_chunk(i, carry):
        for cp in chunk_copies(i):
            cp.start()
        return i

    zero = jax.lax.fori_loop(3, n_chunks, start_chunk, 0) - (n_chunks - 1)
    zero = zero if OPAQUE else 0

    k_v[0:HALO, :] = jnp.zeros((HALO, D), BF16)
    for m in range(3, n_chunks):
        spec_s[m, :, 256:512] = jnp.zeros((spec_s.shape[1], 256), F32)
    with jax.named_scope("conv0"):
        conv = [conv_chunk(zero + i, i + 1, i) for i in range(3)]
        wait_group(0)
        _emit({"A": forward_chunk(0, True)})
        wait_group(1)
        _emit({"A": forward_chunk(1), "P": conv[0]}, ORDER1)
        wait_group(2)
        _emit({"A": forward_chunk(2), "P": conv[1]}, ORDER1)
        _emit({"P": conv[2]})
    with jax.named_scope("mod"):
        wait_group(3)
        for n in range(3):
            modulation(n)
        _emit({"P": gate_chunk(0), "Q": gate_chunk(1, 1)})
        for n in range(3, 5):
            wait_group(n + 1)
            modulation(n)
    with jax.named_scope("mix0"):
        _emit({"P": mix_chunk(0, 0, 0, x2_s), "Q": mix_chunk(1, 1, 1, x2_s)})

    n_mac = H // MAC_G * (D // 128)

    def arrivals():
        for n in range(6, 10):
            wait_group(n)
            if n == 9:
                modulation(5)
            yield

    def third_chunk():
        yield from gate_chunk(2, 2)
        yield from mix_chunk(2, 2)

    with jax.named_scope("step0"):
        _emit({"W": arrivals(), "F": ffn_chunk(0, 2, first=True), "P": third_chunk()},
              "".join("W" + "F" * (b - a) for a, b in zip((0, *CUTS), (*CUTS, 13))) + "P" + "PF" * 7)
    out_copy(0).start()
    out_copy(1).start()

    def step(n_terms, i, carry):
        with jax.named_scope("waitc"):
            for cp in chunk_copies(i + 1):
                cp.wait()
        with jax.named_scope("body"):
            _emit({"F": ffn_chunk(i), "P": prepare(i + 1, n_terms)}, _order(*POS, n_mac))
        out_copy(i).start()
        return carry

    jax.lax.fori_loop(2, n_chunks - 1, functools.partial(step, n_chunks), 0)
    with jax.named_scope("last"):
        _emit({"F": ffn_chunk(n_chunks - 1, last=True)})
    with jax.named_scope("outwait"):
        for i in range(n_chunks - 1):
            out_copy(i).wait()
        for cp in last_copies:
            cp.wait()


@jax.jit
def pallas_adaLN_cond__ssm_conv_h3__glu_gated_swiglu__prompt_kernel(
    A_q: jax.Array,
    A_k: jax.Array,
    A_v: jax.Array,
    A_shift_k: jax.Array,
    A_ssm_k: jax.Array,
    A_ssm_D: jax.Array,
    B_x: jax.Array,
    B_w1: jax.Array,
    B_w3: jax.Array,
    B_w2: jax.Array,
    c: jax.Array,
    w_mod: jax.Array,
):
    del B_x
    B, S, D = A_q.shape
    F = B_w1.shape[1]
    ks = A_shift_k.shape[1]
    assert B == 1 and ks == 4 and S % C == 0 and D % 128 == 0 and F % FT == 0
    n_chunks = S // C
    fwd, inv = _dft_matrices()

    vmem = pltpu.VMEM
    scratch = [
        vmem((S, D), BF16),
        vmem((HALO + S, D), BF16),
        vmem((S, D), BF16),
        vmem((n_chunks, D, C), BF16),
        vmem((D, F), BF16), vmem((D, F), BF16), vmem((F, D), BF16),
        vmem((6, D, D), BF16),
        vmem((S, D), BF16),
        vmem((2, 7, KS // 4, F // 2), U32),
        vmem((2, (D - KS) // 2, F), U32),
        vmem((7, F // 4, KS // 2), U32),
        vmem((F // 2, D - KS), U32),
        vmem((ks, D), BF16), vmem((D // 128, 128), BF16), vmem((1, D), BF16),
        vmem(fwd.shape, BF16), vmem(inv.shape, BF16),
        vmem((6, 8, D), F32),
        vmem((2, H // 2, D), U32), vmem((2, H // 2, D), U32),
        vmem((n_chunks + 1, D // 128 * C, 4 * 128), F32),
        vmem((2, C // 2, D), U32),
        vmem((3, C, D), F32),
        vmem((3, C, D), F32),
        vmem((C, D), F32), vmem((2 * C, D), F32),
        vmem((7 * H, KS // 2), U32),
        vmem((2 * H, D - KS), U32),
        vmem((9 * H, F // 2), U32),
        pltpu.SemaphoreType.DMA((n_chunks - 3,)),
        pltpu.SemaphoreType.DMA((9,)),
        pltpu.SemaphoreType.DMA(()),
    ]
    out = pl.pallas_call(
        _kernel,
        out_shape=jax.ShapeDtypeStruct((S, D), A_q.dtype),
        in_specs=[pl.BlockSpec(memory_space=pl.ANY)] * 13,
        out_specs=pl.BlockSpec(memory_space=pl.ANY),
        scratch_shapes=scratch,
        compiler_params=pltpu.CompilerParams(vmem_limit_bytes=100 * 2**20, **FLAGS),
    )(A_q.reshape(S, D), A_k.reshape(S, D), A_v.reshape(S, D), A_shift_k.T, A_ssm_k,
      A_ssm_D.reshape(D // 128, 128), B_w1, B_w3, B_w2, c, w_mod, fwd, inv)
    return out.reshape(B, S, D)
```

```python
import functools

import numpy as np

import jax
import jax.numpy as jnp
import jax.experimental.pallas as pl
import jax.experimental.pallas.tpu as pltpu

C = 256
H = C // 2
HALO = 16
FT = 256
KS = 512
EPS = 1e-5
SER_PREP = False
SER_GATE = (1, 1)
SER_MIX = (2, 1)
MAC_G = 8
OPAQUE = True
CUTS = (1, 5, 11)
ORDER1 = "A" + "P" * (640 // MAC_G) + "AAAP"
PREP_G = 32
GATE_G = 16
MIX_G = 16
FLAGS = {}
POS = (0,2,11)
F32 = jnp.float32
BF16 = jnp.bfloat16
U32 = jnp.uint32


def _dft_matrices():
    f = np.concatenate([np.arange(0, H, 2), np.arange(1, H, 2)]).astype(np.float64)
    theta = 2.0 * np.pi * (f + 0.5) / (2 * C)
    r = np.arange(H, dtype=np.float64)
    fwd, inv = [], []
    for phase in (0, 1):
        ang = theta[:, None] * (2.0 * r + phase)[None, :]
        m = np.concatenate([np.cos(ang), -np.sin(ang)], axis=0)
        fwd.append(m.reshape(C, H // 16, 2, 8).transpose(0, 1, 3, 2).reshape(C, H))
        inv.append(m.reshape(2, H, H).transpose(2, 1, 0).reshape(H, C) / C)
    return np.stack(fwd).astype(BF16), np.stack(inv).astype(BF16)


def lanes(n):
    return slice(n * 128, (n + 1) * 128)


def _words(x):
    return pltpu.bitcast(x, jnp.uint32)


def _halves(w):
    return pltpu.bitcast(w, BF16)


def _pack(lo, hi):
    return pltpu.bitcast(pltpu.pack_elementwise([lo, hi], packed_dtype=BF16), U32)


def _even(w):
    return pltpu.bitcast(w << 16, F32)


def _odd(w):
    return pltpu.bitcast(w & jnp.uint32(0xFFFF0000), F32)


def _left_operands(a11, a12, a21, a22):
    return [a11 + a22, a21 + a22, a11, a22, a11 + a12, a21 - a11, a12 - a22]


def _right_operands(b11, b12, b21, b22):
    return [b11 + b22, b11, b12 - b22, b21 - b11, b22, b11 + b12, b21 + b22]


def _product_blocks(m):
    return m[0] + m[3] - m[4] + m[6], m[2] + m[4], m[1] + m[3], m[0] - m[1] + m[2] + m[5]


def _dot(a, b):
    return jnp.dot(_halves(a), _halves(b), preferred_element_type=F32)


def _layernorm(x):
    m = jnp.mean(x, axis=-1, keepdims=True)
    d = x - m
    v = jnp.mean(d * d, axis=-1, keepdims=True)
    return d * jax.lax.rsqrt(v + EPS)


def _silu(x):
    hx = 0.5 * x
    return hx * jnp.tanh(hx) + hx


def _order(a, b, c, n_mac):
    mac = ""
    for n in range(c - b):
        mac += "P" * ((n + 1) * n_mac // (c - b) - n * n_mac // (c - b)) + "F"
    return "PP" + "F" * a + "PP" + "F" * (b - a) + "P" + mac + "P" + "FPP" * 4


def _emit(gens, order=""):
    for key in order:
        next(gens[key], None)
    for g in gens.values():
        for _ in g:
            pass


def _kernel(q_hbm, k_hbm, v_hbm, shk_hbm, ssmk_hbm, ssmd_hbm, w1_hbm, w3_hbm, w2_hbm, c_hbm,
            wmod_hbm, fwd_hbm, inv_hbm, out_hbm,
            q_v, k_v, v_v, ssmk_v, w1_v, w3_v, w2_v, wmod_v, out_v, b13_s, r13_s, b2_s, r2_s,
            shk_v, ssmd_v, c_v, fwd_v, inv_v, mod_v,
            xu_s, xk_s, spec_s, ab_s, y_s, gate_s, x2n_s, x2_s, a13_s, hr_s, a2_s,
            sem_in, sem_start, sem_out):
    S, D = q_v.shape
    F = w1_v.shape[1]
    n_chunks = S // C
    PREV = n_chunks

    def aligned(start, size, align):
        return pl.ds(start if isinstance(start, int) else pl.multiple_of(start, align), size)

    def rows(i):
        return aligned(i * C, C, C)

    def chunk_refs(i):
        return [(k_hbm.at[rows(i)], k_v.at[aligned(i * C + HALO, C, HALO)]),
                (v_hbm.at[rows(i)], v_v.at[rows(i)]),
                (ssmk_hbm.at[:, rows(i)], ssmk_v.at[i]),
                (q_hbm.at[rows(i)], q_v.at[rows(i)])]

    def chunk_copies(i):
        return [pltpu.make_async_copy(s, d, sem_in.at[i - 3]) for s, d in chunk_refs(i)]

    def out_copy(i, cols=slice(None)):
        return pltpu.make_async_copy(out_v.at[rows(i), cols], out_hbm.at[rows(i), cols], sem_out)

    last_copies = [out_copy(n_chunks - 1, pl.ds(l, n))
                   for l, n in ((0, KS // 2), (KS // 2, KS // 2), (KS, D - KS))]

    wmod_refs = [(wmod_hbm.at[:, pl.ds(n * D, D)], wmod_v.at[n]) for n in range(6)]
    w13_refs = [(w_hbm.at[:, pl.ds(c0 + j, 128)], w_v.at[:, pl.ds(c0 + j, 128)])
                for j in range(0, F // 2, 128)
                for w_hbm, w_v in ((w1_hbm, w1_v), (w3_hbm, w3_v)) for c0 in (0, F // 2)]
    start_groups = [
        [(shk_hbm, shk_v), (fwd_hbm, fwd_v), (inv_hbm, inv_v), (ssmd_hbm, ssmd_v), (c_hbm, c_v)]
        + chunk_refs(0)[:3],
        chunk_refs(1)[:3],
        chunk_refs(2)[:3],
        wmod_refs[:3] + [chunk_refs(0)[3], chunk_refs(1)[3]],
        wmod_refs[3:4],
        wmod_refs[4:5],
        w13_refs[:2 * CUTS[0]],
        w13_refs[2 * CUTS[0]:2 * CUTS[1]],
        w13_refs[2 * CUTS[1]:2 * CUTS[2]],
        w13_refs[2 * CUTS[2]:] + [chunk_refs(2)[3], wmod_refs[5], (w2_hbm, w2_v)],
    ]
    start_groups = [[pltpu.make_async_copy(s, d, sem_start.at[n]) for s, d in group]
                    for n, group in enumerate(start_groups)]

    def wait_group(n):
        for cp in start_groups[n]:
            cp.wait()

    def spectrum(x_ref, slot, off, tap0=None):
        e = jnp.dot(fwd_v[0], _halves(x_ref[0]), preferred_element_type=F32)
        t = jnp.dot(fwd_v[1], _halves(x_ref[1]), preferred_element_type=F32)
        if tap0 is not None:
            e = jnp.concatenate([e[:H] + tap0, e[H:]], axis=0)
        for n, x in enumerate((e + t, e - t)):
            for l in range(D // 128):
                for part in range(2):
                    spec_s[slot, (2 * l + n) * H:(2 * l + n + 1) * H, lanes(off + part)] = (
                        x[part * H:(part + 1) * H, lanes(l)])

    def chain(ref, val):
        spare = ref.shape[0] - 16
        ref[pl.ds(pl.multiple_of(zero + spare, 16), 16), lanes(0)] = val[-16:, lanes(0)].astype(BF16)

    def ssm_d():
        return jnp.concatenate([ssmd_v[n:n + 1, :] for n in range(D // 128)], axis=1).astype(F32)

    def forward_chunk(i, first=False):
        w = [shk_v[j:j + 1, :].astype(F32) for j in range(4)]
        g = PREP_G
        for r in range(0, H, g):
            base = i * C + 2 * r
            kw = _words(k_v[aligned(base, 2 * g + HALO, HALO), :])
            k0, k1, k2 = kw[8:], pltpu.roll(kw, 1, 0)[8:], pltpu.roll(kw, 2, 0)[8:]
            vw = _words(v_v[aligned(base, 2 * g, 2 * g), :])
            ke, ko, ke1, ko1, ko2 = _even(k0), _odd(k0), _even(k1), _odd(k1), _odd(k2)
            kve = (w[0] * ke + w[1] * ko1 + w[2] * ke1 + w[3] * ko2) * _even(vw)
            kvo = (w[0] * ko + w[1] * ke + w[2] * ko1 + w[3] * ke1) * _odd(vw)
            for n, x in enumerate((kve, kvo)):
                for t in range(0, g, 16):
                    xu_s[n, (r + t) // 2:(r + t) // 2 + 8, :] = _pack(x[t:t + 8], x[t + 8:t + 16])
            if SER_PREP and not isinstance(i, int):
                chain(k_v, kvo)
        yield
        spectrum(xu_s, i, 0)
        yield
        tw = _words(ssmk_v[i].T)
        for t in range(0, H, 16):
            lo, hi = tw[t:t + 8], tw[t + 8:t + 16]
            xk_s[0, t // 2:t // 2 + 8, :] = (lo & U32(0xFFFF)) | (hi << 16)
            xk_s[1, t // 2:t // 2 + 8, :] = (lo >> 16) | (hi & U32(0xFFFF0000))
        yield
        spectrum(xk_s, i, 2, ssm_d() if first else None)
        yield

    def conv_chunk(i, n_terms, dst=0):
        first = n_terms == 1
        if isinstance(i, int):
            terms = [(i - m, m) for m in range(n_terms)]
        else:
            terms = [(jnp.maximum(i - m, 0), m) for m in range(n_terms)]
        def products(row, g):
            re = im = None
            for us, ks in terms:
                ur, ui = spec_s[us, row:row + g, lanes(0)], spec_s[us, row:row + g, lanes(1)]
                kr, ki = spec_s[ks, row:row + g, lanes(2)], spec_s[ks, row:row + g, lanes(3)]
                pr, pi = ur * kr - ui * ki, ur * ki + ui * kr
                re, im = (pr, pi) if re is None else (re + pr, im + pi)
            return re, im

        g = MAC_G
        for l in range(D // 128):
            for r in range(0, H, g):
                pr, pi = products(2 * l * H + r, g)
                qr, qi = products((2 * l + 1) * H + r, g)
                for n, (re, im) in enumerate(((pr + qr, pi + qi), (pr - qr, pi - qi))):
                    last_re = spec_s.at[PREV, l * H + r:l * H + r + g, lanes(2 * n)]
                    last_im = spec_s.at[PREV, l * H + r:l * H + r + g, lanes(2 * n + 1)]
                    if first:
                        ore, oim = re, im
                    else:
                        lre, lim = last_re[...], last_im[...]
                        ore, oim = (re - lim, im + lre) if r < H // 2 else (re + lim, im - lre)
                    last_re[...] = re
                    last_im[...] = im
                    ab_s[n, r:r + g, lanes(l)] = _pack(ore, oim)
                yield
        for n in range(2):
            y_s[dst, n * H:(n + 1) * H, :] = jnp.dot(inv_v[n], _halves(ab_s[n]),
                                                 preferred_element_type=F32)
        yield

    def q_rows(i, r, g):
        qw = _words(q_v[aligned(i * C + 2 * r, 2 * g, 2 * g), :])
        return (r, _even(qw)), (H + r, _odd(qw))

    def gate_chunk(i, dst=0):
        sa, ca1, ga = (mod_v[n, 0:1, :] for n in range(3))
        scale, shift = ga * ca1, ga * sa
        g = GATE_G
        for r in range(0, H, g):
            for off, x in q_rows(i, r, g):
                val = _layernorm(x) * scale + shift
                gate_s[dst, off:off + g, :] = val
            if SER_GATE[isinstance(i, int)] and (not isinstance(i, int) or i == 2):
                chain(q_v, val)
        yield

    def mix_chunk(i, src=0, dst=0, x2_ref=x2n_s):
        sb, cb1 = mod_v[3, 0:1, :], mod_v[4, 0:1, :]
        g = MIX_G
        for r in range(0, H, g):
            h2 = []
            for off, x in q_rows(i, r, g):
                x2 = x + gate_s[src, off:off + g, :] * y_s[src, off:off + g, :]
                x2_ref[dst * C + off:dst * C + off + g, :] = x2
                h2.append(_layernorm(x2) * cb1 + sb)
            w0 = (dst * H + r) // 2
            blocks = [x[:, l:l + KS // 2] for x in h2 for l in (0, KS // 2)]
            for n, x in enumerate(_left_operands(*blocks)):
                a13_s[n * H + w0:n * H + w0 + g // 2, :] = _words(x.astype(BF16))
            for n, x in enumerate(h2):
                hr_s[n * H + w0:n * H + w0 + g // 2, :] = _words(x[:, KS:].astype(BF16))
            if SER_MIX[isinstance(i, int)] and (not isinstance(i, int) or i == 2):
                chain(q_v, h2[1] if SER_MIX[isinstance(i, int)] == 1 else x2)
            yield

    def prepare(i, n_terms):
        yield from gate_chunk(i)
        yield from forward_chunk(i)
        yield from conv_chunk(i, n_terms)
        yield from mix_chunk(i)

    def modulation(n):
        cf = c_v[...].astype(F32)
        sc = jnp.broadcast_to(_silu(cf), (16, D)).astype(BF16)
        m = jnp.dot(sc, wmod_v[n], preferred_element_type=F32)[0:8]
        m = 1.0 + m if n in (1, 4) else m
        mod_v[n] = m * {3: 0.5, 4: 0.5, 5: 2.0}.get(n, 1.0)

    def swiglu(gate, up):
        return (gate * jnp.tanh(gate) + gate) * up

    def store_out(i, cols, src, even, odd):
        gb = mod_v[5, 0:1, cols]
        even = x2_s[src:src + H, cols] + gb * even
        odd = x2_s[src + H:src + C, cols] + gb * odd
        out_v[rows(i), cols] = _halves(_pack(even, odd))

    def right_factors(dst, src, row, col, cols):
        for r in range(0, row, 16):
            w = [_words(src[r0 + r:r0 + r + 16, c0 + cols.start:c0 + cols.stop])
                 for r0 in (0, row) for c0 in (0, col)]
            even = _right_operands(*map(_even, w))
            odd = _right_operands(*map(_odd, w))
            for n in range(7):
                dst[n, r // 2:r // 2 + 8, cols] = (
                    w[0] if n == 1 else w[3] if n == 4 else _pack(even[n], odd[n]))

    def ffn_chunk(i, n=1, first=False, last=False):
        m_rows = n * H

        def words(m):
            return slice(m * H, m * H + m_rows // 2)

        if not first:
            x2_s[0:C, :] = x2n_s[...]
        rest = jnp.concatenate([hr_s[words(0), :], hr_s[words(1), :]], axis=0)
        ft = 128 if first else FT
        for j in range(0, F // 2, ft):
            cols, cols2 = slice(j, j + ft), slice(F // 2 + j, F // 2 + j + ft)
            pre = []
            for t, w_v in enumerate((w1_v, w3_v)):
                if first:
                    right_factors(b13_s.at[t], w_v, KS // 2, F // 2, cols)
                    r13_s[t, :, cols] = _words(w_v[KS:, cols])
                    r13_s[t, :, cols2] = _words(w_v[KS:, cols2])
                c11, c12, c21, c22 = _product_blocks(
                    [_dot(a13_s[words(m), :], b13_s[t, m, :, cols]) for m in range(7)])
                r1, r2 = _dot(rest, r13_s[t, :, cols]), _dot(rest, r13_s[t, :, cols2])
                pre.append((c11 + r1[:m_rows], c12 + r2[:m_rows],
                            c21 + r1[m_rows:], c22 + r2[m_rows:]))
                yield
            act = [swiglu(gate, up) for gate, up in zip(*pre)]
            for m, x in enumerate(_left_operands(*act) + act[1:3]):
                a2_s[words(m), cols] = _words(x.astype(BF16))

        def store(cols, even, odd):
            for t in range(n):
                store_out(i + t, cols, t * C, even[t * H:(t + 1) * H], odd[t * H:(t + 1) * H])

        if first:
            r2_s[...] = _words(w2_v[:, KS:])
        act = jnp.concatenate(
            [jnp.concatenate([a2_s[words(m), :] for m in pair], axis=1) for pair in ((2, 7), (8, 3))],
            axis=0)
        o = _dot(act, r2_s[...])
        store(slice(KS, D), o[:m_rows], o[m_rows:])
        if last:
            last_copies[2].start()
        yield
        if first:
            right_factors(b2_s, w2_v, F // 2, KS // 2, slice(0, KS // 2))
        products = []
        for m in range(7):
            products.append(_dot(a2_s[words(m), :], b2_s[m]))
            yield
        c11, c12, c21, c22 = _product_blocks(products)
        store(slice(0, KS // 2), c11, c21)
        store(slice(KS // 2, KS), c12, c22)
        if last:
            last_copies[0].start()
            last_copies[1].start()

    for group in start_groups:
        for cp in group:
            cp.start()
        pl.delay(1)

    def start_chunk(i, carry):
        for cp in chunk_copies(i):
            cp.start()
        return i

    zero = jax.lax.fori_loop(3, n_chunks, start_chunk, 0) - (n_chunks - 1)
    zero = zero if OPAQUE else 0

    k_v[0:HALO, :] = jnp.zeros((HALO, D), BF16)
    for m in range(3, n_chunks):
        spec_s[m, :, 256:512] = jnp.zeros((spec_s.shape[1], 256), F32)
    with jax.named_scope("conv0"):
        conv = [conv_chunk(zero + i, i + 1, i) for i in range(3)]
        wait_group(0)
        _emit({"A": forward_chunk(0, True)})
        wait_group(1)
        _emit({"A": forward_chunk(1), "P": conv[0]}, ORDER1)
        wait_group(2)
        _emit({"A": forward_chunk(2), "P": conv[1]}, ORDER1)
        _emit({"P": conv[2]})
    with jax.named_scope("mod"):
        wait_group(3)
        for n in range(3):
            modulation(n)
        _emit({"P": gate_chunk(0), "Q": gate_chunk(1, 1)})
        for n in range(3, 5):
            wait_group(n + 1)
            modulation(n)
    with jax.named_scope("mix0"):
        _emit({"P": mix_chunk(0, 0, 0, x2_s), "Q": mix_chunk(1, 1, 1, x2_s)})

    n_mac = H // MAC_G * (D // 128)

    def arrivals():
        for n in range(6, 10):
            wait_group(n)
            if n == 9:
                modulation(5)
            yield

    def third_chunk():
        yield from gate_chunk(2, 2)
        yield from mix_chunk(2, 2)

    with jax.named_scope("step0"):
        _emit({"W": arrivals(), "F": ffn_chunk(0, 2, first=True), "P": third_chunk()},
              "".join("W" + "F" * (b - a) for a, b in zip((0, *CUTS), (*CUTS, 13))) + "P" + "PF" * 7)
    out_copy(0).start()
    out_copy(1).start()

    def step(n_terms, i, carry):
        with jax.named_scope("waitc"):
            for cp in chunk_copies(i + 1):
                cp.wait()
        with jax.named_scope("body"):
            _emit({"F": ffn_chunk(i), "P": prepare(i + 1, n_terms)}, _order(*POS, n_mac))
        out_copy(i).start()
        return carry

    jax.lax.fori_loop(2, n_chunks - 1, functools.partial(step, n_chunks), 0)
    with jax.named_scope("last"):
        _emit({"F": ffn_chunk(n_chunks - 1, last=True)})
    with jax.named_scope("outwait"):
        for i in range(n_chunks - 1):
            out_copy(i).wait()
        for cp in last_copies:
            cp.wait()


@jax.jit
def pallas_adaLN_cond__ssm_conv_h3__glu_gated_swiglu__prompt_kernel(
    A_q: jax.Array,
    A_k: jax.Array,
    A_v: jax.Array,
    A_shift_k: jax.Array,
    A_ssm_k: jax.Array,
    A_ssm_D: jax.Array,
    B_x: jax.Array,
    B_w1: jax.Array,
    B_w3: jax.Array,
    B_w2: jax.Array,
    c: jax.Array,
    w_mod: jax.Array,
):
    del B_x
    B, S, D = A_q.shape
    F = B_w1.shape[1]
    ks = A_shift_k.shape[1]
    assert B == 1 and ks == 4 and S % C == 0 and D % 128 == 0 and F % FT == 0
    n_chunks = S // C
    fwd, inv = _dft_matrices()

    vmem = pltpu.VMEM
    scratch = [
        vmem((S + 16, D), BF16),
        vmem((HALO + S + 16, D), BF16),
        vmem((S, D), BF16),
        vmem((n_chunks, D, C), BF16),
        vmem((D, F), BF16), vmem((D, F), BF16), vmem((F, D), BF16),
        vmem((6, D, D), BF16),
        vmem((S, D), BF16),
        vmem((2, 7, KS // 4, F // 2), U32),
        vmem((2, (D - KS) // 2, F), U32),
        vmem((7, F // 4, KS // 2), U32),
        vmem((F // 2, D - KS), U32),
        vmem((ks, D), BF16), vmem((D // 128, 128), BF16), vmem((1, D), BF16),
        vmem(fwd.shape, BF16), vmem(inv.shape, BF16),
        vmem((6, 8, D), F32),
        vmem((2, H // 2, D), U32), vmem((2, H // 2, D), U32),
        vmem((n_chunks + 1, D // 128 * C, 4 * 128), F32),
        vmem((2, C // 2, D), U32),
        vmem((3, C, D), F32),
        vmem((3, C, D), F32),
        vmem((C, D), F32), vmem((2 * C, D), F32),
        vmem((7 * H, KS // 2), U32),
        vmem((2 * H, D - KS), U32),
        vmem((9 * H, F // 2), U32),
        pltpu.SemaphoreType.DMA((n_chunks - 3,)),
        pltpu.SemaphoreType.DMA((9,)),
        pltpu.SemaphoreType.DMA(()),
    ]
    out = pl.pallas_call(
        _kernel,
        out_shape=jax.ShapeDtypeStruct((S, D), A_q.dtype),
        in_specs=[pl.BlockSpec(memory_space=pl.ANY)] * 13,
        out_specs=pl.BlockSpec(memory_space=pl.ANY),
        scratch_shapes=scratch,
        compiler_params=pltpu.CompilerParams(vmem_limit_bytes=100 * 2**20, **FLAGS),
    )(A_q.reshape(S, D), A_k.reshape(S, D), A_v.reshape(S, D), A_shift_k.T, A_ssm_k,
      A_ssm_D.reshape(D // 128, 128), B_w1, B_w3, B_w2, c, w_mod, fwd, inv)
    return out.reshape(B, S, D)
```

```python
import functools

import numpy as np

import jax
import jax.numpy as jnp
import jax.experimental.pallas as pl
import jax.experimental.pallas.tpu as pltpu

C = 256
H = C // 2
HALO = 16
FT = 256
KS = 512
EPS = 1e-5
SER_PREP = False
SER_GATE = (1, 1)
MAC_G = 8
OPAQUE = True
CUTS = (1, 5, 11)
ORDER1 = "A" + "P" * (640 // MAC_G) + "AAAP"
PREP_G = 32
GATE_G = 16
MIX_G = 32
FLAGS = {}
POS = (0,2,11)
F32 = jnp.float32
BF16 = jnp.bfloat16
U32 = jnp.uint32


def _dft_matrices():
    f = np.concatenate([np.arange(0, H, 2), np.arange(1, H, 2)]).astype(np.float64)
    theta = 2.0 * np.pi * (f + 0.5) / (2 * C)
    r = np.arange(H, dtype=np.float64)
    fwd, inv = [], []
    for phase in (0, 1):
        ang = theta[:, None] * (2.0 * r + phase)[None, :]
        m = np.concatenate([np.cos(ang), -np.sin(ang)], axis=0)
        fwd.append(m.reshape(C, H // 16, 2, 8).transpose(0, 1, 3, 2).reshape(C, H))
        inv.append(m.reshape(2, H, H).transpose(2, 1, 0).reshape(H, C) / C)
    return np.stack(fwd).astype(BF16), np.stack(inv).astype(BF16)


def lanes(n):
    return slice(n * 128, (n + 1) * 128)


def _words(x):
    return pltpu.bitcast(x, jnp.uint32)


def _halves(w):
    return pltpu.bitcast(w, BF16)


def _pack(lo, hi):
    return pltpu.bitcast(pltpu.pack_elementwise([lo, hi], packed_dtype=BF16), U32)


def _even(w):
    return pltpu.bitcast(w << 16, F32)


def _odd(w):
    return pltpu.bitcast(w & jnp.uint32(0xFFFF0000), F32)


def _left_operands(a11, a12, a21, a22):
    return [a11 + a22, a21 + a22, a11, a22, a11 + a12, a21 - a11, a12 - a22]


def _right_operands(b11, b12, b21, b22):
    return [b11 + b22, b11, b12 - b22, b21 - b11, b22, b11 + b12, b21 + b22]


def _product_blocks(m):
    return m[0] + m[3] - m[4] + m[6], m[2] + m[4], m[1] + m[3], m[0] - m[1] + m[2] + m[5]


def _dot(a, b):
    return jnp.dot(_halves(a), _halves(b), preferred_element_type=F32)


def _layernorm(x):
    m = jnp.mean(x, axis=-1, keepdims=True)
    d = x - m
    v = jnp.mean(d * d, axis=-1, keepdims=True)
    return d * jax.lax.rsqrt(v + EPS)


def _silu(x):
    hx = 0.5 * x
    return hx * jnp.tanh(hx) + hx


def _order(a, b, c, n_mac):
    mac = ""
    for n in range(c - b):
        mac += "P" * ((n + 1) * n_mac // (c - b) - n * n_mac // (c - b)) + "F"
    return "PP" + "F" * a + "PP" + "F" * (b - a) + "P" + mac + "P" + "FPP" * 4


def _emit(gens, order=""):
    for key in order:
        next(gens[key], None)
    for g in gens.values():
        for _ in g:
            pass


def _kernel(q_hbm, k_hbm, v_hbm, shk_hbm, ssmk_hbm, ssmd_hbm, w1_hbm, w3_hbm, w2_hbm, c_hbm,
            wmod_hbm, fwd_hbm, inv_hbm, out_hbm,
            q_v, k_v, v_v, ssmk_v, w1_v, w3_v, w2_v, wmod_v, out_v, b13_s, r13_s, b2_s, r2_s,
            shk_v, ssmd_v, c_v, fwd_v, inv_v, mod_v,
            xu_s, xk_s, spec_s, ab_s, y_s, gate_s, x2n_s, x2_s, a13_s, hr_s, a2_s,
            sem_in, sem_start, sem_out):
    S, D = v_v.shape
    F = w1_v.shape[1]
    n_chunks = S // C
    PREV = n_chunks

    def aligned(start, size, align):
        return pl.ds(start if isinstance(start, int) else pl.multiple_of(start, align), size)

    def rows(i):
        return aligned(i * C, C, C)

    def chunk_refs(i):
        return [(k_hbm.at[rows(i)], k_v.at[aligned(i * C + HALO, C, HALO)]),
                (v_hbm.at[rows(i)], v_v.at[rows(i)]),
                (ssmk_hbm.at[:, rows(i)], ssmk_v.at[i]),
                (q_hbm.at[rows(i)], q_v.at[rows(i)])]

    def chunk_copies(i):
        return [pltpu.make_async_copy(s, d, sem_in.at[i - 3]) for s, d in chunk_refs(i)]

    def out_copy(i, cols=slice(None)):
        return pltpu.make_async_copy(out_v.at[rows(i), cols], out_hbm.at[rows(i), cols], sem_out)

    last_copies = [out_copy(n_chunks - 1, pl.ds(l, n))
                   for l, n in ((0, KS // 2), (KS // 2, KS // 2), (KS, D - KS))]

    wmod_refs = [(wmod_hbm.at[:, pl.ds(n * D, D)], wmod_v.at[n]) for n in range(6)]
    w13_refs = [(w_hbm.at[:, pl.ds(c0 + j, 128)], w_v.at[:, pl.ds(c0 + j, 128)])
                for j in range(0, F // 2, 128)
                for w_hbm, w_v in ((w1_hbm, w1_v), (w3_hbm, w3_v)) for c0 in (0, F // 2)]
    start_groups = [
        [(shk_hbm, shk_v), (fwd_hbm, fwd_v), (inv_hbm, inv_v), (ssmd_hbm, ssmd_v), (c_hbm, c_v)]
        + chunk_refs(0)[:3],
        chunk_refs(1)[:3],
        chunk_refs(2)[:3],
        wmod_refs[:3] + [chunk_refs(0)[3], chunk_refs(1)[3]],
        wmod_refs[3:4],
        wmod_refs[4:5],
        w13_refs[:2 * CUTS[0]],
        w13_refs[2 * CUTS[0]:2 * CUTS[1]],
        w13_refs[2 * CUTS[1]:2 * CUTS[2]],
        w13_refs[2 * CUTS[2]:] + [chunk_refs(2)[3], wmod_refs[5], (w2_hbm, w2_v)],
    ]
    start_groups = [[pltpu.make_async_copy(s, d, sem_start.at[n]) for s, d in group]
                    for n, group in enumerate(start_groups)]

    def wait_group(n):
        for cp in start_groups[n]:
            cp.wait()

    def spectrum(x_ref, slot, off, tap0=None):
        e = jnp.dot(fwd_v[0], _halves(x_ref[0]), preferred_element_type=F32)
        t = jnp.dot(fwd_v[1], _halves(x_ref[1]), preferred_element_type=F32)
        if tap0 is not None:
            e = jnp.concatenate([e[:H] + tap0, e[H:]], axis=0)
        for n, x in enumerate((e + t, e - t)):
            for l in range(D // 128):
                for part in range(2):
                    spec_s[slot, (2 * l + n) * H:(2 * l + n + 1) * H, lanes(off + part)] = (
                        x[part * H:(part + 1) * H, lanes(l)])

    def chain(ref, val):
        spare = ref.shape[0] - 16
        ref[pl.ds(pl.multiple_of(zero + spare, 16), 16), lanes(0)] = val[-16:, lanes(0)].astype(BF16)

    def ssm_d():
        return jnp.concatenate([ssmd_v[n:n + 1, :] for n in range(D // 128)], axis=1).astype(F32)

    def forward_chunk(i, first=False):
        w = [shk_v[j:j + 1, :].astype(F32) for j in range(4)]
        g = PREP_G
        for r in range(0, H, g):
            base = i * C + 2 * r
            kw = _words(k_v[aligned(base, 2 * g + HALO, HALO), :])
            k0, k1, k2 = kw[8:], pltpu.roll(kw, 1, 0)[8:], pltpu.roll(kw, 2, 0)[8:]
            vw = _words(v_v[aligned(base, 2 * g, 2 * g), :])
            ke, ko, ke1, ko1, ko2 = _even(k0), _odd(k0), _even(k1), _odd(k1), _odd(k2)
            kve = (w[0] * ke + w[1] * ko1 + w[2] * ke1 + w[3] * ko2) * _even(vw)
            kvo = (w[0] * ko + w[1] * ke + w[2] * ko1 + w[3] * ke1) * _odd(vw)
            for n, x in enumerate((kve, kvo)):
                for t in range(0, g, 16):
                    xu_s[n, (r + t) // 2:(r + t) // 2 + 8, :] = _pack(x[t:t + 8], x[t + 8:t + 16])
            if SER_PREP and not isinstance(i, int):
                chain(k_v, kvo)
        yield
        spectrum(xu_s, i, 0)
        yield
        tw = _words(ssmk_v[i].T)
        for t in range(0, H, 16):
            lo, hi = tw[t:t + 8], tw[t + 8:t + 16]
            xk_s[0, t // 2:t // 2 + 8, :] = (lo & U32(0xFFFF)) | (hi << 16)
            xk_s[1, t // 2:t // 2 + 8, :] = (lo >> 16) | (hi & U32(0xFFFF0000))
        yield
        spectrum(xk_s, i, 2, ssm_d() if first else None)
        yield

    def conv_chunk(i, n_terms, dst=0):
        first = n_terms == 1
        if isinstance(i, int):
            terms = [(i - m, m) for m in range(n_terms)]
        else:
            terms = [(jnp.maximum(i - m, 0), m) for m in range(n_terms)]
        def products(row, g):
            re = im = None
            for us, ks in terms:
                ur, ui = spec_s[us, row:row + g, lanes(0)], spec_s[us, row:row + g, lanes(1)]
                kr, ki = spec_s[ks, row:row + g, lanes(2)], spec_s[ks, row:row + g, lanes(3)]
                pr, pi = ur * kr - ui * ki, ur * ki + ui * kr
                re, im = (pr, pi) if re is None else (re + pr, im + pi)
            return re, im

        g = MAC_G
        for l in range(D // 128):
            for r in range(0, H, g):
                pr, pi = products(2 * l * H + r, g)
                qr, qi = products((2 * l + 1) * H + r, g)
                for n, (re, im) in enumerate(((pr + qr, pi + qi), (pr - qr, pi - qi))):
                    last_re = spec_s.at[PREV, l * H + r:l * H + r + g, lanes(2 * n)]
                    last_im = spec_s.at[PREV, l * H + r:l * H + r + g, lanes(2 * n + 1)]
                    if first:
                        ore, oim = re, im
                    else:
                        lre, lim = last_re[...], last_im[...]
                        ore, oim = (re - lim, im + lre) if r < H // 2 else (re + lim, im - lre)
                    last_re[...] = re
                    last_im[...] = im
                    ab_s[n, r:r + g, lanes(l)] = _pack(ore, oim)
                yield
        for n in range(2):
            y_s[dst, n * H:(n + 1) * H, :] = jnp.dot(inv_v[n], _halves(ab_s[n]),
                                                 preferred_element_type=F32)
        yield

    def q_rows(i, r, g):
        qw = _words(q_v[aligned(i * C + 2 * r, 2 * g, 2 * g), :])
        return (r, _even(qw)), (H + r, _odd(qw))

    def gate_chunk(i, dst=0):
        sa, ca1, ga = (mod_v[n, 0:1, :] for n in range(3))
        scale, shift = ga * ca1, ga * sa
        g = GATE_G
        for r in range(0, H, g):
            for off, x in q_rows(i, r, g):
                val = _layernorm(x) * scale + shift
                gate_s[dst, off:off + g, :] = val
            if SER_GATE[isinstance(i, int)] and (not isinstance(i, int) or i == 2):
                chain(q_v, val)
        yield

    def residual(i, src, r, g):
        return [(off, x + gate_s[src, off:off + g, :] * y_s[src, off:off + g, :])
                for off, x in q_rows(i, r, g)]

    def store_operands(normed, row):
        sb, cb1 = mod_v[3, 0:1, :], mod_v[4, 0:1, :]
        h2 = [x * cb1 + sb for x in normed]
        lo, hi = row // 2, (row + h2[0].shape[0]) // 2
        blocks = [x[:, l:l + KS // 2] for x in h2 for l in (0, KS // 2)]
        for n, x in enumerate(_left_operands(*blocks)):
            a13_s[n * H + lo:n * H + hi, :] = _words(x.astype(BF16))
        for n, x in enumerate(h2):
            hr_s[n * H + lo:n * H + hi, :] = _words(x[:, KS:].astype(BF16))

    def mix_chunk(i, src=0):
        g = MIX_G
        for r in range(0, H, g):
            x2 = residual(i, src, r, g)
            for off, x in x2:
                x2n_s[off:off + g, :] = x
            store_operands([_layernorm(x) for _, x in x2], r)
            if not isinstance(i, int):
                chain(q_v, x2[1][1])
            yield

    def prepare(i, n_terms):
        yield from gate_chunk(i)
        yield from forward_chunk(i)
        yield from conv_chunk(i, n_terms)
        yield from mix_chunk(i)

    def modulation(n):
        cf = c_v[...].astype(F32)
        sc = jnp.broadcast_to(_silu(cf), (16, D)).astype(BF16)
        m = jnp.dot(sc, wmod_v[n], preferred_element_type=F32)[0:8]
        m = 1.0 + m if n in (1, 4) else m
        mod_v[n] = m * {3: 0.5, 4: 0.5, 5: 2.0}.get(n, 1.0)

    def swiglu(gate, up):
        return (gate * jnp.tanh(gate) + gate) * up

    def store_out(i, cols, src, even, odd):
        gb = mod_v[5, 0:1, cols]
        even = x2_s[src:src + H, cols] + gb * even
        odd = x2_s[src + H:src + C, cols] + gb * odd
        out_v[rows(i), cols] = _halves(_pack(even, odd))

    def right_factors(dst, src, row, col, cols):
        for r in range(0, row, 16):
            w = [_words(src[r0 + r:r0 + r + 16, c0 + cols.start:c0 + cols.stop])
                 for r0 in (0, row) for c0 in (0, col)]
            even = _right_operands(*map(_even, w))
            odd = _right_operands(*map(_odd, w))
            for n in range(7):
                dst[n, r // 2:r // 2 + 8, cols] = (
                    w[0] if n == 1 else w[3] if n == 4 else _pack(even[n], odd[n]))

    def ffn_chunk(i, n=1, first=False, last=False):
        m_rows = n * H

        def words(m):
            return slice(m * H, m * H + m_rows // 2)

        if not first:
            x2_s[0:C, :] = x2n_s[...]
        rest = jnp.concatenate([hr_s[words(0), :], hr_s[words(1), :]], axis=0)
        ft = 128 if first else FT
        for j in range(0, F // 2, ft):
            cols, cols2 = slice(j, j + ft), slice(F // 2 + j, F // 2 + j + ft)
            pre = []
            for t, w_v in enumerate((w1_v, w3_v)):
                if first:
                    r13_s[t, :, cols] = _words(w_v[KS:, cols])
                    r13_s[t, :, cols2] = _words(w_v[KS:, cols2])
                    right_factors(b13_s.at[t], w_v, KS // 2, F // 2, cols)
                c11, c12, c21, c22 = _product_blocks(
                    [_dot(a13_s[words(m), :], b13_s[t, m, :, cols]) for m in range(7)])
                r1, r2 = _dot(rest, r13_s[t, :, cols]), _dot(rest, r13_s[t, :, cols2])
                pre.append((c11 + r1[:m_rows], c12 + r2[:m_rows],
                            c21 + r1[m_rows:], c22 + r2[m_rows:]))
                yield
            act = [swiglu(gate, up) for gate, up in zip(*pre)]
            for m, x in enumerate(_left_operands(*act) + act[1:3]):
                a2_s[words(m), cols] = _words(x.astype(BF16))

        def store(cols, even, odd):
            for t in range(n):
                store_out(i + t, cols, t * C, even[t * H:(t + 1) * H], odd[t * H:(t + 1) * H])

        if first:
            r2_s[...] = _words(w2_v[:, KS:])
        act = jnp.concatenate(
            [jnp.concatenate([a2_s[words(m), :] for m in pair], axis=1) for pair in ((2, 7), (8, 3))],
            axis=0)
        o = _dot(act, r2_s[...])
        store(slice(KS, D), o[:m_rows], o[m_rows:])
        if last:
            last_copies[2].start()
        yield
        if first:
            right_factors(b2_s, w2_v, F // 2, KS // 2, slice(0, KS // 2))
        p = {}
        for m in (0, 1, 2, 4, 5):
            p[m] = _dot(a2_s[words(m), :], b2_s[m])
            yield
        store(slice(KS // 2, KS), p[2] + p[4], p[0] - p[1] + p[2] + p[5])
        if last:
            last_copies[1].start()
        for m in (3, 6):
            p[m] = _dot(a2_s[words(m), :], b2_s[m])
            yield
        store(slice(0, KS // 2), p[0] + p[3] - p[4] + p[6], p[1] + p[3])
        if last:
            last_copies[0].start()

    for group in start_groups:
        for cp in group:
            cp.start()
        pl.delay(1)

    def start_chunk(i, carry):
        for cp in chunk_copies(i):
            cp.start()
        return i

    zero = jax.lax.fori_loop(3, n_chunks, start_chunk, 0) - (n_chunks - 1)
    zero = zero if OPAQUE else 0

    k_v[0:HALO, :] = jnp.zeros((HALO, D), BF16)
    for m in range(3, n_chunks):
        spec_s[m, :, 256:512] = jnp.zeros((spec_s.shape[1], 256), F32)
    with jax.named_scope("conv0"):
        conv = [conv_chunk(zero + i, i + 1, i) for i in range(3)]
        wait_group(0)
        _emit({"A": forward_chunk(0, True)})
        wait_group(1)
        _emit({"A": forward_chunk(1), "P": conv[0]}, ORDER1)
        wait_group(2)
        _emit({"A": forward_chunk(2), "P": conv[1]}, ORDER1)
        _emit({"P": conv[2]})
    with jax.named_scope("mod"):
        wait_group(3)
        for n in range(3):
            modulation(n)
        _emit({"P": gate_chunk(0), "Q": gate_chunk(1, 1)})
        for i in range(2):
            for r in range(0, H, 16):
                for off, x in residual(i, i, r, 16):
                    x2_s[i * C + off:i * C + off + 16, :] = x
                    gate_s[i, off:off + 16, :] = _layernorm(x)
        for n in range(3, 5):
            wait_group(n + 1)
            modulation(n)
    with jax.named_scope("mix0"):
        for i in range(2):
            for r in range(0, H, 16):
                store_operands([gate_s[i, off:off + 16, :] for off in (r, H + r)], i * H + r)

    n_mac = H // MAC_G * (D // 128)

    def arrivals():
        for n in range(6, 10):
            wait_group(n)
            if n == 9:
                modulation(5)
            yield

    def third_chunk():
        yield from gate_chunk(2, 2)
        yield from mix_chunk(2, 2)

    with jax.named_scope("step0"):
        _emit({"W": arrivals(), "F": ffn_chunk(0, 2, first=True), "P": third_chunk()},
              "".join("W" + "F" * (b - a) for a, b in zip((0, *CUTS), (*CUTS, 13))) + "P" + "PF" * 7)
    out_copy(0).start()
    out_copy(1).start()

    def step(n_terms, i, carry):
        with jax.named_scope("waitc"):
            for cp in chunk_copies(i + 1):
                cp.wait()
        with jax.named_scope("body"):
            _emit({"F": ffn_chunk(i), "P": prepare(i + 1, n_terms)}, _order(*POS, n_mac))
        out_copy(i).start()
        return carry

    jax.lax.fori_loop(2, n_chunks - 1, functools.partial(step, n_chunks), 0)
    with jax.named_scope("last"):
        _emit({"F": ffn_chunk(n_chunks - 1, last=True)})
    with jax.named_scope("outwait"):
        for i in range(n_chunks - 1):
            out_copy(i).wait()
        for cp in last_copies:
            cp.wait()


@jax.jit
def pallas_adaLN_cond__ssm_conv_h3__glu_gated_swiglu__prompt_kernel(
    A_q: jax.Array,
    A_k: jax.Array,
    A_v: jax.Array,
    A_shift_k: jax.Array,
    A_ssm_k: jax.Array,
    A_ssm_D: jax.Array,
    B_x: jax.Array,
    B_w1: jax.Array,
    B_w3: jax.Array,
    B_w2: jax.Array,
    c: jax.Array,
    w_mod: jax.Array,
):
    del B_x
    B, S, D = A_q.shape
    F = B_w1.shape[1]
    ks = A_shift_k.shape[1]
    assert B == 1 and ks == 4 and S % C == 0 and D % 128 == 0 and F % FT == 0
    n_chunks = S // C
    fwd, inv = _dft_matrices()

    vmem = pltpu.VMEM
    scratch = [
        vmem((S + 16, D), BF16),
        vmem((HALO + S + 16, D), BF16),
        vmem((S, D), BF16),
        vmem((n_chunks, D, C), BF16),
        vmem((D, F), BF16), vmem((D, F), BF16), vmem((F, D), BF16),
        vmem((6, D, D), BF16),
        vmem((S, D), BF16),
        vmem((2, 7, KS // 4, F // 2), U32),
        vmem((2, (D - KS) // 2, F), U32),
        vmem((7, F // 4, KS // 2), U32),
        vmem((F // 2, D - KS), U32),
        vmem((ks, D), BF16), vmem((D // 128, 128), BF16), vmem((1, D), BF16),
        vmem(fwd.shape, BF16), vmem(inv.shape, BF16),
        vmem((6, 8, D), F32),
        vmem((2, H // 2, D), U32), vmem((2, H // 2, D), U32),
        vmem((n_chunks + 1, D // 128 * C, 4 * 128), F32),
        vmem((2, C // 2, D), U32),
        vmem((3, C, D), F32),
        vmem((3, C, D), F32),
        vmem((C, D), F32), vmem((2 * C, D), F32),
        vmem((7 * H, KS // 2), U32),
        vmem((2 * H, D - KS), U32),
        vmem((9 * H, F // 2), U32),
        pltpu.SemaphoreType.DMA((n_chunks - 3,)),
        pltpu.SemaphoreType.DMA((9,)),
        pltpu.SemaphoreType.DMA(()),
    ]
    out = pl.pallas_call(
        _kernel,
        out_shape=jax.ShapeDtypeStruct((S, D), A_q.dtype),
        in_specs=[pl.BlockSpec(memory_space=pl.ANY)] * 13,
        out_specs=pl.BlockSpec(memory_space=pl.ANY),
        scratch_shapes=scratch,
        compiler_params=pltpu.CompilerParams(vmem_limit_bytes=100 * 2**20, **FLAGS),
    )(A_q.reshape(S, D), A_k.reshape(S, D), A_v.reshape(S, D), A_shift_k.T, A_ssm_k,
      A_ssm_D.reshape(D // 128, 128), B_w1, B_w3, B_w2, c, w_mod, fwd, inv)
    return out.reshape(B, S, D)
```

```python
import functools

import numpy as np

import jax
import jax.numpy as jnp
import jax.experimental.pallas as pl
import jax.experimental.pallas.tpu as pltpu

C = 256
H = C // 2
HALO = 16
FT = 256
KS = 512
EPS = 1e-5
SER_GATE = (1, 1)
OPAQUE = True
CUTS = (1, 3, 7, 11)
ORDER1 = "A" + "P" * (80) + "AAAP"
PREP_G = 32
GATE_G = 16
MIX_G = 32
FLAGS = {}
POS = (1, 3, 14)
EARLY = ((0, 0),)
F32 = jnp.float32
BF16 = jnp.bfloat16
U32 = jnp.uint32


def _dft_matrices():
    f = np.concatenate([np.arange(0, H, 2), np.arange(1, H, 2)]).astype(np.float64)
    theta = 2.0 * np.pi * (f + 0.5) / (2 * C)
    r = np.arange(H, dtype=np.float64)
    fwd, inv = [], []
    for phase in (0, 1):
        ang = theta[:, None] * (2.0 * r + phase)[None, :]
        m = np.concatenate([np.cos(ang), -np.sin(ang)], axis=0)
        fwd.append(m)
        inv.append(m.reshape(2, H // 8, 8, H).transpose(3, 1, 0, 2).reshape(H, C) / C)
    return np.stack(fwd).astype(BF16), np.stack(inv).astype(BF16)


def lanes(n):
    return slice(n * 128, (n + 1) * 128)


def _words(x):
    return pltpu.bitcast(x, jnp.uint32)


def _halves(w):
    return pltpu.bitcast(w, BF16)


def _to_words(x):
    return _words(x.astype(BF16))


def _interleave(even, odd):
    even, odd = (pltpu.bitcast(x.astype(BF16).astype(F32), U32) for x in (even, odd))
    return _halves((even >> 16) | odd)


def _even(w):
    return pltpu.bitcast(w << 16, F32)


def _odd(w):
    return pltpu.bitcast(w & jnp.uint32(0xFFFF0000), F32)


def _left_operands(a11, a12, a21, a22):
    return [a11 + a22, a21 + a22, a11, a22, a11 + a12, a21 - a11, a12 - a22]


def _right_operands(b11, b12, b21, b22):
    return [b11 + b22, b11, b12 - b22, b21 - b11, b22, b11 + b12, b21 + b22]


def _product_blocks(m):
    return m[0] + m[3] - m[4] + m[6], m[2] + m[4], m[1] + m[3], m[0] - m[1] + m[2] + m[5]


def _dot(a, b):
    return jnp.dot(_halves(a), _halves(b), preferred_element_type=F32)


def _layernorm(x):
    m = jnp.mean(x, axis=-1, keepdims=True)
    d = x - m
    v = jnp.mean(d * d, axis=-1, keepdims=True)
    return d * jax.lax.rsqrt(v + EPS)


def _silu(x):
    hx = 0.5 * x
    return hx * jnp.tanh(hx) + hx


def _order(a, b, c, n_mac):
    order = ["F"] * 15
    for pos, piece in ((c, "P" * (n_mac + 1)), (b, "P"), (a, "PP"), (0, "PP")):
        order.insert(pos, piece)
    return "".join(order)


def _emit(gens, order=""):
    for key in order:
        next(gens[key], None)
    for g in gens.values():
        for _ in g:
            pass


def _kernel(q_hbm, k_hbm, v_hbm, shk_hbm, ssmk_hbm, ssmd_hbm, w1_hbm, w3_hbm, w2_hbm, c_hbm,
            wmod_hbm, fwd_hbm, inv_hbm, out_hbm,
            q_v, k_v, v_v, ssmk_v, w1_v, w3_v, w2_v, wmod_v, out_v, b13_s, r13_s, b2_s, r2_s,
            shk_v, ssmd_v, c_v, fwd_v, inv_v, mod_v,
            ue_s, uo_s, ke_s, ko_s, spec_s, ye_s, yo_s, y_s, gate_s, x2n_s, x2_s, a13_s, hr_s, a2_s,
            sem_in, sem_start, sem_out):
    S, D = v_v.shape
    F = w1_v.shape[1]
    n_chunks = S // C
    PREV = n_chunks

    def aligned(start, size, align):
        return pl.ds(start if isinstance(start, int) else pl.multiple_of(start, align), size)

    def rows(i):
        return aligned(i * C, C, C)

    def chunk_refs(i):
        return [(k_hbm.at[rows(i)], k_v.at[aligned(i * C + HALO, C, HALO)]),
                (v_hbm.at[rows(i)], v_v.at[rows(i)]),
                (ssmk_hbm.at[:, rows(i)], ssmk_v.at[i]),
                (q_hbm.at[rows(i)], q_v.at[rows(i)])]

    def chunk_copies(i):
        return [pltpu.make_async_copy(s, d, sem_in.at[i - 3]) for s, d in chunk_refs(i)]

    def out_copy(i, cols=slice(None)):
        return pltpu.make_async_copy(out_v.at[rows(i), cols], out_hbm.at[rows(i), cols], sem_out)

    last_copies = [out_copy(n_chunks - 1, pl.ds(l, n))
                   for l, n in ((0, KS // 2), (KS // 2, KS // 2), (KS, D - KS))]

    wmod_refs = [(wmod_hbm.at[:, pl.ds(n * D, D)], wmod_v.at[n]) for n in range(6)]
    w13_refs = [(w_hbm.at[:, pl.ds(c0 + j, 128)], w_v.at[:, pl.ds(c0 + j, 128)])
                for j in range(0, F // 2, 128)
                for w_hbm, w_v in ((w1_hbm, w1_v), (w3_hbm, w3_v)) for c0 in (0, F // 2)]
    start_groups = [
        [(shk_hbm, shk_v), (fwd_hbm, fwd_v), (inv_hbm, inv_v), (ssmd_hbm, ssmd_v), (c_hbm, c_v)]
        + chunk_refs(0)[:3],
        chunk_refs(1)[:3],
        chunk_refs(2)[:3],
        wmod_refs[:3] + [chunk_refs(0)[3], chunk_refs(1)[3]],
        wmod_refs[3:4],
        wmod_refs[4:5],
        *(w13_refs[2 * a:2 * b] for a, b in zip((0, *CUTS), CUTS)),
        w13_refs[2 * CUTS[-1]:] + [chunk_refs(2)[3], wmod_refs[5], (w2_hbm, w2_v)],
    ]
    start_groups = [[pltpu.make_async_copy(s, d, sem_start.at[n]) for s, d in group]
                    for n, group in enumerate(start_groups)]

    def wait_group(n):
        for cp in start_groups[n]:
            cp.wait()

    def spectrum(even_ref, odd_ref, slot, off, tap0=None):
        e = jnp.dot(fwd_v[0], _halves(even_ref[...]), preferred_element_type=F32)
        t = jnp.dot(fwd_v[1], _halves(odd_ref[...]), preferred_element_type=F32)
        if tap0 is not None:
            e = jnp.concatenate([e[:H] + tap0, e[H:]], axis=0)
        for n, x in enumerate((e + t, e - t)):
            for l in range(D // 128):
                for part in range(2):
                    spec_s[slot, (2 * l + n) * H:(2 * l + n + 1) * H, lanes(off + part)] = (
                        x[part * H:(part + 1) * H, lanes(l)])

    def chain(ref, val):
        spare = ref.shape[0] - 16
        ref[pl.ds(pl.multiple_of(zero + spare, 16), 16), lanes(0)] = val[-16:, lanes(0)].astype(BF16)

    def ssm_d():
        return jnp.concatenate([ssmd_v[n:n + 1, :] for n in range(D // 128)], axis=1).astype(F32)

    def forward_chunk(i, first=False):
        w = [shk_v[j:j + 1, :].astype(F32) for j in range(4)]
        g = PREP_G
        for r in range(0, H, g):
            base = i * C + 2 * r
            kw = _words(k_v[aligned(base, 2 * g + HALO, HALO), :])
            k0, k1, k2 = kw[8:], pltpu.roll(kw, 1, 0)[8:], pltpu.roll(kw, 2, 0)[8:]
            vw = _words(v_v[aligned(base, 2 * g, 2 * g), :])
            ke, ko, ke1, ko1, ko2 = _even(k0), _odd(k0), _even(k1), _odd(k1), _odd(k2)
            kve = (w[0] * ke + w[1] * ko1 + w[2] * ke1 + w[3] * ko2) * _even(vw)
            kvo = (w[0] * ko + w[1] * ke + w[2] * ko1 + w[3] * ke1) * _odd(vw)
            ue_s[r // 2:(r + g) // 2, :] = _to_words(kve)
            uo_s[r // 2:(r + g) // 2, :] = _to_words(kvo)
        yield
        spectrum(ue_s, uo_s, i, 0)
        yield
        tw = _words(ssmk_v[i].T)
        ke_s[...] = _to_words(_even(tw))
        ko_s[...] = _to_words(_odd(tw))
        yield
        spectrum(ke_s, ko_s, i, 2, ssm_d() if first else None)
        yield

    def conv_chunk(i, n_terms, dst=0):
        first = n_terms == 1
        if isinstance(i, int):
            terms = [(i - m, m) for m in range(n_terms)]
        else:
            terms = [(jnp.maximum(i - m, 0), m) for m in range(n_terms)]
        def products(row, g):
            re = im = None
            for us, ks in terms:
                ur, ui = spec_s[us, row:row + g, lanes(0)], spec_s[us, row:row + g, lanes(1)]
                kr, ki = spec_s[ks, row:row + g, lanes(2)], spec_s[ks, row:row + g, lanes(3)]
                pr, pi = ur * kr - ui * ki, ur * ki + ui * kr
                re, im = (pr, pi) if re is None else (re + pr, im + pi)
            return re, im

        g = 8
        for l in range(D // 128):
            for r in range(0, H, g):
                pr, pi = products(2 * l * H + r, g)
                qr, qi = products((2 * l + 1) * H + r, g)
                for n, (re, im) in enumerate(((pr + qr, pi + qi), (pr - qr, pi - qi))):
                    last_re = spec_s.at[PREV, l * H + r:l * H + r + g, lanes(2 * n)]
                    last_im = spec_s.at[PREV, l * H + r:l * H + r + g, lanes(2 * n + 1)]
                    if first:
                        ore, oim = re, im
                    else:
                        lre, lim = last_re[...], last_im[...]
                        ore, oim = (re - lim, im + lre) if r < H // 2 else (re + lim, im - lre)
                    last_re[...] = re
                    last_im[...] = im
                    (ye_s, yo_s)[n][r:r + g, lanes(l)] = _to_words(
                        jnp.concatenate([ore, oim], axis=0))
                yield
        for n in range(2):
            y_s[dst, n * H:(n + 1) * H, :] = jnp.dot(inv_v[n], _halves((ye_s, yo_s)[n][...]),
                                                 preferred_element_type=F32)
        yield

    def q_rows(i, r, g):
        qw = _words(q_v[aligned(i * C + 2 * r, 2 * g, 2 * g), :])
        return (r, _even(qw)), (H + r, _odd(qw))

    def gate_chunk(i, dst=0):
        sa, ca1, ga = (mod_v[n, 0:1, :] for n in range(3))
        scale, shift = ga * ca1, ga * sa
        g = GATE_G
        for r in range(0, H, g):
            for off, x in q_rows(i, r, g):
                val = _layernorm(x) * scale + shift
                gate_s[dst, off:off + g, :] = val
            if SER_GATE[isinstance(i, int)] and (not isinstance(i, int) or i == 2):
                chain(q_v, val)
        yield

    def residual(i, src, r, g):
        return [(off, x + gate_s[src, off:off + g, :] * y_s[src, off:off + g, :])
                for off, x in q_rows(i, r, g)]

    def store_operands(normed, row):
        sb, cb1 = mod_v[3, 0:1, :], mod_v[4, 0:1, :]
        h2 = [x * cb1 + sb for x in normed]
        lo, hi = row // 2, (row + h2[0].shape[0]) // 2
        blocks = [x[:, l:l + KS // 2] for x in h2 for l in (0, KS // 2)]
        for n, x in enumerate(_left_operands(*blocks)):
            a13_s[n * H + lo:n * H + hi, :] = _to_words(x)
        for n, x in enumerate(h2):
            hr_s[n * H + lo:n * H + hi, :] = _to_words(x[:, KS:])

    def mix_chunk(i, src=0):
        g = MIX_G
        for r in range(0, H, g):
            x2 = residual(i, src, r, g)
            for off, x in x2:
                x2n_s[off:off + g, :] = x
            store_operands([_layernorm(x) for _, x in x2], r)
            if not isinstance(i, int):
                chain(q_v, x2[1][1])
            yield

    def prepare(i, n_terms):
        yield from gate_chunk(i)
        yield from forward_chunk(i)
        yield from conv_chunk(i, n_terms)
        yield from mix_chunk(i)

    def modulation(n):
        cf = c_v[...].astype(F32)
        sc = jnp.broadcast_to(_silu(cf), (16, D)).astype(BF16)
        m = jnp.dot(sc, wmod_v[n], preferred_element_type=F32)[0:8]
        m = 1.0 + m if n in (1, 4) else m
        mod_v[n] = m * {3: 0.5, 4: 0.5, 5: 2.0}.get(n, 1.0)

    def swiglu(gate, up):
        return (gate * jnp.tanh(gate) + gate) * up

    def store_out(i, cols, src, even, odd):
        gb = mod_v[5, 0:1, cols]
        even = x2_s[src:src + H, cols] + gb * even
        odd = x2_s[src + H:src + C, cols] + gb * odd
        out_v[rows(i), cols] = _interleave(even, odd)

    def right_factors(dst, base, src, row, col, cols):
        for r in range(0, row, 16):
            w = [src[r0 + r:r0 + r + 16, c0 + cols.start:c0 + cols.stop]
                 for r0 in (0, row) for c0 in (0, col)]
            for n, x in enumerate(_right_operands(*(x.astype(F32) for x in w))):
                lo = ((base + n) * row + r) // 2
                dst[lo:lo + 8, cols] = (
                    _words(w[0]) if n == 1 else _words(w[3]) if n == 4 else _to_words(x))

    def ffn_chunk(i, n=1, first=False, last=False):
        m_rows = n * H

        def factor(m, size):
            return slice(m * size, (m + 1) * size)

        def words(m):
            return slice(m * H, m * H + m_rows // 2)

        if not first:
            x2_s[0:C, :] = x2n_s[...]
        rest = jnp.concatenate([hr_s[words(0), :], hr_s[words(1), :]], axis=0)
        ft = 128 if first else FT
        early = {}
        if not (first or last):
            for t, j in EARLY:
                early[t, j] = [_dot(rest, r13_s[t, :, c0 + j:c0 + j + ft]) for c0 in (0, F // 2)]
            yield
        for j in range(0, F // 2, ft):
            cols, cols2 = slice(j, j + ft), slice(F // 2 + j, F // 2 + j + ft)
            pre = []
            for t, w_v in enumerate((w1_v, w3_v)):
                if first:
                    r13_s[t, :, cols] = _words(w_v[KS:, cols])
                    r13_s[t, :, cols2] = _words(w_v[KS:, cols2])
                    right_factors(b13_s, 7 * t, w_v, KS // 2, F // 2, cols)
                c11, c12, c21, c22 = _product_blocks(
                    [_dot(a13_s[words(m), :], b13_s[factor(7 * t + m, KS // 4), cols])
                     for m in range(7)])
                r1, r2 = early.get((t, j)) or (
                    _dot(rest, r13_s[t, :, cols]), _dot(rest, r13_s[t, :, cols2]))
                pre.append((c11 + r1[:m_rows], c12 + r2[:m_rows],
                            c21 + r1[m_rows:], c22 + r2[m_rows:]))
                yield
            act = [swiglu(gate, up) for gate, up in zip(*pre)]
            for m, x in enumerate(_left_operands(*act) + act[1:3]):
                a2_s[words(m), cols] = _to_words(x)

        def store(cols, even, odd):
            for t in range(n):
                store_out(i + t, cols, t * C, even[t * H:(t + 1) * H], odd[t * H:(t + 1) * H])

        if first:
            r2_s[...] = _words(w2_v[:, KS:])
        act = jnp.concatenate(
            [jnp.concatenate([a2_s[words(m), :] for m in pair], axis=1) for pair in ((2, 7), (8, 3))],
            axis=0)
        o = _dot(act, r2_s[...])
        store(slice(KS, D), o[:m_rows], o[m_rows:])
        if last:
            last_copies[2].start()
        yield
        if first:
            right_factors(b2_s, 0, w2_v, F // 2, KS // 2, slice(0, KS // 2))
        p = {}
        for m in (0, 1, 2, 4, 5):
            p[m] = _dot(a2_s[words(m), :], b2_s[factor(m, F // 4), :])
            yield
        store(slice(KS // 2, KS), p[2] + p[4], p[0] - p[1] + p[2] + p[5])
        if last:
            last_copies[1].start()
        for m in (3, 6):
            p[m] = _dot(a2_s[words(m), :], b2_s[factor(m, F // 4), :])
            yield
        store(slice(0, KS // 2), p[0] + p[3] - p[4] + p[6], p[1] + p[3])
        if last:
            last_copies[0].start()

    for group in start_groups:
        for cp in group:
            cp.start()
        pl.delay(1)

    def start_chunk(i, carry):
        for cp in chunk_copies(i):
            cp.start()
        return i

    zero = jax.lax.fori_loop(3, n_chunks, start_chunk, 0) - (n_chunks - 1)
    zero = zero if OPAQUE else 0

    k_v[0:HALO, :] = jnp.zeros((HALO, D), BF16)
    for m in range(3, n_chunks):
        spec_s[m, :, 256:512] = jnp.zeros((spec_s.shape[1], 256), F32)
    with jax.named_scope("conv0"):
        conv = [conv_chunk(zero + i, i + 1, i) for i in range(3)]
        wait_group(0)
        _emit({"A": forward_chunk(0, True)})
        wait_group(1)
        _emit({"A": forward_chunk(1), "P": conv[0]}, ORDER1)
        wait_group(2)
        _emit({"A": forward_chunk(2), "P": conv[1]}, ORDER1)
        _emit({"P": conv[2]})
    with jax.named_scope("mod"):
        wait_group(3)
        for n in range(3):
            modulation(n)
        _emit({"P": gate_chunk(0), "Q": gate_chunk(1, 1)})
        for i in range(2):
            for r in range(0, H, 16):
                for off, x in residual(i, i, r, 16):
                    x2_s[i * C + off:i * C + off + 16, :] = x
                    gate_s[i, off:off + 16, :] = _layernorm(x)
        for n in range(3, 5):
            wait_group(n + 1)
            modulation(n)
    with jax.named_scope("mix0"):
        for i in range(2):
            for r in range(0, H, 16):
                store_operands([gate_s[i, off:off + 16, :] for off in (r, H + r)], i * H + r)

    n_mac = H // 8 * (D // 128)

    def arrivals():
        for n in range(6, len(start_groups)):
            wait_group(n)
            if n == len(start_groups) - 1:
                modulation(5)
            yield

    def third_chunk():
        yield from gate_chunk(2, 2)
        yield from mix_chunk(2, 2)

    with jax.named_scope("step0"):
        _emit({"W": arrivals(), "F": ffn_chunk(0, 2, first=True), "P": third_chunk()},
              "".join("W" + "F" * (b - a) for a, b in zip((0, *CUTS), (*CUTS, 13))) + "P" + "PF" * 7)
    out_copy(0).start()
    out_copy(1).start()

    def step(n_terms, i, carry):
        with jax.named_scope("waitc"):
            for cp in chunk_copies(i + 1):
                cp.wait()
        with jax.named_scope("body"):
            _emit({"F": ffn_chunk(i), "P": prepare(i + 1, n_terms)}, _order(*POS, n_mac))
        out_copy(i).start()
        return carry

    jax.lax.fori_loop(2, n_chunks - 1, functools.partial(step, n_chunks), 0)
    with jax.named_scope("last"):
        _emit({"F": ffn_chunk(n_chunks - 1, last=True)})
    with jax.named_scope("outwait"):
        for i in range(n_chunks - 1):
            out_copy(i).wait()
        for cp in last_copies:
            cp.wait()


@jax.jit
def pallas_adaLN_cond__ssm_conv_h3__glu_gated_swiglu__prompt_kernel(
    A_q: jax.Array,
    A_k: jax.Array,
    A_v: jax.Array,
    A_shift_k: jax.Array,
    A_ssm_k: jax.Array,
    A_ssm_D: jax.Array,
    B_x: jax.Array,
    B_w1: jax.Array,
    B_w3: jax.Array,
    B_w2: jax.Array,
    c: jax.Array,
    w_mod: jax.Array,
):
    del B_x
    B, S, D = A_q.shape
    F = B_w1.shape[1]
    ks = A_shift_k.shape[1]
    assert B == 1 and ks == 4 and S % C == 0 and D % 128 == 0 and F % FT == 0
    n_chunks = S // C
    fwd, inv = _dft_matrices()

    vmem = pltpu.VMEM
    scratch = [
        vmem((S + 16, D), BF16),
        vmem((HALO + S, D), BF16),
        vmem((S, D), BF16),
        vmem((n_chunks, D, C), BF16),
        vmem((D, F), BF16), vmem((D, F), BF16), vmem((F, D), BF16),
        vmem((6, D, D), BF16),
        vmem((S, D), BF16),
        vmem((14 * KS // 4, F // 2), U32),
        vmem((2, (D - KS) // 2, F), U32),
        vmem((7 * F // 4, KS // 2), U32),
        vmem((F // 2, D - KS), U32),
        vmem((ks, D), BF16), vmem((D // 128, 128), BF16), vmem((1, D), BF16),
        vmem(fwd.shape, BF16), vmem(inv.shape, BF16),
        vmem((6, 8, D), F32),
        *[vmem((H // 2, D), U32)] * 4,
        vmem((n_chunks + 1, D // 128 * C, 4 * 128), F32),
        *[vmem((H, D), U32)] * 2,
        vmem((3, C, D), F32),
        vmem((3, C, D), F32),
        vmem((C, D), F32), vmem((2 * C, D), F32),
        vmem((7 * H, KS // 2), U32),
        vmem((2 * H, D - KS), U32),
        vmem((9 * H, F // 2), U32),
        pltpu.SemaphoreType.DMA((n_chunks - 3,)),
        pltpu.SemaphoreType.DMA((7 + len(CUTS),)),
        pltpu.SemaphoreType.DMA(()),
    ]
    out = pl.pallas_call(
        _kernel,
        out_shape=jax.ShapeDtypeStruct((S, D), A_q.dtype),
        in_specs=[pl.BlockSpec(memory_space=pl.ANY)] * 13,
        out_specs=pl.BlockSpec(memory_space=pl.ANY),
        scratch_shapes=scratch,
        compiler_params=pltpu.CompilerParams(vmem_limit_bytes=100 * 2**20, **FLAGS),
    )(A_q.reshape(S, D), A_k.reshape(S, D), A_v.reshape(S, D), A_shift_k.T, A_ssm_k,
      A_ssm_D.reshape(D // 128, 128), B_w1, B_w3, B_w2, c, w_mod, fwd, inv)
    return out.reshape(B, S, D)
```

```python
import numpy as np

import jax
import jax.numpy as jnp
import jax.experimental.pallas as pl
import jax.experimental.pallas.tpu as pltpu

C = 256
H = C // 2
HALO = 16
KS = 512
EPS = 1e-5
CUTS = (1, 3, 7, 11)
F32 = jnp.float32
BF16 = jnp.bfloat16
U32 = jnp.uint32


def _dft_matrices():
    f = np.concatenate([np.arange(0, H, 2), np.arange(1, H, 2)]).astype(np.float64)
    theta = 2.0 * np.pi * (f + 0.5) / (2 * C)
    r = np.arange(H, dtype=np.float64)
    fwd, inv = [], []
    for phase in (0, 1):
        ang = theta[:, None] * (2.0 * r + phase)[None, :]
        m = np.concatenate([np.cos(ang), -np.sin(ang)], axis=0)
        fwd.append(m)
        inv.append(m.reshape(2, H // 8, 8, H).transpose(3, 1, 0, 2).reshape(H, C) / C)
    return np.stack(fwd).astype(BF16), np.stack(inv).astype(BF16)


def _lanes(n):
    return slice(n * 128, (n + 1) * 128)


def _words(x):
    return pltpu.bitcast(x, U32)


def _halves(w):
    return pltpu.bitcast(w, BF16)


def _to_words(x):
    return _words(x.astype(BF16))


def _interleave(even, odd):
    even, odd = (pltpu.bitcast(x.astype(BF16).astype(F32), U32) for x in (even, odd))
    return _halves((even >> 16) | odd)


def _even(w):
    return pltpu.bitcast(w << 16, F32)


def _odd(w):
    return pltpu.bitcast(w & U32(0xFFFF0000), F32)


def _left_operands(a11, a12, a21, a22):
    return [a11 + a22, a21 + a22, a11, a22, a11 + a12, a21 - a11, a12 - a22]


def _right_operands(b11, b12, b21, b22):
    return [b11 + b22, b11, b12 - b22, b21 - b11, b22, b11 + b12, b21 + b22]


def _product_blocks(m):
    return m[0] + m[3] - m[4] + m[6], m[2] + m[4], m[1] + m[3], m[0] - m[1] + m[2] + m[5]


def _dot(a, b):
    return jnp.dot(_halves(a), _halves(b), preferred_element_type=F32)


def _layernorm(x):
    m = jnp.mean(x, axis=-1, keepdims=True)
    d = x - m
    v = jnp.mean(d * d, axis=-1, keepdims=True)
    return d * jax.lax.rsqrt(v + EPS)


def _silu(x):
    hx = 0.5 * x
    return hx * jnp.tanh(hx) + hx


def _emit(gens, order=""):
    for key in order:
        next(gens[key], None)
    for g in gens.values():
        for _ in g:
            pass


def _kernel(q_hbm, k_hbm, v_hbm, shk_hbm, ssmk_hbm, ssmd_hbm, w1_hbm, w3_hbm, w2_hbm, c_hbm,
            wmod_hbm, fwd_hbm, inv_hbm, out_hbm,
            q_v, k_v, v_v, ssmk_v, w1_v, w3_v, w2_v, wmod_v, out_v, b13_s, r13_s, b2_s, r2_s,
            shk_v, ssmd_v, c_v, fwd_v, inv_v, mod_v,
            ue_s, uo_s, ke_s, ko_s, spec_s, ye_s, yo_s, y_s, gate_s, x2n_s, x2_s, a13_s, hr_s, a2_s,
            sem_in, sem_start, sem_out):
    S, D = v_v.shape
    F = w1_v.shape[1]
    n_chunks = S // C
    prev = n_chunks
    n_mac = H // 8 * (D // 128)

    def aligned(start, size, align):
        return pl.ds(start if isinstance(start, int) else pl.multiple_of(start, align), size)

    def rows(i):
        return aligned(i * C, C, C)

    def chunk_refs(i):
        return [(k_hbm.at[rows(i)], k_v.at[aligned(i * C + HALO, C, HALO)]),
                (v_hbm.at[rows(i)], v_v.at[rows(i)]),
                (ssmk_hbm.at[:, rows(i)], ssmk_v.at[i]),
                (q_hbm.at[rows(i)], q_v.at[rows(i)])]

    def chunk_copies(i):
        return [pltpu.make_async_copy(s, d, sem_in.at[i - 3]) for s, d in chunk_refs(i)]

    def out_copy(i, cols=slice(None)):
        return pltpu.make_async_copy(out_v.at[rows(i), cols], out_hbm.at[rows(i), cols], sem_out)

    last_copies = [out_copy(n_chunks - 1, pl.ds(l, n))
                   for l, n in ((0, KS // 2), (KS // 2, KS // 2), (KS, D - KS))]

    wmod_refs = [(wmod_hbm.at[:, pl.ds(n * D, D)], wmod_v.at[n]) for n in range(6)]
    w13_refs = [(w_hbm.at[:, pl.ds(c0 + j, 128)], w_v.at[:, pl.ds(c0 + j, 128)])
                for j in range(0, F // 2, 128)
                for w_hbm, w_v in ((w1_hbm, w1_v), (w3_hbm, w3_v)) for c0 in (0, F // 2)]
    start_groups = [
        [(shk_hbm, shk_v), (fwd_hbm, fwd_v), (inv_hbm, inv_v), (ssmd_hbm, ssmd_v), (c_hbm, c_v)]
        + chunk_refs(0)[:3],
        chunk_refs(1)[:3],
        chunk_refs(2)[:3],
        wmod_refs[:3] + [chunk_refs(0)[3], chunk_refs(1)[3]],
        wmod_refs[3:4],
        wmod_refs[4:5],
        *(w13_refs[2 * a:2 * b] for a, b in zip((0, *CUTS), CUTS)),
        w13_refs[2 * CUTS[-1]:] + [chunk_refs(2)[3], wmod_refs[5], (w2_hbm, w2_v)],
    ]
    start_groups = [[pltpu.make_async_copy(s, d, sem_start.at[n]) for s, d in group]
                    for n, group in enumerate(start_groups)]

    def wait_group(n):
        for cp in start_groups[n]:
            cp.wait()

    def spectrum(even_ref, odd_ref, slot, off, tap0=None):
        e = jnp.dot(fwd_v[0], _halves(even_ref[...]), preferred_element_type=F32)
        t = jnp.dot(fwd_v[1], _halves(odd_ref[...]), preferred_element_type=F32)
        if tap0 is not None:
            e = jnp.concatenate([e[:H] + tap0, e[H:]], axis=0)
        for n, x in enumerate((e + t, e - t)):
            for l in range(D // 128):
                for part in range(2):
                    spec_s[slot, (2 * l + n) * H:(2 * l + n + 1) * H, _lanes(off + part)] = (
                        x[part * H:(part + 1) * H, _lanes(l)])

    def chain(ref, val):
        spare = ref.shape[0] - 16
        at = pl.ds(pl.multiple_of(zero + spare, 16), 16)
        ref[at, _lanes(0)] = val[-16:, _lanes(0)].astype(BF16)

    def ssm_d():
        tiles = [ssmd_v[n:n + 1, :] for n in range(D // 128)]
        return jnp.concatenate(tiles, axis=1).astype(F32)

    def forward_chunk(i, first=False):
        w = [shk_v[j:j + 1, :].astype(F32) for j in range(4)]
        g = 32
        for r in range(0, H, g):
            base = i * C + 2 * r
            kw = _words(k_v[aligned(base, 2 * g + HALO, HALO), :])
            k0, k1, k2 = kw[8:], pltpu.roll(kw, 1, 0)[8:], pltpu.roll(kw, 2, 0)[8:]
            vw = _words(v_v[aligned(base, 2 * g, 2 * g), :])
            ke, ko, ke1, ko1, ko2 = _even(k0), _odd(k0), _even(k1), _odd(k1), _odd(k2)
            kve = (w[0] * ke + w[1] * ko1 + w[2] * ke1 + w[3] * ko2) * _even(vw)
            kvo = (w[0] * ko + w[1] * ke + w[2] * ko1 + w[3] * ke1) * _odd(vw)
            ue_s[r // 2:(r + g) // 2, :] = _to_words(kve)
            uo_s[r // 2:(r + g) // 2, :] = _to_words(kvo)
        yield
        spectrum(ue_s, uo_s, i, 0)
        yield
        tw = _words(ssmk_v[i].T)
        ke_s[...] = _to_words(_even(tw))
        ko_s[...] = _to_words(_odd(tw))
        yield
        spectrum(ke_s, ko_s, i, 2, ssm_d() if first else None)
        yield

    def conv_chunk(i, n_terms, dst=0):
        first = n_terms == 1
        terms = [(jnp.maximum(i - m, 0), m) for m in range(n_terms)]

        def products(row, g):
            re = im = None
            for us, ks in terms:
                ur, ui = spec_s[us, row:row + g, _lanes(0)], spec_s[us, row:row + g, _lanes(1)]
                kr, ki = spec_s[ks, row:row + g, _lanes(2)], spec_s[ks, row:row + g, _lanes(3)]
                pr, pi = ur * kr - ui * ki, ur * ki + ui * kr
                re, im = (pr, pi) if re is None else (re + pr, im + pi)
            return re, im

        g = 8
        for l in range(D // 128):
            for r in range(0, H, g):
                pr, pi = products(2 * l * H + r, g)
                qr, qi = products((2 * l + 1) * H + r, g)
                for n, (re, im) in enumerate(((pr + qr, pi + qi), (pr - qr, pi - qi))):
                    last_re = spec_s.at[prev, l * H + r:l * H + r + g, _lanes(2 * n)]
                    last_im = spec_s.at[prev, l * H + r:l * H + r + g, _lanes(2 * n + 1)]
                    if first:
                        ore, oim = re, im
                    else:
                        lre, lim = last_re[...], last_im[...]
                        ore, oim = (re - lim, im + lre) if r < H // 2 else (re + lim, im - lre)
                    last_re[...] = re
                    last_im[...] = im
                    (ye_s, yo_s)[n][r:r + g, _lanes(l)] = _to_words(
                        jnp.concatenate([ore, oim], axis=0))
                yield
        for n in range(2):
            y_s[dst, n * H:(n + 1) * H, :] = jnp.dot(
                inv_v[n], _halves((ye_s, yo_s)[n][...]), preferred_element_type=F32)
        yield

    def q_rows(i, r, g):
        qw = _words(q_v[aligned(i * C + 2 * r, 2 * g, 2 * g), :])
        return (r, _even(qw)), (H + r, _odd(qw))

    def gate_chunk(i, dst=0, chained=True):
        sa, ca1, ga = (mod_v[n, 0:1, :] for n in range(3))
        scale, shift = ga * ca1, ga * sa
        g = 16
        for r in range(0, H, g):
            for off, x in q_rows(i, r, g):
                val = _layernorm(x) * scale + shift
                gate_s[dst, off:off + g, :] = val
            if chained:
                chain(q_v, val)
        yield

    def residual(i, src, r, g):
        return [(off, x + gate_s[src, off:off + g, :] * y_s[src, off:off + g, :])
                for off, x in q_rows(i, r, g)]

    def store_operands(normed, row):
        sb, cb1 = mod_v[3, 0:1, :], mod_v[4, 0:1, :]
        h2 = [x * cb1 + sb for x in normed]
        lo, hi = row // 2, (row + h2[0].shape[0]) // 2
        blocks = [x[:, l:l + KS // 2] for x in h2 for l in (0, KS // 2)]
        for n, x in enumerate(_left_operands(*blocks)):
            a13_s[n * H + lo:n * H + hi, :] = _to_words(x)
        for n, x in enumerate(h2):
            hr_s[n * H + lo:n * H + hi, :] = _to_words(x[:, KS:])

    def mix_chunk(i, src=0, chained=True):
        g = 32
        for r in range(0, H, g):
            x2 = residual(i, src, r, g)
            for off, x in x2:
                x2n_s[off:off + g, :] = x
            store_operands([_layernorm(x) for _, x in x2], r)
            if chained:
                chain(q_v, x2[1][1])
            yield

    def prepare(i, n_terms):
        yield from gate_chunk(i)
        yield from forward_chunk(i)
        yield from conv_chunk(i, n_terms)
        yield from mix_chunk(i)

    def modulation(n):
        cf = c_v[...].astype(F32)
        sc = jnp.broadcast_to(_silu(cf), (16, D)).astype(BF16)
        m = jnp.dot(sc, wmod_v[n], preferred_element_type=F32)[0:8]
        m = 1.0 + m if n in (1, 4) else m
        mod_v[n] = m * {3: 0.5, 4: 0.5, 5: 2.0}.get(n, 1.0)

    def swiglu(gate, up):
        return (gate * jnp.tanh(gate) + gate) * up

    def store_out(i, cols, src, even, odd):
        gb = mod_v[5, 0:1, cols]
        even = x2_s[src:src + H, cols] + gb * even
        odd = x2_s[src + H:src + C, cols] + gb * odd
        out_v[rows(i), cols] = _interleave(even, odd)

    def right_factors(dst, base, src, row, col, cols):
        for r in range(0, row, 16):
            w = [src[r0 + r:r0 + r + 16, c0 + cols.start:c0 + cols.stop]
                 for r0 in (0, row) for c0 in (0, col)]
            for n, x in enumerate(_right_operands(*(x.astype(F32) for x in w))):
                lo = ((base + n) * row + r) // 2
                dst[lo:lo + 8, cols] = (
                    _words(w[0]) if n == 1 else _words(w[3]) if n == 4 else _to_words(x))

    def ffn_chunk(i, n=1, first=False, last=False):
        m_rows = n * H

        def factor(m, size):
            return slice(m * size, (m + 1) * size)

        def words(m):
            return slice(m * H, m * H + m_rows // 2)

        if not first:
            x2_s[0:C, :] = x2n_s[...]
        rest = jnp.concatenate([hr_s[words(0), :], hr_s[words(1), :]], axis=0)
        ft = 128 if first else 256
        early = None
        if not (first or last):
            early = [_dot(rest, r13_s[0, :, c0:c0 + ft]) for c0 in (0, F // 2)]
            yield
        for j in range(0, F // 2, ft):
            cols, cols2 = slice(j, j + ft), slice(F // 2 + j, F // 2 + j + ft)
            pre = []
            for t, w_v in enumerate((w1_v, w3_v)):
                if first:
                    r13_s[t, :, cols] = _words(w_v[KS:, cols])
                    r13_s[t, :, cols2] = _words(w_v[KS:, cols2])
                    right_factors(b13_s, 7 * t, w_v, KS // 2, F // 2, cols)
                c11, c12, c21, c22 = _product_blocks(
                    [_dot(a13_s[words(m), :], b13_s[factor(7 * t + m, KS // 4), cols])
                     for m in range(7)])
                if early is not None and t == j == 0:
                    r1, r2 = early
                else:
                    r1, r2 = _dot(rest, r13_s[t, :, cols]), _dot(rest, r13_s[t, :, cols2])
                pre.append((c11 + r1[:m_rows], c12 + r2[:m_rows],
                            c21 + r1[m_rows:], c22 + r2[m_rows:]))
                yield
            act = [swiglu(gate, up) for gate, up in zip(*pre)]
            for m, x in enumerate(_left_operands(*act) + act[1:3]):
                a2_s[words(m), cols] = _to_words(x)

        def store(cols, even, odd):
            for t in range(n):
                store_out(i + t, cols, t * C, even[t * H:(t + 1) * H], odd[t * H:(t + 1) * H])

        if first:
            r2_s[...] = _words(w2_v[:, KS:])
        act = jnp.concatenate(
            [jnp.concatenate([a2_s[words(m), :] for m in pair], axis=1)
             for pair in ((2, 7), (8, 3))], axis=0)
        o = _dot(act, r2_s[...])
        store(slice(KS, D), o[:m_rows], o[m_rows:])
        if last:
            last_copies[2].start()
        yield
        if first:
            right_factors(b2_s, 0, w2_v, F // 2, KS // 2, slice(0, KS // 2))
        p = {}
        for m in (0, 1, 2, 4, 5):
            p[m] = _dot(a2_s[words(m), :], b2_s[factor(m, F // 4), :])
            yield
        store(slice(KS // 2, KS), p[2] + p[4], p[0] - p[1] + p[2] + p[5])
        if last:
            last_copies[1].start()
        for m in (3, 6):
            p[m] = _dot(a2_s[words(m), :], b2_s[factor(m, F // 4), :])
            yield
        store(slice(0, KS // 2), p[0] + p[3] - p[4] + p[6], p[1] + p[3])
        if last:
            last_copies[0].start()

    for group in start_groups:
        for cp in group:
            cp.start()
        pl.delay(1)

    def start_chunk(i, carry):
        for cp in chunk_copies(i):
            cp.start()
        return i

    zero = jax.lax.fori_loop(3, n_chunks, start_chunk, 0) - (n_chunks - 1)

    k_v[0:HALO, :] = jnp.zeros((HALO, D), BF16)
    for m in range(3, n_chunks):
        spec_s[m, :, 256:512] = jnp.zeros((spec_s.shape[1], 256), F32)
    conv = [conv_chunk(zero + i, i + 1, i) for i in range(3)]
    order = "A" + "P" * n_mac + "AAAP"
    wait_group(0)
    _emit({"A": forward_chunk(0, True)})
    wait_group(1)
    _emit({"A": forward_chunk(1), "P": conv[0]}, order)
    wait_group(2)
    _emit({"A": forward_chunk(2), "P": conv[1]}, order)
    _emit({"P": conv[2]})
    wait_group(3)
    for n in range(3):
        modulation(n)
    _emit({"P": gate_chunk(0, 0, False), "Q": gate_chunk(1, 1, False)})
    for i in range(2):
        for r in range(0, H, 16):
            for off, x in residual(i, i, r, 16):
                x2_s[i * C + off:i * C + off + 16, :] = x
                gate_s[i, off:off + 16, :] = _layernorm(x)
    for n in range(3, 5):
        wait_group(n + 1)
        modulation(n)
    for i in range(2):
        for r in range(0, H, 16):
            store_operands([gate_s[i, off:off + 16, :] for off in (r, H + r)], i * H + r)

    def arrivals():
        for n in range(6, len(start_groups)):
            wait_group(n)
            if n == len(start_groups) - 1:
                modulation(5)
            yield

    def third_chunk():
        yield from gate_chunk(2, 2)
        yield from mix_chunk(2, 2, False)

    _emit({"W": arrivals(), "F": ffn_chunk(0, 2, first=True), "P": third_chunk()},
          "".join("W" + "F" * (b - a) for a, b in zip((0, *CUTS), (*CUTS, 13))) + "P" + "PF" * 7)
    out_copy(0).start()
    out_copy(1).start()

    def step(i, carry):
        for cp in chunk_copies(i + 1):
            cp.wait()
        _emit({"F": ffn_chunk(i), "P": prepare(i + 1, n_chunks)},
              "PPF" "PPFF" "P" + "F" * 11 + "P" * (n_mac + 1))
        out_copy(i).start()
        return carry

    jax.lax.fori_loop(2, n_chunks - 1, step, 0)
    _emit({"F": ffn_chunk(n_chunks - 1, last=True)})
    for i in range(n_chunks - 1):
        out_copy(i).wait()
    for cp in last_copies:
        cp.wait()


@jax.jit
def pallas_adaLN_cond__ssm_conv_h3__glu_gated_swiglu__prompt_kernel(
    A_q: jax.Array,
    A_k: jax.Array,
    A_v: jax.Array,
    A_shift_k: jax.Array,
    A_ssm_k: jax.Array,
    A_ssm_D: jax.Array,
    B_x: jax.Array,
    B_w1: jax.Array,
    B_w3: jax.Array,
    B_w2: jax.Array,
    c: jax.Array,
    w_mod: jax.Array,
):
    del B_x
    B, S, D = A_q.shape
    F = B_w1.shape[1]
    ks = A_shift_k.shape[1]
    assert B == 1 and ks == 4 and S % C == 0 and D % 128 == 0 and F % 512 == 0
    n_chunks = S // C
    fwd, inv = _dft_matrices()

    vmem = pltpu.VMEM
    scratch = [
        vmem((S + 16, D), BF16),
        vmem((HALO + S, D), BF16),
        vmem((S, D), BF16),
        vmem((n_chunks, D, C), BF16),
        vmem((D, F), BF16), vmem((D, F), BF16), vmem((F, D), BF16),
        vmem((6, D, D), BF16),
        vmem((S, D), BF16),
        vmem((14 * KS // 4, F // 2), U32),
        vmem((2, (D - KS) // 2, F), U32),
        vmem((7 * F // 4, KS // 2), U32),
        vmem((F // 2, D - KS), U32),
        vmem((ks, D), BF16), vmem((D // 128, 128), BF16), vmem((1, D), BF16),
        vmem(fwd.shape, BF16), vmem(inv.shape, BF16),
        vmem((6, 8, D), F32),
        *[vmem((H // 2, D), U32)] * 4,
        vmem((n_chunks + 1, D // 128 * C, 4 * 128), F32),
        *[vmem((H, D), U32)] * 2,
        vmem((3, C, D), F32),
        vmem((3, C, D), F32),
        vmem((C, D), F32), vmem((2 * C, D), F32),
        vmem((7 * H, KS // 2), U32),
        vmem((2 * H, D - KS), U32),
        vmem((9 * H, F // 2), U32),
        pltpu.SemaphoreType.DMA((n_chunks - 3,)),
        pltpu.SemaphoreType.DMA((7 + len(CUTS),)),
        pltpu.SemaphoreType.DMA(()),
    ]
    out = pl.pallas_call(
        _kernel,
        out_shape=jax.ShapeDtypeStruct((S, D), A_q.dtype),
        in_specs=[pl.BlockSpec(memory_space=pl.ANY)] * 13,
        out_specs=pl.BlockSpec(memory_space=pl.ANY),
        scratch_shapes=scratch,
        compiler_params=pltpu.CompilerParams(vmem_limit_bytes=100 * 2**20),
    )(A_q.reshape(S, D), A_k.reshape(S, D), A_v.reshape(S, D), A_shift_k.T, A_ssm_k,
      A_ssm_D.reshape(D // 128, 128), B_w1, B_w3, B_w2, c, w_mod, fwd, inv)
    return out.reshape(B, S, D)
```

```python
import numpy as np

import jax
import jax.numpy as jnp
import jax.experimental.pallas as pl
import jax.experimental.pallas.tpu as pltpu

C = 256
H = C // 2
HALO = 16
KS = 512
EPS = 1e-5
CUTS = (1, 3, 7, 11)
F32 = jnp.float32
BF16 = jnp.bfloat16
U32 = jnp.uint32


def _dft_matrices():
    f = np.concatenate([np.arange(0, H, 2), np.arange(1, H, 2)]).astype(np.float64)
    theta = 2.0 * np.pi * (f + 0.5) / (2 * C)
    r = np.arange(H, dtype=np.float64)
    ang = np.stack([theta[:, None] * (2.0 * r + phase)[None, :] for phase in (0, 1)])
    return np.concatenate([np.cos(ang), -np.sin(ang)], axis=1).astype(BF16)


def _lanes(n):
    return slice(n * 128, (n + 1) * 128)


def _words(x):
    return pltpu.bitcast(x, U32)


def _halves(w):
    return pltpu.bitcast(w, BF16)


def _to_words(x):
    return _words(x.astype(BF16))


def _interleave(even, odd):
    even, odd = (pltpu.bitcast(x.astype(BF16).astype(F32), U32) for x in (even, odd))
    return _halves((even >> 16) | odd)


def _even(w):
    return pltpu.bitcast(w << 16, F32)


def _odd(w):
    return pltpu.bitcast(w & U32(0xFFFF0000), F32)


def _left_operands(a11, a12, a21, a22):
    return [a11 + a22, a21 + a22, a11, a22, a11 + a12, a21 - a11, a12 - a22]


def _right_operands(b11, b12, b21, b22):
    return [b11 + b22, b11, b12 - b22, b21 - b11, b22, b11 + b12, b21 + b22]


def _product_blocks(m):
    return m[0] + m[3] - m[4] + m[6], m[2] + m[4], m[1] + m[3], m[0] - m[1] + m[2] + m[5]


def _dot(a, b):
    return jnp.dot(_halves(a), _halves(b), preferred_element_type=F32)


def _layernorm(x):
    m = jnp.mean(x, axis=-1, keepdims=True)
    d = x - m
    v = jnp.mean(d * d, axis=-1, keepdims=True)
    return d * jax.lax.rsqrt(v + EPS)


def _silu(x):
    hx = 0.5 * x
    return hx * jnp.tanh(hx) + hx


def _emit(gens, order=""):
    for key in order:
        next(gens[key], None)
    for g in gens.values():
        for _ in g:
            pass


def _kernel(q_hbm, k_hbm, v_hbm, shk_hbm, ssmk_hbm, ssmd_hbm, w1_hbm, w3_hbm, w2_hbm, c_hbm,
            wmod_hbm, fwd_hbm, out_hbm,
            q_v, k_v, v_v, ssmk_v, w1_v, w3_v, w2_v, wmod_v, out_v, b13_s, r13_s, b2_s, r2_s,
            shk_v, ssmd_v, c_v, fwd_v, inv_v, mod_v,
            ue_s, uo_s, ke_s, ko_s, spec_s, ye_s, yo_s, y_s, gate_s, x2n_s, x2_s, a13_s, hr_s, a2_s,
            sem_in, sem_start, sem_out):
    S, D = v_v.shape
    F = w1_v.shape[1]
    n_chunks = S // C
    prev = n_chunks
    n_mac = H // 8 * (D // 128)

    def aligned(start, size, align):
        return pl.ds(start if isinstance(start, int) else pl.multiple_of(start, align), size)

    def rows(i):
        return aligned(i * C, C, C)

    def chunk_refs(i):
        return [(k_hbm.at[rows(i)], k_v.at[aligned(i * C + HALO, C, HALO)]),
                (v_hbm.at[rows(i)], v_v.at[rows(i)]),
                (ssmk_hbm.at[:, rows(i)], ssmk_v.at[i]),
                (q_hbm.at[rows(i)], q_v.at[rows(i)])]

    def chunk_copies(i):
        return [pltpu.make_async_copy(s, d, sem_in.at[i - 3]) for s, d in chunk_refs(i)]

    def out_copy(i, cols=slice(None)):
        return pltpu.make_async_copy(out_v.at[rows(i), cols], out_hbm.at[rows(i), cols], sem_out)

    last_copies = [out_copy(n_chunks - 1, pl.ds(l, n))
                   for l, n in ((0, KS // 2), (KS // 2, KS // 2), (KS, D - KS))]

    wmod_refs = [(wmod_hbm.at[:, pl.ds(n * D, D)], wmod_v.at[n]) for n in range(6)]
    w13_refs = [(w_hbm.at[:, pl.ds(c0 + j, 128)], w_v.at[:, pl.ds(c0 + j, 128)])
                for j in range(0, F // 2, 128)
                for w_hbm, w_v in ((w1_hbm, w1_v), (w3_hbm, w3_v)) for c0 in (0, F // 2)]
    start_groups = [
        [(fwd_hbm, fwd_v)],
        [(shk_hbm, shk_v), (ssmd_hbm, ssmd_v), (c_hbm, c_v)] + chunk_refs(0)[:3],
        chunk_refs(1)[:3],
        chunk_refs(2)[:3],
        wmod_refs[:3] + [chunk_refs(0)[3], chunk_refs(1)[3]],
        wmod_refs[3:4],
        wmod_refs[4:5],
        *(w13_refs[2 * a:2 * b] for a, b in zip((0, *CUTS), CUTS)),
        w13_refs[2 * CUTS[-1]:] + [chunk_refs(2)[3], wmod_refs[5], (w2_hbm, w2_v)],
    ]
    start_groups = [[pltpu.make_async_copy(s, d, sem_start.at[n]) for s, d in group]
                    for n, group in enumerate(start_groups)]

    def wait_group(n):
        for cp in start_groups[n]:
            cp.wait()

    def spectrum(even_ref, odd_ref, slot, off, tap0=None):
        e = jnp.dot(fwd_v[0], _halves(even_ref[...]), preferred_element_type=F32)
        t = jnp.dot(fwd_v[1], _halves(odd_ref[...]), preferred_element_type=F32)
        if tap0 is not None:
            e = jnp.concatenate([e[:H] + tap0, e[H:]], axis=0)
        for n, x in enumerate((e + t, e - t)):
            for l in range(D // 128):
                for part in range(2):
                    spec_s[slot, (2 * l + n) * H:(2 * l + n + 1) * H, _lanes(off + part)] = (
                        x[part * H:(part + 1) * H, _lanes(l)])

    def chain(ref, val):
        spare = ref.shape[0] - 16
        at = pl.ds(pl.multiple_of(zero + spare, 16), 16)
        ref[at, _lanes(0)] = val[-16:, _lanes(0)].astype(BF16)

    def ssm_d():
        tiles = [ssmd_v[n:n + 1, :] for n in range(D // 128)]
        return jnp.concatenate(tiles, axis=1).astype(F32)

    def forward_chunk(i, first=False):
        w = [shk_v[j:j + 1, :].astype(F32) for j in range(4)]
        g = 64
        for r in range(0, H, g):
            base = i * C + 2 * r
            kw = _words(k_v[aligned(base, 2 * g + HALO, HALO), :])
            k0, k1, k2 = kw[8:], pltpu.roll(kw, 1, 0)[8:], pltpu.roll(kw, 2, 0)[8:]
            vw = _words(v_v[aligned(base, 2 * g, 2 * g), :])
            ke, ko, ke1, ko1, ko2 = _even(k0), _odd(k0), _even(k1), _odd(k1), _odd(k2)
            kve = (w[0] * ke + w[1] * ko1 + w[2] * ke1 + w[3] * ko2) * _even(vw)
            kvo = (w[0] * ko + w[1] * ke + w[2] * ko1 + w[3] * ke1) * _odd(vw)
            ue_s[r // 2:(r + g) // 2, :] = _to_words(kve)
            uo_s[r // 2:(r + g) // 2, :] = _to_words(kvo)
        yield
        spectrum(ue_s, uo_s, i, 0)
        yield
        tw = _words(ssmk_v[i].T)
        ke_s[...] = _to_words(_even(tw))
        ko_s[...] = _to_words(_odd(tw))
        yield
        spectrum(ke_s, ko_s, i, 2, ssm_d() if first else None)
        yield

    def conv_chunk(i, n_terms, dst=0):
        first = n_terms == 1
        terms = [(jnp.maximum(i - m, 0), m) for m in range(n_terms)]

        def products(row, g):
            re = im = None
            for us, ks in terms:
                ur, ui = spec_s[us, row:row + g, _lanes(0)], spec_s[us, row:row + g, _lanes(1)]
                kr, ki = spec_s[ks, row:row + g, _lanes(2)], spec_s[ks, row:row + g, _lanes(3)]
                pr, pi = ur * kr - ui * ki, ur * ki + ui * kr
                re, im = (pr, pi) if re is None else (re + pr, im + pi)
            return re, im

        g = 8
        for l in range(D // 128):
            for r in range(0, H, g):
                pr, pi = products(2 * l * H + r, g)
                qr, qi = products((2 * l + 1) * H + r, g)
                for n, (re, im) in enumerate(((pr + qr, pi + qi), (pr - qr, pi - qi))):
                    last_re = spec_s.at[prev, l * H + r:l * H + r + g, _lanes(2 * n)]
                    last_im = spec_s.at[prev, l * H + r:l * H + r + g, _lanes(2 * n + 1)]
                    if first:
                        ore, oim = re, im
                    else:
                        lre, lim = last_re[...], last_im[...]
                        ore, oim = (re - lim, im + lre) if r < H // 2 else (re + lim, im - lre)
                    last_re[...] = re
                    last_im[...] = im
                    (ye_s, yo_s)[n][r:r + g, _lanes(l)] = _to_words(
                        jnp.concatenate([ore, oim], axis=0))
                yield
        for n in range(2):
            y_s[dst, n * H:(n + 1) * H, :] = jnp.dot(
                inv_v[n], _halves((ye_s, yo_s)[n][...]), preferred_element_type=F32)
        yield

    def q_rows(i, r, g):
        qw = _words(q_v[aligned(i * C + 2 * r, 2 * g, 2 * g), :])
        return (r, _even(qw)), (H + r, _odd(qw))

    def gate_chunk(i, dst=0, chained=True):
        sa, ca1, ga = (mod_v[n, 0:1, :] for n in range(3))
        scale, shift = ga * ca1, ga * sa
        g = 16
        for r in range(0, H, g):
            for off, x in q_rows(i, r, g):
                val = _layernorm(x) * scale + shift
                gate_s[dst, off:off + g, :] = val
            if chained:
                chain(q_v, val)
        yield

    def residual(i, src, r, g):
        return [(off, x + gate_s[src, off:off + g, :] * y_s[src, off:off + g, :])
                for off, x in q_rows(i, r, g)]

    def store_operands(normed, row):
        sb, cb1 = mod_v[3, 0:1, :], mod_v[4, 0:1, :]
        h2 = [x * cb1 + sb for x in normed]
        lo, hi = row // 2, (row + h2[0].shape[0]) // 2
        blocks = [x[:, l:l + KS // 2] for x in h2 for l in (0, KS // 2)]
        for n, x in enumerate(_left_operands(*blocks)):
            a13_s[n * H + lo:n * H + hi, :] = _to_words(x)
        for n, x in enumerate(h2):
            hr_s[n * H + lo:n * H + hi, :] = _to_words(x[:, KS:])

    def mix_chunk(i, src=0, chained=True):
        g = 64
        for r in range(0, H, g):
            x2 = residual(i, src, r, g)
            for off, x in x2:
                x2n_s[off:off + g, :] = x
            store_operands([_layernorm(x) for _, x in x2], r)
            if chained:
                chain(q_v, x2[1][1])
            yield

    def prepare(i, n_terms):
        yield from forward_chunk(i)
        yield from gate_chunk(i)
        yield from conv_chunk(i, n_terms)
        yield from mix_chunk(i)

    def modulation(n):
        cf = c_v[...].astype(F32)
        sc = jnp.broadcast_to(_silu(cf), (16, D)).astype(BF16)
        m = jnp.dot(sc, wmod_v[n], preferred_element_type=F32)[0:8]
        m = 1.0 + m if n in (1, 4) else m
        mod_v[n] = m * {3: 0.5, 4: 0.5, 5: 2.0}.get(n, 1.0)

    def swiglu(gate, up):
        return (gate * jnp.tanh(gate) + gate) * up

    def store_out(i, cols, src, even, odd):
        gb = mod_v[5, 0:1, cols]
        even = x2_s[src:src + H, cols] + gb * even
        odd = x2_s[src + H:src + C, cols] + gb * odd
        out_v[rows(i), cols] = _interleave(even, odd)

    def right_factors(dst, base, src, row, col, cols):
        for r in range(0, row, 16):
            w = [src[r0 + r:r0 + r + 16, c0 + cols.start:c0 + cols.stop]
                 for r0 in (0, row) for c0 in (0, col)]
            for n, x in enumerate(_right_operands(*(x.astype(F32) for x in w))):
                lo = ((base + n) * row + r) // 2
                dst[lo:lo + 8, cols] = (
                    _words(w[0]) if n == 1 else _words(w[3]) if n == 4 else _to_words(x))

    def ffn_chunk(i, n=1, first=False, last=False):
        m_rows = n * H

        def factor(m, size):
            return slice(m * size, (m + 1) * size)

        def words(m):
            return slice(m * H, m * H + m_rows // 2)

        rest = jnp.concatenate([hr_s[words(0), :], hr_s[words(1), :]], axis=0)
        ft = 128 if first else 256
        early = None
        if not (first or last):
            early = [_dot(rest, r13_s[0, :, c0:c0 + ft]) for c0 in (0, F // 2)]
            yield
        for j in range(0, F // 2, ft):
            cols, cols2 = slice(j, j + ft), slice(F // 2 + j, F // 2 + j + ft)
            pre = []
            for t, w_v in enumerate((w1_v, w3_v)):
                if first:
                    r13_s[t, :, cols] = _words(w_v[KS:, cols])
                    r13_s[t, :, cols2] = _words(w_v[KS:, cols2])
                    right_factors(b13_s, 7 * t, w_v, KS // 2, F // 2, cols)
                c11, c12, c21, c22 = _product_blocks(
                    [_dot(a13_s[words(m), :], b13_s[factor(7 * t + m, KS // 4), cols])
                     for m in range(7)])
                if early is not None and t == j == 0:
                    r1, r2 = early
                else:
                    r1, r2 = _dot(rest, r13_s[t, :, cols]), _dot(rest, r13_s[t, :, cols2])
                pre.append((c11 + r1[:m_rows], c12 + r2[:m_rows],
                            c21 + r1[m_rows:], c22 + r2[m_rows:]))
                yield
            act = [swiglu(gate, up) for gate, up in zip(*pre)]
            for m, x in enumerate(_left_operands(*act) + act[1:3]):
                a2_s[words(m), cols] = _to_words(x)

        if not first:
            x2_s[0:C, :] = x2n_s[...]

        def store(cols, even, odd):
            for t in range(n):
                store_out(i + t, cols, t * C, even[t * H:(t + 1) * H], odd[t * H:(t + 1) * H])

        if first:
            r2_s[...] = _words(w2_v[:, KS:])
        act = jnp.concatenate(
            [jnp.concatenate([a2_s[words(m), :] for m in pair], axis=1)
             for pair in ((2, 7), (8, 3))], axis=0)
        o = _dot(act, r2_s[...])
        store(slice(KS, D), o[:m_rows], o[m_rows:])
        if last:
            last_copies[2].start()
        yield
        if first:
            right_factors(b2_s, 0, w2_v, F // 2, KS // 2, slice(0, KS // 2))
        p = {}
        for m in (0, 1, 2, 4, 5):
            p[m] = _dot(a2_s[words(m), :], b2_s[factor(m, F // 4), :])
            yield
        store(slice(KS // 2, KS), p[2] + p[4], p[0] - p[1] + p[2] + p[5])
        if last:
            last_copies[1].start()
        for m in (3, 6):
            p[m] = _dot(a2_s[words(m), :], b2_s[factor(m, F // 4), :])
            yield
        store(slice(0, KS // 2), p[0] + p[3] - p[4] + p[6], p[1] + p[3])
        if last:
            last_copies[0].start()

    for group in start_groups:
        for cp in group:
            cp.start()
        pl.delay(1)

    def start_chunk(i, carry):
        for cp in chunk_copies(i):
            cp.start()
        return i

    zero = jax.lax.fori_loop(3, n_chunks, start_chunk, 0) - (n_chunks - 1)

    k_v[0:HALO, :] = jnp.zeros((HALO, D), BF16)
    for m in range(3, n_chunks):
        spec_s[m, :, 256:512] = jnp.zeros((spec_s.shape[1], 256), F32)
    conv = [conv_chunk(zero + i, i + 1, i) for i in range(3)]
    order = "A" + "P" * n_mac + "AAAP"
    wait_group(0)
    for n in range(2):
        m = fwd_v[n].astype(F32)
        m = jnp.concatenate([m[f0 + f:f0 + f + 8] for f in range(0, H, 8) for f0 in (0, H)], axis=0)
        inv_v[n] = (m.T * (1.0 / C)).astype(BF16)
    wait_group(1)
    _emit({"A": forward_chunk(0, True)})
    wait_group(2)
    _emit({"A": forward_chunk(1), "P": conv[0]}, order)
    wait_group(3)
    _emit({"A": forward_chunk(2), "P": conv[1]}, order)
    _emit({"P": conv[2]})
    wait_group(4)
    for n in range(3):
        modulation(n)
    _emit({"P": gate_chunk(0, 0, False), "Q": gate_chunk(1, 1, False)})
    for i in range(2):
        for r in range(0, H, 16):
            for off, x in residual(i, i, r, 16):
                x2_s[i * C + off:i * C + off + 16, :] = x
                gate_s[i, off:off + 16, :] = _layernorm(x)
    for n in range(3, 5):
        wait_group(n + 2)
        modulation(n)
    for i in range(2):
        for r in range(0, H, 16):
            store_operands([gate_s[i, off:off + 16, :] for off in (r, H + r)], i * H + r)

    def arrivals():
        for n in range(7, len(start_groups)):
            wait_group(n)
            if n == len(start_groups) - 1:
                modulation(5)
            yield

    def third_chunk():
        yield from gate_chunk(2, 2)
        yield from mix_chunk(2, 2, False)

    _emit({"W": arrivals(), "F": ffn_chunk(0, 2, first=True), "P": third_chunk()},
          "".join("W" + "F" * (b - a) for a, b in zip((0, *CUTS), (*CUTS, 13))) + "P" + "PF" * 7)
    out_copy(0).start()
    out_copy(1).start()

    def step(i, carry):
        for cp in chunk_copies(i + 1):
            cp.wait()
        _emit({"F": ffn_chunk(i), "P": prepare(i + 1, n_chunks)},
              "PF" * 3 + "P" + "F" * 11 + "P" * (n_mac + 2))
        out_copy(i).start()
        return carry

    jax.lax.fori_loop(2, n_chunks - 1, step, 0)
    _emit({"F": ffn_chunk(n_chunks - 1, last=True)})
    for i in range(n_chunks - 1):
        out_copy(i).wait()
    for cp in last_copies:
        cp.wait()


@jax.jit
def pallas_adaLN_cond__ssm_conv_h3__glu_gated_swiglu__prompt_kernel(
    A_q: jax.Array,
    A_k: jax.Array,
    A_v: jax.Array,
    A_shift_k: jax.Array,
    A_ssm_k: jax.Array,
    A_ssm_D: jax.Array,
    B_x: jax.Array,
    B_w1: jax.Array,
    B_w3: jax.Array,
    B_w2: jax.Array,
    c: jax.Array,
    w_mod: jax.Array,
):
    del B_x
    B, S, D = A_q.shape
    F = B_w1.shape[1]
    ks = A_shift_k.shape[1]
    assert B == 1 and ks == 4 and S % C == 0 and D % 128 == 0 and F % 512 == 0
    n_chunks = S // C
    fwd = _dft_matrices()

    vmem = pltpu.VMEM
    scratch = [
        vmem((S + 16, D), BF16),
        vmem((HALO + S, D), BF16),
        vmem((S, D), BF16),
        vmem((n_chunks, D, C), BF16),
        vmem((D, F), BF16), vmem((D, F), BF16), vmem((F, D), BF16),
        vmem((6, D, D), BF16),
        vmem((S, D), BF16),
        vmem((14 * KS // 4, F // 2), U32),
        vmem((2, (D - KS) // 2, F), U32),
        vmem((7 * F // 4, KS // 2), U32),
        vmem((F // 2, D - KS), U32),
        vmem((ks, D), BF16), vmem((D // 128, 128), BF16), vmem((1, D), BF16),
        vmem((2, C, H), BF16), vmem((2, H, C), BF16),
        vmem((6, 8, D), F32),
        *[vmem((H // 2, D), U32)] * 4,
        vmem((n_chunks + 1, D // 128 * C, 4 * 128), F32),
        *[vmem((H, D), U32)] * 2,
        vmem((3, C, D), F32),
        vmem((3, C, D), F32),
        vmem((C, D), F32), vmem((2 * C, D), F32),
        vmem((7 * H, KS // 2), U32),
        vmem((2 * H, D - KS), U32),
        vmem((9 * H, F // 2), U32),
        pltpu.SemaphoreType.DMA((n_chunks - 3,)),
        pltpu.SemaphoreType.DMA((8 + len(CUTS),)),
        pltpu.SemaphoreType.DMA(()),
    ]
    out = pl.pallas_call(
        _kernel,
        out_shape=jax.ShapeDtypeStruct((S, D), A_q.dtype),
        in_specs=[pl.BlockSpec(memory_space=pl.ANY)] * 12,
        out_specs=pl.BlockSpec(memory_space=pl.ANY),
        scratch_shapes=scratch,
        compiler_params=pltpu.CompilerParams(vmem_limit_bytes=100 * 2**20),
    )(A_q.reshape(S, D), A_k.reshape(S, D), A_v.reshape(S, D), A_shift_k.T, A_ssm_k,
      A_ssm_D.reshape(D // 128, 128), B_w1, B_w3, B_w2, c, w_mod, fwd)
    return out.reshape(B, S, D)
```
